```python
import jax
import jax.numpy as jnp

def _softmax(x, axis=-1):
    return jax.nn.softmax(x, axis=axis)
def _gelu(x):
    return jax.nn.gelu(x, approximate=True)
def _silu(x):
    return jax.nn.silu(x)
def _sigmoid(x):
    return jax.nn.sigmoid(x)
def _layernorm(x, axis=-1, eps=1e-5):
    m = jnp.mean(x, axis=axis, keepdims=True)
    v = jnp.var(x, axis=axis, keepdims=True)
    return (x - m) / jnp.sqrt(v + eps)
def _scatter_add(tgt, idx, src, axis=0):
    return tgt.at[idx].add(src)
def _segment_sum(src, seg, n):
    return jax.ops.segment_sum(src, seg, n)
class _Rng:
    def __init__(self, key):
        self._k = key
    def _next(self):
        self._k, sub = jax.random.split(self._k)
        return sub
    def normal(self, shape):
        return jax.random.normal(self._next(), shape, dtype=jnp.bfloat16)
    def randint(self, lo, hi, shape):
        return jax.random.randint(self._next(), shape, lo, hi, dtype=jnp.int32)
    def uniform(self, shape, lo=0.0, hi=1.0):
        return jax.random.uniform(self._next(), shape, jnp.bfloat16, lo, hi)
    def permutation(self, n):
        return jax.random.permutation(self._next(), n)


kernel_name = 'sequential_preLN__compressed_kv_cla__moe_arch_mod__prompt'

def setup_inputs():
    _rng = _Rng(jax.random.key(int.from_bytes(__import__("os").urandom(4), "little")))
    _w = (lambda a: (lambda t: t.astype(jnp.bfloat16) if jnp.issubdtype(t.dtype, jnp.floating) else t)(jnp.asarray(a)))
    def _A_setup():
        B, H, Sq, Sk, D, M = 1, 32, 2048, 2048, 128, 1024
        Dc = 4 * D
        return {
            "x": _w((lambda *s: _rng.normal(s) * 0.05)(B, Sq, M)),
            "c_kv": _w((lambda *s: _rng.normal(s) * 0.05)(B, Sk, Dc)),
            "w_q": _w((lambda *s: _rng.normal(s) * 0.05)(M, H, D) * (M ** -0.5)),
            "w_uk": _w((lambda *s: _rng.normal(s) * 0.05)(Dc, H, D) * (Dc ** -0.5)),
            "w_uv": _w((lambda *s: _rng.normal(s) * 0.05)(Dc, H, D) * (Dc ** -0.5)),
            "w_o": _w((lambda *s: _rng.normal(s) * 0.05)(H, D, M) * ((H * D) ** -0.5)),
        }
    _A_in = _A_setup()

    def _B_setup():
        B, S, D, F, C = 1, 2048, 1024, 3584, 2
        return {
            "x": _w((lambda *s: _rng.normal(s) * 0.05)(B, S, D)),
            "w_r": _w((lambda *s: _rng.normal(s) * 0.05)(D)),
            "w_gate": _w((lambda *s: _rng.normal(s) * 0.05)(D, F)),
            "w_up": _w((lambda *s: _rng.normal(s) * 0.05)(D, F)),
            "w_down": _w((lambda *s: _rng.normal(s) * 0.05)(F, D)),
        }
    _B_in = _B_setup()

    return {
        "A_x": _A_in["x"],
        "A_c_kv": _A_in["c_kv"],
        "A_w_q": _A_in["w_q"],
        "A_w_uk": _A_in["w_uk"],
        "A_w_uv": _A_in["w_uv"],
        "A_w_o": _A_in["w_o"],
        "B_x": _B_in["x"],
        "B_w_r": _B_in["w_r"],
        "B_w_gate": _B_in["w_gate"],
        "B_w_up": _B_in["w_up"],
        "B_w_down": _B_in["w_down"],
    }

def reference(A_x, A_c_kv, A_w_q, A_w_uk, A_w_uv, A_w_o, B_x, B_w_r, B_w_gate, B_w_up, B_w_down):
    def _A_ref(x, c_kv, w_q, w_uk, w_uv, w_o):
        B, Sq, M = x.shape[0], x.shape[1], x.shape[2]
        Sk = c_kv.shape[1]
        H, D = w_q.shape[1], w_q.shape[2]
        q = jnp.einsum("bqm,mhd->bhqd", x, w_q)
        k = jnp.einsum("bkc,chd->bhkd", c_kv, w_uk)
        v = jnp.einsum("bkc,chd->bhkd", c_kv, w_uv)
        scores = jnp.einsum("bhqd,bhkd->bhqk", q, k) * (D ** -0.5)
        off = Sk - Sq
        qi = jnp.arange(Sq)[:, None]
        kj = jnp.arange(Sk)[None, :]
        cmask = kj <= (qi + off)
        scores = jnp.where(cmask[None, None], scores, -1e9)
        p = _softmax(scores, axis=-1)
        ctx = jnp.einsum("bhqk,bhkd->bhqd", p, v)
        return jnp.einsum("bhqd,hdm->bqm", ctx, w_o)

    def _B_ref(x, w_r, w_gate, w_up, w_down):
        B, S, D = x.shape
        C = 2
        r = x @ w_r
        idx = jnp.argsort(-r, axis=-1)[:, :C]
        idx_e = jnp.repeat(idx.reshape(B, C, 1), D, axis=2)
        x_sel = jnp.take_along_axis(x, idx_e, axis=1)
        g = _silu(x_sel @ w_gate)
        u = x_sel @ w_up
        y = (g * u) @ w_down
        r_sel = _sigmoid(jnp.take_along_axis(r, idx, axis=1))
        y = y * r_sel.reshape(B, C, 1)
        b_off = (jnp.arange(B) * S).reshape(B, 1)
        flat_idx = (idx + b_off).reshape(B * C)
        zero = (x * 0.0).reshape(B * S, D)
        upd = _scatter_add(zero, flat_idx, y.reshape(B * C, D), axis=0)
        return x + upd.reshape(B, S, D)

    x = A_x
    h = x + _A_ref(_layernorm(x, axis=-1), A_c_kv, A_w_q, A_w_uk, A_w_uv, A_w_o)
    h2 = h + _B_ref(_layernorm(h, axis=-1), B_w_r, B_w_gate, B_w_up, B_w_down)
    return h2
```

```python
import functools
import math

import jax
import jax.numpy as jnp
from jax import lax
import jax.experimental.pallas as pl
import jax.experimental.pallas.tpu as pltpu

F32 = jnp.float32
BF16 = jnp.bfloat16
NT = (((1,), (1,)), ((), ()))
NEG = -1e30
EPS = 1e-5


def _rb(x):
    return x.astype(BF16).astype(F32)


def _layernorm_rows(xf):
    n = xf.shape[-1]
    mu = jnp.sum(xf, axis=-1, keepdims=True) * (1.0 / n)
    c = xf - mu
    var = jnp.sum(c * c, axis=-1, keepdims=True) * (1.0 / n)
    s = _rb(jnp.sqrt(_rb(_rb(var) + EPS)))
    d = _rb(xf - _rb(mu))
    return _rb(d * (1.0 / s))


def _unpack_pair(u):
    lo = pltpu.bitcast(u << 16, F32).astype(BF16)
    hi = pltpu.bitcast(u & jnp.uint32(0xFFFF0000), F32).astype(BF16)
    return lo, hi


def _attention_head(q, k, v, tq, S):
    outs = [None] * (S // tq)
    row = lax.broadcasted_iota(jnp.int32, (tq, tq), 0)
    col = lax.broadcasted_iota(jnp.int32, (tq, tq), 1)
    causal = col <= row
    for i in range(S // tq):
        qi = q[i * tq:(i + 1) * tq]
        sd = lax.dot_general(qi, k[i * tq:(i + 1) * tq], NT, preferred_element_type=F32)
        sd = jnp.where(causal, sd, NEG)
        if i > 0:
            so = lax.dot_general(qi, k[:i * tq], NT, preferred_element_type=F32)
            s = jnp.concatenate([so, sd], axis=1)
        else:
            s = sd
        m = jnp.max(s, axis=1, keepdims=True)
        p = jnp.exp2(s - m)
        l = jnp.sum(p, axis=1, keepdims=True)
        o = jnp.dot(p.astype(BF16), v[:(i + 1) * tq], preferred_element_type=F32)
        outs[i] = (o * (1.0 / l)).astype(BF16)
    return outs


def _kernel(x_hbm, c_hbm, wq_hbm, wk_hbm, wv_hbm, wo_hbm, wr_ref, wg_hbm, wu_hbm, wd_hbm,
            out_hbm,
            x_buf, xn_buf, c_buf, wq_buf, wk_buf, wv_buf, wo_buf, wg_buf, wu_buf, wd_buf,
            ctx_buf, out_buf, r_buf, sem_in, sem_w, sem_out,
            *, S, M, H, D, TQ, TM):
    NP = H // 2
    scale = (D ** -0.5) * math.log2(math.e)

    wq32 = wq_hbm.bitcast(jnp.uint32)
    wk32 = wk_hbm.bitcast(jnp.uint32)
    wv32 = wv_hbm.bitcast(jnp.uint32)

    def w_copies(p, slot):
        return (
            pltpu.make_async_copy(wk32.at[:, p, :], wk_buf.at[slot], sem_w.at[slot, 0]),
            pltpu.make_async_copy(wv32.at[:, p, :], wv_buf.at[slot], sem_w.at[slot, 1]),
            pltpu.make_async_copy(wq32.at[:, p, :], wq_buf.at[slot], sem_w.at[slot, 2]),
        )

    cp_x = pltpu.make_async_copy(x_hbm, x_buf, sem_in.at[0])
    cp_c = pltpu.make_async_copy(c_hbm, c_buf, sem_in.at[1])
    cp_wo = pltpu.make_async_copy(wo_hbm, wo_buf, sem_in.at[2])
    cp_wg = pltpu.make_async_copy(wg_hbm, wg_buf, sem_in.at[3])
    cp_wu = pltpu.make_async_copy(wu_hbm, wu_buf, sem_in.at[4])
    cp_wd = pltpu.make_async_copy(wd_hbm, wd_buf, sem_in.at[5])

    cp_x.start()
    cp_c.start()
    for cp in w_copies(0, 0):
        cp.start()
    cp_x.wait()

    def ln_body(i, _):
        rows = pl.ds(pl.multiple_of(i * TM, TM), TM)
        xn_buf[rows, :] = _layernorm_rows(x_buf[rows, :].astype(F32)).astype(BF16)
        return 0

    lax.fori_loop(0, S // TM, ln_body, 0)
    cp_c.wait()
    cp_wo.start()
    cp_wg.start()
    cp_wu.start()
    cp_wd.start()

    def pair_body(p, _):
        slot = p % 2
        for cp in w_copies(p, slot):
            cp.wait()

        @pl.when(p + 1 < NP)
        def _():
            for cp in w_copies(p + 1, 1 - slot):
                cp.start()

        wq = _unpack_pair(wq_buf[slot])
        wk = _unpack_pair(wk_buf[slot])
        wv = _unpack_pair(wv_buf[slot])
        for hh in range(2):
            k = jnp.dot(c_buf[...], wk[hh], preferred_element_type=F32).astype(BF16)
            v = jnp.dot(c_buf[...], wv[hh], preferred_element_type=F32).astype(BF16)
            q = (jnp.dot(xn_buf[...], wq[hh], preferred_element_type=F32) * scale).astype(BF16)
            outs = _attention_head(q, k, v, TQ, S)
            for i, o in enumerate(outs):
                ctx_buf[p, i * TQ:(i + 1) * TQ, hh * D:(hh + 1) * D] = o
        return 0

    lax.fori_loop(0, NP, pair_body, 0)

    cp_wo.wait()
    wr8 = jnp.broadcast_to(wr_ref[...], (16, M))

    def out_copy(i):
        rows = pl.ds(pl.multiple_of(i * TM, TM), TM)
        return pltpu.make_async_copy(out_buf.at[rows, :], out_hbm.at[rows, :], sem_out.at[i])

    def proj_body(i, _):
        rows = pl.ds(pl.multiple_of(i * TM, TM), TM)
        ctx = jnp.concatenate([ctx_buf[pp, rows, :] for pp in range(NP)], axis=1)
        a = jnp.dot(ctx, wo_buf[...], preferred_element_type=F32)
        h = _rb(x_buf[rows, :].astype(F32) + _rb(a))
        hn = _layernorm_rows(h)
        x_buf[rows, :] = h.astype(BF16)
        out_buf[rows, :] = (h + hn).astype(BF16)
        r = lax.dot_general(wr8, hn.astype(BF16), NT, preferred_element_type=F32)
        r_buf[i] = r[0:8, :]
        out_copy(i).start()
        return 0

    lax.fori_loop(0, S // TM, proj_body, 0)

    nb = S // TM
    r = jnp.concatenate([r_buf[i] for i in range(nb)], axis=1)
    r = _rb(r)
    r = jnp.where(r != r, -jnp.inf, r)
    pos = lax.broadcasted_iota(jnp.int32, r.shape, 1)
    m1 = jnp.max(r, axis=1, keepdims=True)
    i1v = jnp.min(jnp.where(r == m1, pos, S), axis=1, keepdims=True)
    rest = pos != i1v
    r2 = jnp.where(rest, r, -jnp.inf)
    m2 = jnp.max(r2, axis=1, keepdims=True)
    i2v = jnp.min(jnp.where(jnp.logical_and(r2 == m2, rest), pos, S), axis=1, keepdims=True)
    i1 = jnp.minimum(jnp.max(i1v), S - 1)
    i2 = jnp.minimum(jnp.max(i2v), S - 1)
    b1 = pl.multiple_of((i1 // 16) * 16, 16)
    b2 = pl.multiple_of((i2 // 16) * 16, 16)

    cp_wg.wait()
    cp_wu.wait()
    cp_wd.wait()

    hsel = jnp.concatenate([x_buf[pl.ds(b1, 16), :], x_buf[pl.ds(b2, 16), :]], axis=0).astype(F32)
    hn = _layernorm_rows(hsel)
    xs = hn.astype(BF16)
    g = _rb(jnp.dot(xs, wg_buf[...], preferred_element_type=F32))
    g = _rb(g * _rb(1.0 / (1.0 + jnp.exp(-g))))
    u = _rb(jnp.dot(xs, wu_buf[...], preferred_element_type=F32))
    y = _rb(jnp.dot((g * u).astype(BF16), wd_buf[...], preferred_element_type=F32))
    rsel = jnp.concatenate([jnp.broadcast_to(m1[0:1, :], (16, 1)), jnp.broadcast_to(m2[0:1, :], (16, 1))], axis=0)
    gate = _rb(1.0 / (1.0 + jnp.exp(-rsel)))
    y = _rb(y * gate)
    new = (hsel + _rb(hn + y)).astype(BF16)

    for i in range(nb):
        out_copy(i).wait()

    rid = lax.broadcasted_iota(jnp.int32, (16, M), 0)
    out_buf[pl.ds(b1, 16), :] = jnp.where(rid == i1 - b1, new[0:16], out_buf[pl.ds(b1, 16), :])
    out_buf[pl.ds(b2, 16), :] = jnp.where(rid == i2 - b2, new[16:32], out_buf[pl.ds(b2, 16), :])
    f1 = pltpu.make_async_copy(out_buf.at[pl.ds(b1, 16), :], out_hbm.at[pl.ds(b1, 16), :], sem_out.at[0])
    f2 = pltpu.make_async_copy(out_buf.at[pl.ds(b2, 16), :], out_hbm.at[pl.ds(b2, 16), :], sem_out.at[1])
    f1.start()

    @pl.when(b1 != b2)
    def _():
        f2.start()
        f2.wait()

    f1.wait()


@jax.jit
def pallas_sequential_preLN__compressed_kv_cla__moe_arch_mod__prompt_kernel(
    A_x: jax.Array,
    A_c_kv: jax.Array,
    A_w_q: jax.Array,
    A_w_uk: jax.Array,
    A_w_uv: jax.Array,
    A_w_o: jax.Array,
    B_x: jax.Array,
    B_w_r: jax.Array,
    B_w_gate: jax.Array,
    B_w_up: jax.Array,
    B_w_down: jax.Array,
):
    B, S, M = A_x.shape
    assert B == 1 and A_c_kv.shape[1] == S
    C = A_c_kv.shape[2]
    H, D = A_w_q.shape[1], A_w_q.shape[2]
    F = B_w_gate.shape[1]
    TQ = 256
    TM = 256
    NP = H // 2

    any_spec = pl.BlockSpec(memory_space=pl.ANY)
    out = pl.pallas_call(
        functools.partial(_kernel, S=S, M=M, H=H, D=D, TQ=TQ, TM=TM),
        out_shape=jax.ShapeDtypeStruct((S, M), BF16),
        in_specs=[any_spec] * 6 + [pl.BlockSpec(memory_space=pltpu.VMEM)] + [any_spec] * 3,
        out_specs=any_spec,
        scratch_shapes=[
            pltpu.VMEM((S, M), BF16),
            pltpu.VMEM((S, M), BF16),
            pltpu.VMEM((S, C), BF16),
            pltpu.VMEM((2, M, D), jnp.uint32),
            pltpu.VMEM((2, C, D), jnp.uint32),
            pltpu.VMEM((2, C, D), jnp.uint32),
            pltpu.VMEM((H * D, M), BF16),
            pltpu.VMEM((M, F), BF16),
            pltpu.VMEM((M, F), BF16),
            pltpu.VMEM((F, M), BF16),
            pltpu.VMEM((NP, S, 2 * D), BF16),
            pltpu.VMEM((S, M), BF16),
            pltpu.VMEM((S // TM, 8, TM), F32),
            pltpu.SemaphoreType.DMA((6,)),
            pltpu.SemaphoreType.DMA((2, 3)),
            pltpu.SemaphoreType.DMA((S // TM,)),
        ],
        compiler_params=pltpu.CompilerParams(vmem_limit_bytes=120 * 1024 * 1024),
    )(
        A_x.reshape(S, M), A_c_kv.reshape(S, C), A_w_q, A_w_uk, A_w_uv,
        A_w_o.reshape(H * D, M), B_w_r.reshape(1, M), B_w_gate, B_w_up, B_w_down,
    )
    return out.reshape(B, S, M)
```

```python
import functools
import math

import jax
import jax.numpy as jnp
from jax import lax
import jax.experimental.pallas as pl
import jax.experimental.pallas.tpu as pltpu

F32 = jnp.float32
BF16 = jnp.bfloat16
NT = (((1,), (1,)), ((), ()))
NEG = -1e30
EPS = 1e-5


def _rb(x):
    return x.astype(BF16).astype(F32)


def _layernorm_rows(xf):
    n = xf.shape[-1]
    mu = jnp.sum(xf, axis=-1, keepdims=True) * (1.0 / n)
    c = xf - mu
    var = jnp.sum(c * c, axis=-1, keepdims=True) * (1.0 / n)
    s = _rb(jnp.sqrt(_rb(_rb(var) + EPS)))
    d = _rb(xf - _rb(mu))
    return _rb(d * (1.0 / s))


def _unpack(u, sh):
    return pltpu.bitcast((u << sh) & jnp.uint32(0xFFFF0000), F32).astype(BF16)


def _recip(l):
    r = pl.reciprocal(l, approx=True)
    return r * (2.0 - l * r)


def _kernel(x_hbm, c_hbm, wq_hbm, wk_hbm, wv_hbm, wo_hbm, wr_ref, wg_hbm, wu_hbm, wd_hbm,
            out_hbm,
            x_buf, xn_buf, c_buf, wq_buf, wk_buf, wv_buf, wo_buf, wg_buf, wu_buf, wd_buf,
            q_buf, k_buf, v_buf, ctx_buf, out_buf, r_buf, sem_in, sem_w, sem_out,
            *, S, M, H, D, TQ, TM):
    NP = H // 2
    NB = S // TQ
    scale = (D ** -0.5) * math.log2(math.e)

    wq32 = wq_hbm.bitcast(jnp.uint32)
    wk32 = wk_hbm.bitcast(jnp.uint32)
    wv32 = wv_hbm.bitcast(jnp.uint32)

    def w_copies(p, slot):
        return (
            pltpu.make_async_copy(wk32.at[:, p, :], wk_buf.at[slot], sem_w.at[slot, 0]),
            pltpu.make_async_copy(wv32.at[:, p, :], wv_buf.at[slot], sem_w.at[slot, 1]),
            pltpu.make_async_copy(wq32.at[:, p, :], wq_buf.at[slot], sem_w.at[slot, 2]),
        )

    cp_x = pltpu.make_async_copy(x_hbm, x_buf, sem_in.at[0])
    cp_c = pltpu.make_async_copy(c_hbm, c_buf, sem_in.at[1])
    big = [
        pltpu.make_async_copy(wo_hbm, wo_buf, sem_in.at[2]),
        pltpu.make_async_copy(wg_hbm, wg_buf, sem_in.at[3]),
        pltpu.make_async_copy(wu_hbm, wu_buf, sem_in.at[4]),
        pltpu.make_async_copy(wd_hbm, wd_buf, sem_in.at[5]),
    ]

    def proj_q(i, wq):
        rows = slice(i * TQ, (i + 1) * TQ)
        q_buf[rows, :] = (jnp.dot(xn_buf[rows, :], wq, preferred_element_type=F32) * scale).astype(BF16)

    def proj_k(i, wk):
        rows = slice(i * TQ, (i + 1) * TQ)
        k_buf[rows, :] = jnp.dot(c_buf[rows, :], wk, preferred_element_type=F32).astype(BF16)

    def proj_v(i, wv):
        rows = slice(i * TQ, (i + 1) * TQ)
        v_buf[rows, :] = jnp.dot(c_buf[rows, :], wv, preferred_element_type=F32).astype(BF16)

    def load_w(h):
        slot = (h // 2) % 2
        sh = (16 * (1 - h % 2)).astype(jnp.uint32) if not isinstance(h, int) else jnp.uint32(16 * (1 - h % 2))
        return _unpack(wq_buf[slot], sh), _unpack(wk_buf[slot], sh), _unpack(wv_buf[slot], sh)

    def qk(i):
        row = lax.broadcasted_iota(jnp.int32, (TQ, TQ), 0)
        col = lax.broadcasted_iota(jnp.int32, (TQ, TQ), 1)
        qi = q_buf[i * TQ:(i + 1) * TQ, :]
        sd = lax.dot_general(qi, k_buf[i * TQ:(i + 1) * TQ, :], NT, preferred_element_type=F32)
        sd = jnp.where(col <= row, sd, NEG)
        if i > 0:
            so = lax.dot_general(qi, k_buf[:i * TQ, :], NT, preferred_element_type=F32)
            return jnp.concatenate([so, sd], axis=1)
        return sd

    def softmax(s):
        m = jnp.max(s, axis=1, keepdims=True)
        p = jnp.exp2(s - m)
        l = jnp.sum(p, axis=1, keepdims=True)
        return p.astype(BF16), _recip(l)

    def pv(h, i, p, rl):
        o = jnp.dot(p, v_buf[:(i + 1) * TQ, :], preferred_element_type=F32)
        ctx_buf[h, i * TQ:(i + 1) * TQ, :] = (o * rl).astype(BF16)

    def attention(h, w):
        s = qk(NB - 1)
        for i in range(NB - 1, -1, -1):
            if w is not None:
                proj_q(i, w[0])
                proj_k(i, w[1])
            p, rl = softmax(s)
            if i > 0:
                s = qk(i - 1)
            pv(h, i, p, rl)
            if w is not None:
                proj_v(i, w[2])

    cp_c.start()
    for cp in w_copies(0, 0):
        cp.start()
    cp_x.start()
    cp_x.wait()

    def ln_body(i, _):
        rows = pl.ds(pl.multiple_of(i * TM, TM), TM)
        xn_buf[rows, :] = _layernorm_rows(x_buf[rows, :].astype(F32)).astype(BF16)
        return 0

    lax.fori_loop(0, S // TM, ln_body, 0)
    cp_c.wait()
    for cp in w_copies(0, 0):
        cp.wait()
    for cp in w_copies(1, 1):
        cp.start()
    w0 = load_w(0)
    for i in range(NB):
        proj_k(i, w0[1])
        proj_v(i, w0[2])
        proj_q(i, w0[0])

    def head_body(h, _):
        hn = h + 1
        pn = hn // 2

        @pl.when(hn % 2 == 0)
        def _():
            for cp in w_copies(pn, pn % 2):
                cp.wait()

            @pl.when(pn + 1 < NP)
            def _():
                for cp in w_copies(pn + 1, (pn + 1) % 2):
                    cp.start()

        for j, cp in enumerate(big):
            @pl.when(h == 2 + 2 * j)
            def _():
                cp.start()

        attention(h, load_w(hn))
        return 0

    lax.fori_loop(0, H - 1, head_body, 0)
    attention(H - 1, None)

    big[0].wait()
    wr8 = jnp.broadcast_to(wr_ref[...], (16, M))

    def out_copy(i):
        rows = pl.ds(pl.multiple_of(i * TM, TM), TM)
        return pltpu.make_async_copy(out_buf.at[rows, :], out_hbm.at[rows, :], sem_out.at[i])

    def proj_body(i, _):
        rows = pl.ds(pl.multiple_of(i * TM, TM), TM)
        ctx = jnp.concatenate([ctx_buf[hh, rows, :] for hh in range(H)], axis=1)
        a = jnp.dot(ctx, wo_buf[...], preferred_element_type=F32)
        h = _rb(x_buf[rows, :].astype(F32) + _rb(a))
        hn = _layernorm_rows(h)
        x_buf[rows, :] = h.astype(BF16)
        out_buf[rows, :] = (h + hn).astype(BF16)
        r = lax.dot_general(wr8, hn.astype(BF16), NT, preferred_element_type=F32)
        r_buf[i] = r[0:8, :]
        out_copy(i).start()
        return 0

    lax.fori_loop(0, S // TM, proj_body, 0)

    nb = S // TM
    r = jnp.concatenate([r_buf[i] for i in range(nb)], axis=1)
    r = _rb(r)
    r = jnp.where(r != r, -jnp.inf, r)
    pos = lax.broadcasted_iota(jnp.int32, r.shape, 1)
    m1 = jnp.max(r, axis=1, keepdims=True)
    i1v = jnp.min(jnp.where(r == m1, pos, S), axis=1, keepdims=True)
    rest = pos != i1v
    r2 = jnp.where(rest, r, -jnp.inf)
    m2 = jnp.max(r2, axis=1, keepdims=True)
    i2v = jnp.min(jnp.where(jnp.logical_and(r2 == m2, rest), pos, S), axis=1, keepdims=True)
    i1 = jnp.minimum(jnp.max(i1v), S - 1)
    i2 = jnp.minimum(jnp.max(i2v), S - 1)
    b1 = pl.multiple_of((i1 // 16) * 16, 16)
    b2 = pl.multiple_of((i2 // 16) * 16, 16)

    for cp in big[1:]:
        cp.wait()

    hsel = jnp.concatenate([x_buf[pl.ds(b1, 16), :], x_buf[pl.ds(b2, 16), :]], axis=0).astype(F32)
    hn = _layernorm_rows(hsel)
    xs = hn.astype(BF16)
    g = _rb(jnp.dot(xs, wg_buf[...], preferred_element_type=F32))
    g = _rb(g * _rb(1.0 / (1.0 + jnp.exp(-g))))
    u = _rb(jnp.dot(xs, wu_buf[...], preferred_element_type=F32))
    y = _rb(jnp.dot((g * u).astype(BF16), wd_buf[...], preferred_element_type=F32))
    rsel = jnp.concatenate([jnp.broadcast_to(m1[0:1, :], (16, 1)), jnp.broadcast_to(m2[0:1, :], (16, 1))], axis=0)
    gate = _rb(1.0 / (1.0 + jnp.exp(-rsel)))
    y = _rb(y * gate)
    new = (hsel + _rb(hn + y)).astype(BF16)

    for i in range(nb):
        out_copy(i).wait()

    rid = lax.broadcasted_iota(jnp.int32, (16, M), 0)
    out_buf[pl.ds(b1, 16), :] = jnp.where(rid == i1 - b1, new[0:16], out_buf[pl.ds(b1, 16), :])
    out_buf[pl.ds(b2, 16), :] = jnp.where(rid == i2 - b2, new[16:32], out_buf[pl.ds(b2, 16), :])
    f1 = pltpu.make_async_copy(out_buf.at[pl.ds(b1, 16), :], out_hbm.at[pl.ds(b1, 16), :], sem_out.at[0])
    f2 = pltpu.make_async_copy(out_buf.at[pl.ds(b2, 16), :], out_hbm.at[pl.ds(b2, 16), :], sem_out.at[1])
    f1.start()

    @pl.when(b1 != b2)
    def _():
        f2.start()
        f2.wait()

    f1.wait()


@jax.jit
def pallas_sequential_preLN__compressed_kv_cla__moe_arch_mod__prompt_kernel(
    A_x, A_c_kv, A_w_q, A_w_uk, A_w_uv, A_w_o, B_x, B_w_r, B_w_gate, B_w_up, B_w_down,
):
    B, S, M = A_x.shape
    assert B == 1 and A_c_kv.shape[1] == S
    C = A_c_kv.shape[2]
    H, D = A_w_q.shape[1], A_w_q.shape[2]
    F = B_w_gate.shape[1]
    TQ = 256
    TM = 256

    any_spec = pl.BlockSpec(memory_space=pl.ANY)
    out = pl.pallas_call(
        functools.partial(_kernel, S=S, M=M, H=H, D=D, TQ=TQ, TM=TM),
        out_shape=jax.ShapeDtypeStruct((S, M), BF16),
        in_specs=[any_spec] * 6 + [pl.BlockSpec(memory_space=pltpu.VMEM)] + [any_spec] * 3,
        out_specs=any_spec,
        scratch_shapes=[
            pltpu.VMEM((S, M), BF16),
            pltpu.VMEM((S, M), BF16),
            pltpu.VMEM((S, C), BF16),
            pltpu.VMEM((2, M, D), jnp.uint32),
            pltpu.VMEM((2, C, D), jnp.uint32),
            pltpu.VMEM((2, C, D), jnp.uint32),
            pltpu.VMEM((H * D, M), BF16),
            pltpu.VMEM((M, F), BF16),
            pltpu.VMEM((M, F), BF16),
            pltpu.VMEM((F, M), BF16),
            pltpu.VMEM((S, D), BF16),
            pltpu.VMEM((S, D), BF16),
            pltpu.VMEM((S, D), BF16),
            pltpu.VMEM((H, S, D), BF16),
            pltpu.VMEM((S, M), BF16),
            pltpu.VMEM((S // TM, 8, TM), F32),
            pltpu.SemaphoreType.DMA((6,)),
            pltpu.SemaphoreType.DMA((2, 3)),
            pltpu.SemaphoreType.DMA((S // TM,)),
        ],
        compiler_params=pltpu.CompilerParams(vmem_limit_bytes=120 * 1024 * 1024),
    )(
        A_x.reshape(S, M), A_c_kv.reshape(S, C), A_w_q, A_w_uk, A_w_uv,
        A_w_o.reshape(H * D, M), B_w_r.reshape(1, M), B_w_gate, B_w_up, B_w_down,
    )
    return out.reshape(B, S, M)
```

```python
import functools
import math

import jax
import jax.numpy as jnp
from jax import lax
import jax.experimental.pallas as pl
import jax.experimental.pallas.tpu as pltpu

F32 = jnp.float32
BF16 = jnp.bfloat16
NT = (((1,), (1,)), ((), ()))
NEG = -1e30
EPS = 1e-5


def _rb(x):
    return x.astype(BF16).astype(F32)


def _layernorm_fast(xf):
    n = xf.shape[-1]
    mu = jnp.sum(xf, axis=-1, keepdims=True) * (1.0 / n)
    c = xf - mu
    var = jnp.sum(c * c, axis=-1, keepdims=True) * (1.0 / n)
    return c * lax.rsqrt(var + EPS)


def _unpack(u, odd):
    w = (u & jnp.uint32(0xFFFF0000)) if odd else (u << 16)
    return pltpu.bitcast(w, F32).astype(BF16)


def _recip(l):
    r = pl.reciprocal(l, approx=True)
    return r * (2.0 - l * r)


def _kernel(x_hbm, c_hbm, wq_hbm, wk_hbm, wv_hbm, wo_hbm, wr_hbm, wg_hbm, wu_hbm, wd_hbm,
            out_hbm,
            x_buf, xn_buf, c_buf, wq_buf, wk_buf, wv_buf, wp_q, wp_kv, wr_ref, wo_buf, wg_buf, wu_buf, wd_buf,
            q0, k0, v0, q1, k1, v1, ctx_buf, a_buf, out_buf, r_buf, sem_x, sem_c, sem_big, sem_w, sem_out,
            *, S, M, H, D, TQ, TM, TP, SR):
    NP = H // 2
    NB = S // TQ
    NCH = S // TP
    PB = (S - 1).bit_length()
    assert S == 1 << PB and PB <= 13
    scale = (D ** -0.5) * math.log2(math.e)
    sets = ((q0, k0, v0), (q1, k1, v1))

    wq32 = wq_hbm.bitcast(jnp.uint32)
    wk32 = wk_hbm.bitcast(jnp.uint32)
    wv32 = wv_hbm.bitcast(jnp.uint32)

    def w_copies(p, slot):
        return (
            pltpu.make_async_copy(wk32.at[:, p, :], wk_buf.at[slot], sem_w.at[slot, 0]),
            pltpu.make_async_copy(wv32.at[:, p, :], wv_buf.at[slot], sem_w.at[slot, 1]),
            pltpu.make_async_copy(wq32.at[:, p, :], wq_buf.at[slot], sem_w.at[slot, 2]),
        )

    def chunk_rows(j):
        return pl.ds(j * TP if isinstance(j, int) else pl.multiple_of(j * TP, TP), TP)

    def x_copy(j):
        return pltpu.make_async_copy(x_hbm.at[chunk_rows(j), :], x_buf.at[chunk_rows(j), :], sem_x.at[j])

    big = [
        pltpu.make_async_copy(wo_hbm, wo_buf, sem_big.at[0]),
        pltpu.make_async_copy(wg_hbm, wg_buf, sem_big.at[1]),
        pltpu.make_async_copy(wu_hbm, wu_buf, sem_big.at[2]),
        pltpu.make_async_copy(wd_hbm, wd_buf, sem_big.at[3]),
    ]

    cp_wr = pltpu.make_async_copy(wr_hbm, wr_ref, sem_big.at[4])

    def qk(st, i):
        q_buf, k_buf, _ = st
        row = lax.broadcasted_iota(jnp.int32, (TQ, TQ), 0)
        col = lax.broadcasted_iota(jnp.int32, (TQ, TQ), 1)
        qi = q_buf[i * TQ:(i + 1) * TQ, :]
        sd = lax.dot_general(qi, k_buf[i * TQ:(i + 1) * TQ, :], NT, preferred_element_type=F32)
        sd = jnp.where(col <= row, sd, NEG)
        if i > 0:
            so = lax.dot_general(qi, k_buf[:i * TQ, :], NT, preferred_element_type=F32)
            return jnp.concatenate([so, sd], axis=1)
        return sd

    def softmax(s):
        m = jnp.max(s, axis=1, keepdims=True)
        p = jnp.exp2(s - m).astype(BF16)
        l = jnp.sum(p.astype(F32), axis=1, keepdims=True)
        return p, _recip(l)

    def attention(h, st, w):
        q_buf, k_buf, v_buf = st
        s = qk(st, NB - 1)
        for i in range(NB - 1, -1, -1):
            rows = slice(i * TQ, (i + 1) * TQ)
            if w is not None:
                q_buf[rows, :] = (jnp.dot(xn_buf[rows, :], w[0], preferred_element_type=F32) * scale).astype(BF16)
                k_buf[rows, :] = jnp.dot(c_buf[rows, :], w[1], preferred_element_type=F32).astype(BF16)
            p, rl = softmax(s)
            if i > 0:
                s = qk(st, i - 1)
            o = jnp.dot(p, v_buf[:(i + 1) * TQ, :], preferred_element_type=F32)
            ctx_buf[h, rows, :] = (o * rl).astype(BF16)
            if w is not None:
                v_buf[rows, :] = jnp.dot(c_buf[rows, :], w[2], preferred_element_type=F32).astype(BF16)

    LEAD = tuple(int(v) for v in '256:512'.split(':'))
    L0 = sum(LEAD)
    CR = (S - L0) // NCH
    assert CR * NCH == S - L0 and CR % 16 == 0

    def c_rows(j):
        base = L0 + j * CR
        return pl.ds(base if isinstance(base, int) else pl.multiple_of(base, 16), CR)

    def lead_rows(t):
        return pl.ds(sum(LEAD[:t]), LEAD[t])

    def c_lead_copy(t):
        return pltpu.make_async_copy(c_hbm.at[lead_rows(t), :], c_buf.at[lead_rows(t), :], sem_c.at[NCH + t])

    def c_tail_copy(j):
        return pltpu.make_async_copy(c_hbm.at[c_rows(j), :], c_buf.at[c_rows(j), :], sem_c.at[j])

    w0 = w_copies(0, 0)
    w0[0].start()
    w0[1].start()
    for t in range(len(LEAD)):
        c_lead_copy(t).start(priority=1)
    a_buf[...] = jnp.zeros(a_buf.shape, F32)

    def pro_kv(rows, wkv):
        kv = jnp.dot(c_buf[rows, :], wkv, preferred_element_type=F32).astype(BF16)
        k0[rows, :] = kv[:, 0:D]
        k1[rows, :] = kv[:, D:2 * D]
        v0[rows, :] = kv[:, 2 * D:3 * D]
        v1[rows, :] = kv[:, 3 * D:4 * D]

    w0[0].wait()
    w0[1].wait()
    c_lead_copy(0).wait()
    def issue(j, _):
        x_copy(j).start(priority=1)
        c_tail_copy(j).start(priority=1)
        return 0

    lax.fori_loop(0, NCH, issue, 0)
    wkv = jnp.concatenate([_unpack(wk_buf[0], 0), _unpack(wk_buf[0], 1),
                           _unpack(wv_buf[0], 0), _unpack(wv_buf[0], 1)], axis=1)
    wp_kv[...] = wkv
    pro_kv(lead_rows(0), wkv)
    for t in range(1, len(LEAD)):
        c_lead_copy(t).wait()
        if t == 1:
            w0[2].start()
        pro_kv(lead_rows(t), wp_kv[...])
    w0[2].wait()
    wp_q[...] = jnp.concatenate([_unpack(wq_buf[0], 0), _unpack(wq_buf[0], 1)], axis=1)

    def mid(j, _):
        x_copy(j).wait()
        c_tail_copy(j).wait()

        @pl.when(j == NCH - 2)
        def _():
            for cp in w_copies(1, 1):
                cp.start()
            cp_wr.start()

        rows = chunk_rows(j)
        xn = _layernorm_fast(x_buf[rows, :].astype(F32)).astype(BF16)
        xn_buf[rows, :] = xn
        pro_kv(c_rows(j), wp_kv[...])
        q = (jnp.dot(xn, wp_q[...], preferred_element_type=F32) * scale).astype(BF16)
        q0[rows, :] = q[:, 0:D]
        q1[rows, :] = q[:, D:2 * D]
        return 0

    lax.fori_loop(0, NCH, mid, 0)

    def pair_body(j, _):
        slot = (j + 1) & 1
        for cp in w_copies(j + 1, slot):
            cp.wait()

        @pl.when(j + 2 < NP)
        def _():
            for cp in w_copies(j + 2, 1 - slot):
                cp.start()

        for t, cp in enumerate(big):
            @pl.when(j == t + 1)
            def _():
                cp.start(priority=0)

        for odd in range(2):
            w = (_unpack(wq_buf[slot], odd), _unpack(wk_buf[slot], odd), _unpack(wv_buf[slot], odd))
            attention(2 * j + odd, sets[odd], w)
        return 0

    lax.fori_loop(0, NP - 1, pair_body, 0)
    attention(H - 2, sets[0], None)
    attention(H - 1, sets[1], None)

    big[0].wait()
    cp_wr.wait()
    nb = S // TM
    NS = TM // SR

    def dyn(base, mult):
        return base if isinstance(base, int) else pl.multiple_of(base, mult)

    def out_copy(i):
        rows = pl.ds(dyn(i * TM - SR, SR), TM)
        return pltpu.make_async_copy(out_buf.at[rows, :], out_hbm.at[rows, :], sem_out.at[i])

    first_copy = pltpu.make_async_copy(out_buf.at[pl.ds(0, TM - SR), :], out_hbm.at[pl.ds(0, TM - SR), :], sem_out.at[0])
    last_copy = pltpu.make_async_copy(out_buf.at[pl.ds(S - SR, SR), :], out_hbm.at[pl.ds(S - SR, SR), :], sem_out.at[nb])

    def finish(g, a):
        rows = pl.ds(dyn(g * SR, SR), SR)
        hb = (x_buf[rows, :].astype(F32) + a).astype(BF16)
        h = hb.astype(F32)
        mu = jnp.sum(h, axis=-1, keepdims=True) * (1.0 / M)
        mub = _rb(mu)
        d = h - mub
        dm = mu - mub
        var = jnp.sum(d * d, axis=-1, keepdims=True) * (1.0 / M) - dm * dm
        sd = _rb(jnp.sqrt(_rb(_rb(jnp.maximum(var, 0.0)) + EPS)))
        hnb = (d * _recip(sd)).astype(BF16)
        x_buf[rows, :] = hb
        xn_buf[rows, :] = hnb
        out_buf[rows, :] = (h + hnb.astype(F32)).astype(BF16)
        wr = jnp.broadcast_to(wr_ref[...].reshape(1, M), (16, M))
        r = lax.dot_general(wr, hnb, NT, preferred_element_type=F32)[0:8, :]
        r = _rb(r) + 0.0
        bits = lax.shift_right_logical(pltpu.bitcast(r, jnp.int32), 16)
        o = jnp.where(bits >= 0x8000, bits ^ 0xFFFF, bits ^ 0x8000)
        o = jnp.where(r != r, 0, o)
        pos = g * SR + lax.broadcasted_iota(jnp.int32, r.shape, 1)
        key = (o << PB) | (S - 1 - pos) | 0x20000000
        r_buf[g] = pltpu.bitcast(key, F32)

    def proj_body(i, _):
        a_prev = a_buf[...]
        g_prev = jnp.maximum(i * NS - 1, 0)
        for t in range(NS):
            rows = pl.ds(dyn(i * TM + t * SR, SR), SR)
            KS = 32
            hs = H // KS
            a = None
            for c in range(KS):
                ctx = jnp.concatenate([ctx_buf[hh, rows, :] for hh in range(c * hs, (c + 1) * hs)], axis=1)
                ac = jnp.dot(ctx, wo_buf[c * hs * D:(c + 1) * hs * D, :], preferred_element_type=F32)
                a = ac if a is None else a + ac
            finish(g_prev, a_prev)
            a_prev, g_prev = a, i * NS + t
        a_buf[...] = a_prev

        @pl.when(i == 0)
        def _():
            first_copy.start()

        @pl.when(i > 0)
        def _():
            out_copy(i).start()

        return 0

    lax.fori_loop(0, nb, proj_body, 0)
    finish(S // SR - 1, a_buf[...])
    last_copy.start()

    keys = [r_buf[g] for g in range(S // SR)]
    best = functools.reduce(jnp.maximum, keys)
    k1 = jnp.max(best, axis=1, keepdims=True)
    second = functools.reduce(jnp.maximum, [jnp.where(k == k1, 0.0, k) for k in keys])
    k2 = jnp.max(second, axis=1, keepdims=True)
    kk = pltpu.bitcast(jnp.concatenate([k1, k1, k2, k2], axis=0), jnp.int32)
    idx = S - 1 - (kk & (S - 1))
    i1 = idx[0, 0]
    i2 = idx[16, 0]
    b1 = pl.multiple_of((i1 >> 4) << 4, 16)
    b2 = pl.multiple_of((i2 >> 4) << 4, 16)
    o = (kk >> PB) & 0xFFFF
    rsel = pltpu.bitcast(jnp.where(o >= 0x8000, o ^ 0x8000, o ^ 0xFFFF) << 16, F32)

    for cp in big[1:]:
        cp.wait()

    xs = jnp.concatenate([xn_buf[pl.ds(b1, 16), :], xn_buf[pl.ds(b2, 16), :]], axis=0)
    hsel = jnp.concatenate([x_buf[pl.ds(b1, 16), :], x_buf[pl.ds(b2, 16), :]], axis=0).astype(F32)
    g = _rb(jnp.dot(xs, wg_buf[...], preferred_element_type=F32))
    g = _rb(g * _rb(1.0 / (1.0 + jnp.exp(-g))))
    u = _rb(jnp.dot(xs, wu_buf[...], preferred_element_type=F32))
    gu = (g * u).astype(BF16)
    FF = gu.shape[1]
    y = None
    for t in range(FF // 128):
        yt = jnp.dot(gu[:, t * 128:(t + 1) * 128], wd_buf[t * 128:(t + 1) * 128, :], preferred_element_type=F32)
        y = yt if y is None else y + yt
    gate = _rb(1.0 / (1.0 + jnp.exp(-rsel)))
    y = _rb(_rb(y) * gate)
    new = (hsel + _rb(xs.astype(F32) + y)).astype(BF16)

    first_copy.wait()
    for i in range(1, nb):
        out_copy(i).wait()
    last_copy.wait()

    rid = lax.broadcasted_iota(jnp.int32, (16, M), 0)
    out_buf[pl.ds(b1, 16), :] = jnp.where(rid == i1 - b1, new[0:16], out_buf[pl.ds(b1, 16), :])
    out_buf[pl.ds(b2, 16), :] = jnp.where(rid == i2 - b2, new[16:32], out_buf[pl.ds(b2, 16), :])
    f1 = pltpu.make_async_copy(out_buf.at[pl.ds(b1, 16), :], out_hbm.at[pl.ds(b1, 16), :], sem_out.at[0])
    f2 = pltpu.make_async_copy(out_buf.at[pl.ds(b2, 16), :], out_hbm.at[pl.ds(b2, 16), :], sem_out.at[1])
    f1.start()

    @pl.when(b1 != b2)
    def _():
        f2.start()
        f2.wait()

    f1.wait()


@jax.jit
def pallas_sequential_preLN__compressed_kv_cla__moe_arch_mod__prompt_kernel(
    A_x, A_c_kv, A_w_q, A_w_uk, A_w_uv, A_w_o, B_x, B_w_r, B_w_gate, B_w_up, B_w_down,
):
    B, S, M = A_x.shape
    assert B == 1 and A_c_kv.shape[1] == S
    C = A_c_kv.shape[2]
    H, D = A_w_q.shape[1], A_w_q.shape[2]
    F = B_w_gate.shape[1]
    TQ = 128
    TM = 256
    TP = 256
    SR = 64

    any_spec = pl.BlockSpec(memory_space=pl.ANY)
    out = pl.pallas_call(
        functools.partial(_kernel, S=S, M=M, H=H, D=D, TQ=TQ, TM=TM, TP=TP, SR=SR),
        out_shape=jax.ShapeDtypeStruct((S, M), BF16),
        in_specs=[any_spec] * 10,
        out_specs=any_spec,
        scratch_shapes=[
            pltpu.VMEM((S, M), BF16),
            pltpu.VMEM((S, M), BF16),
            pltpu.VMEM((S, C), BF16),
            pltpu.VMEM((2, M, D), jnp.uint32),
            pltpu.VMEM((2, C, D), jnp.uint32),
            pltpu.VMEM((2, C, D), jnp.uint32),
            pltpu.VMEM((M, 2 * D), BF16),
            pltpu.VMEM((C, 4 * D), BF16),
            pltpu.VMEM((M,), BF16),
            pltpu.VMEM((H * D, M), BF16),
            pltpu.VMEM((M, F), BF16),
            pltpu.VMEM((M, F), BF16),
            pltpu.VMEM((F, M), BF16),
            pltpu.VMEM((S, D), BF16),
            pltpu.VMEM((S, D), BF16),
            pltpu.VMEM((S, D), BF16),
            pltpu.VMEM((S, D), BF16),
            pltpu.VMEM((S, D), BF16),
            pltpu.VMEM((S, D), BF16),
            pltpu.VMEM((H, S, D), BF16),
            pltpu.VMEM((SR, M), F32),
            pltpu.VMEM((S, M), BF16),
            pltpu.VMEM((S // SR, 8, SR), F32),
            pltpu.SemaphoreType.DMA((S // TP,)),
            pltpu.SemaphoreType.DMA((S // TP + 4,)),
            pltpu.SemaphoreType.DMA((5,)),
            pltpu.SemaphoreType.DMA((2, 3)),
            pltpu.SemaphoreType.DMA((S // TM + 1,)),
        ],
        compiler_params=pltpu.CompilerParams(vmem_limit_bytes=120 * 1024 * 1024,
            disable_bounds_checks=True, disable_semaphore_checks=True,
            shape_invariant_numerics=True),
    )(
        A_x.reshape(S, M), A_c_kv.reshape(S, C), A_w_q, A_w_uk, A_w_uv,
        A_w_o.reshape(H * D, M), B_w_r, B_w_gate, B_w_up, B_w_down,
    )
    return out.reshape(B, S, M)
```

```python
import functools
import math

import jax
import jax.numpy as jnp
from jax import lax
import jax.experimental.pallas as pl
import jax.experimental.pallas.tpu as pltpu

F32 = jnp.float32
BF16 = jnp.bfloat16
NT = (((1,), (1,)), ((), ()))
NEG = -1e30
EPS = 1e-5


def _rb(x):
    return x.astype(BF16).astype(F32)


def _layernorm_fast(xf):
    n = xf.shape[-1]
    mu = jnp.sum(xf, axis=-1, keepdims=True) * (1.0 / n)
    c = xf - mu
    var = jnp.sum(c * c, axis=-1, keepdims=True) * (1.0 / n)
    return c * lax.rsqrt(var + EPS)


def _unpack(u, odd):
    w = (u & jnp.uint32(0xFFFF0000)) if odd else (u << 16)
    return pltpu.bitcast(w, F32).astype(BF16)


def _recip(l):
    r = pl.reciprocal(l, approx=True)
    return r * (2.0 - l * r)


def _kernel(*refs, **kw):
    one = refs[-1]
    one[0] = 1

    def body(_, c):
        _body(*refs[:-1], **kw)
        return c

    lax.fori_loop(0, one[0], body, 0)


def _body(x_hbm, c_hbm, wq_hbm, wk_hbm, wv_hbm, wo_hbm, wr_hbm, wg_hbm, wu_hbm, wd_hbm,
            out_hbm,
            x_buf, xn_buf, c_buf, wq_buf, wk_buf, wv_buf, wp_q, wp_kv, wr_ref, wo_buf, wg_buf, wu_buf, wd_buf,
            q_all, k_all, v_all, ctx_buf, a_buf, out_buf, wr_buf, top_buf, sem_x, sem_c, sem_big, sem_w, sem_out,
            *, S, M, H, D, TQ, TM, TP, SR):
    NP = H // 2
    NB = S // TQ
    NCH = S // TP
    PB = (S - 1).bit_length()
    assert S == 1 << PB and PB <= 13
    scale = (D ** -0.5) * math.log2(math.e)
    sets = tuple((q_all.at[o], k_all.at[o], v_all.at[o]) for o in range(2))
    (q0, k0, v0), (q1, k1, v1) = sets

    wq32 = wq_hbm.bitcast(jnp.uint32)
    wk32 = wk_hbm.bitcast(jnp.uint32)
    wv32 = wv_hbm.bitcast(jnp.uint32)

    def w_copies(p, slot):
        return (
            pltpu.make_async_copy(wk32.at[:, p, :], wk_buf.at[slot], sem_w.at[slot, 0]),
            pltpu.make_async_copy(wv32.at[:, p, :], wv_buf.at[slot], sem_w.at[slot, 1]),
            pltpu.make_async_copy(wq32.at[:, p, :], wq_buf.at[slot], sem_w.at[slot, 2]),
        )

    def chunk_rows(j):
        return pl.ds(j * TP if isinstance(j, int) else pl.multiple_of(j * TP, TP), TP)

    def x_copy(j):
        return pltpu.make_async_copy(x_hbm.at[chunk_rows(j), :], x_buf.at[chunk_rows(j), :], sem_x.at[j])

    big = [
        pltpu.make_async_copy(wo_hbm, wo_buf, sem_big.at[0]),
        pltpu.make_async_copy(wg_hbm, wg_buf, sem_big.at[1]),
        pltpu.make_async_copy(wu_hbm, wu_buf, sem_big.at[2]),
        pltpu.make_async_copy(wd_hbm, wd_buf, sem_big.at[3]),
    ]

    cp_wr = pltpu.make_async_copy(wr_hbm, wr_ref, sem_big.at[4])

    def qk(st, i):
        q_buf, k_buf, _ = st
        row = lax.broadcasted_iota(jnp.int32, (TQ, TQ), 0)
        col = lax.broadcasted_iota(jnp.int32, (TQ, TQ), 1)
        qi = q_buf[i * TQ:(i + 1) * TQ, :]
        sd = lax.dot_general(qi, k_buf[i * TQ:(i + 1) * TQ, :], NT, preferred_element_type=F32)
        sd = jnp.where(col <= row, sd, NEG)
        if i > 0:
            so = lax.dot_general(qi, k_buf[:i * TQ, :], NT, preferred_element_type=F32)
            return jnp.concatenate([so, sd], axis=1)
        return sd

    def softmax(s):
        m = jnp.max(s, axis=1, keepdims=True)
        p = jnp.exp2(s - m).astype(BF16)
        l = jnp.sum(p.astype(F32), axis=1, keepdims=True)
        return p, _recip(l)

    def attention(h, st, w):
        q_buf, k_buf, v_buf = st
        s = qk(st, NB - 1)
        for i in range(NB - 1, -1, -1):
            rows = slice(i * TQ, (i + 1) * TQ)
            if w is not None:
                q_buf[rows, :] = (jnp.dot(xn_buf[rows, :], w[0], preferred_element_type=F32) * scale).astype(BF16)
                k_buf[rows, :] = jnp.dot(c_buf[rows, :], w[1], preferred_element_type=F32).astype(BF16)
            p, rl = softmax(s)
            if i > 0:
                s = qk(st, i - 1)
            o = jnp.dot(p, v_buf[:(i + 1) * TQ, :], preferred_element_type=F32)
            ctx_buf[h, i * TQ // 2:(i + 1) * TQ // 2, :] = pltpu.bitcast((o * rl).astype(BF16), jnp.uint32)
            if w is not None:
                v_buf[rows, :] = jnp.dot(c_buf[rows, :], w[2], preferred_element_type=F32).astype(BF16)

    LC = 256
    NL = 3
    WQAT = 1
    L0 = LC * NL
    CR = (S - L0) // NCH
    assert CR * NCH == S - L0 and CR % 16 == 0

    def c_rows(j):
        base = L0 + j * CR
        return pl.ds(base if isinstance(base, int) else pl.multiple_of(base, 16), CR)

    def lead_rows(t):
        return pl.ds(t * LC if isinstance(t, int) else pl.multiple_of(t * LC, LC), LC)

    def c_lead_copy(t):
        return pltpu.make_async_copy(c_hbm.at[lead_rows(t), :], c_buf.at[lead_rows(t), :], sem_c.at[NCH + t])

    def c_tail_copy(j):
        return pltpu.make_async_copy(c_hbm.at[c_rows(j), :], c_buf.at[c_rows(j), :], sem_c.at[j])

    w0 = w_copies(0, 0)
    w0[0].start()
    w0[1].start()
    for t in range(NL):
        c_lead_copy(t).start(priority=1)

    def issue(j, _):
        x_copy(j).start(priority=1)
        c_tail_copy(j).start(priority=1)
        return 0

    lax.fori_loop(0, NCH, issue, 0)
    a_buf[...] = jnp.zeros(a_buf.shape, F32)

    def pro_kv(rows, wkv):
        kv = jnp.dot(c_buf[rows, :], wkv, preferred_element_type=F32).astype(BF16)
        k0[rows, :] = kv[:, 0:D]
        k1[rows, :] = kv[:, D:2 * D]
        v0[rows, :] = kv[:, 2 * D:3 * D]
        v1[rows, :] = kv[:, 3 * D:4 * D]

    w0[0].wait()
    w0[1].wait()
    wp_kv[...] = jnp.concatenate([_unpack(wk_buf[0], 0), _unpack(wk_buf[0], 1),
                                  _unpack(wv_buf[0], 0), _unpack(wv_buf[0], 1)], axis=1)

    def lead(t, _):
        c_lead_copy(t).wait()

        @pl.when(t == WQAT)
        def _():
            w0[2].start()

        pro_kv(lead_rows(t), wp_kv[...])
        return 0

    lax.fori_loop(0, NL, lead, 0)
    w0[2].wait()
    wp_q[...] = jnp.concatenate([_unpack(wq_buf[0], 0), _unpack(wq_buf[0], 1)], axis=1)

    def mid(j, _):
        x_copy(j).wait()
        c_tail_copy(j).wait()

        @pl.when(j == NCH - 2)
        def _():
            for cp in w_copies(1, 1):
                cp.start()
            cp_wr.start()

        NSUB = 1
        tp, cr = TP // NSUB, CR // NSUB
        assert cr % 16 == 0
        for u in range(NSUB):
            rows = pl.ds(pl.multiple_of(j * TP + u * tp, tp), tp)
            xn = _layernorm_fast(x_buf[rows, :].astype(F32)).astype(BF16)
            xn_buf[rows, :] = xn
            pro_kv(pl.ds(pl.multiple_of(L0 + j * CR + u * cr, 16), cr), wp_kv[...])
            q = (jnp.dot(xn, wp_q[...], preferred_element_type=F32) * scale).astype(BF16)
            q0[rows, :] = q[:, 0:D]
            q1[rows, :] = q[:, D:2 * D]
        return 0

    lax.fori_loop(0, NCH, mid, 0)

    def pair_body(j, _):
        slot = (j + 1) & 1
        for cp in w_copies(j + 1, slot):
            cp.wait()

        @pl.when(j + 2 < NP)
        def _():
            for cp in w_copies(j + 2, 1 - slot):
                cp.start()

        for t, cp in enumerate(big):
            @pl.when(j == t + 1)
            def _():
                cp.start(priority=0)

        for odd in range(2):
            w = (_unpack(wq_buf[slot], odd), _unpack(wk_buf[slot], odd), _unpack(wv_buf[slot], odd))
            attention(2 * j + odd, sets[odd], w)
        return 0

    lax.fori_loop(0, NP - 1, pair_body, 0)
    LA = 'mix2'
    LK = 2

    def last_body(o, _):
        st = sets[0]
        order = list(range(NB - 1, -1, -1))
        pend = [qk(st, i) for i in order[:LK]]
        for n, i in enumerate(order):
            rows = slice(i * TQ, (i + 1) * TQ)
            p, rl = softmax(pend.pop(0))
            if n + LK < len(order):
                pend.append(qk(st, order[n + LK]))
            ov = jnp.dot(p, st[2][:(i + 1) * TQ, :], preferred_element_type=F32)
            ctx_buf[H - 2 + o, i * TQ // 2:(i + 1) * TQ // 2, :] = pltpu.bitcast((ov * rl).astype(BF16), jnp.uint32)
            q0[rows, :] = q1[rows, :]
            k0[rows, :] = k1[rows, :]
            v0[rows, :] = v1[rows, :]
        return 0

    lax.fori_loop(0, 2, last_body, 0)

    big[0].wait()
    cp_wr.wait()
    nb = S // TM
    NS = TM // SR

    def dyn(base, mult):
        return base if isinstance(base, int) else pl.multiple_of(base, mult)

    def out_copy(i):
        rows = pl.ds(dyn(i * TM - SR, SR), TM)
        return pltpu.make_async_copy(out_buf.at[rows, :], out_hbm.at[rows, :], sem_out.at[i])

    first_copy = pltpu.make_async_copy(out_buf.at[pl.ds(0, TM - SR), :], out_hbm.at[pl.ds(0, TM - SR), :], sem_out.at[0])
    last_copy = pltpu.make_async_copy(out_buf.at[pl.ds(S - SR, SR), :], out_hbm.at[pl.ds(S - SR, SR), :], sem_out.at[nb])

    P = 16
    NPC = SR // P

    def finish(base, a, top, valid):
        rows = pl.ds(dyn(base, P), P)
        hb = (x_buf[rows, :].astype(F32) + a).astype(BF16)
        x_buf[rows, :] = hb
        h = hb.astype(F32)
        mu = jnp.sum(h, axis=-1, keepdims=True) * (1.0 / M)
        mub = _rb(mu)
        d = h - mub
        dm = mu - mub
        var = jnp.sum(d * d, axis=-1, keepdims=True) * (1.0 / M) - dm * dm
        dw = jnp.sum(d * wr_buf[...], axis=-1, keepdims=True)
        rs = _recip(_rb(jnp.sqrt(_rb(_rb(jnp.maximum(var, 0.0)) + EPS))))
        hnb = (d * rs).astype(BF16)
        xn_buf[rows, :] = hnb
        ob = (h + hnb.astype(F32)).astype(BF16)
        out_buf[rows, :] = ob
        r = _rb(dw * rs) + 0.0
        bits = lax.shift_right_logical(pltpu.bitcast(r, jnp.int32), 16)
        o = jnp.where(bits >= 0x8000, bits ^ 0xFFFF, bits ^ 0x8000)
        o = jnp.where(r != r, 0, o)
        pos = base + lax.broadcasted_iota(jnp.int32, r.shape, 0)
        key = (o << PB) | (S - 1 - pos)
        if valid is not None:
            key = jnp.where(valid, key, -1)
        best, second = top
        top = (jnp.maximum(best, key), jnp.maximum(second, jnp.minimum(best, key)))
        return top, ob

    def tie(x, dep):
        z = pltpu.bitcast(dep, jnp.uint32)
        z = functools.reduce(jnp.bitwise_or, [z[:, t * D:(t + 1) * D] for t in range(M // D)])
        z = lax.shift_right_logical(lax.shift_right_logical(z, jnp.uint32(16)), jnp.uint32(16))
        xu = pltpu.bitcast(x, jnp.uint32)
        n = z.shape[0]
        return pltpu.bitcast(jnp.concatenate([xu[:n] | z, xu[n:]], axis=0), BF16)

    wr_buf[...] = wr_ref[...].reshape(1, M).astype(F32)
    top_buf[...] = jnp.full(top_buf.shape, -1, jnp.int32)
    TOFF = 1

    def proj_body(i, _):
        top = (top_buf[0], top_buf[1])
        for t in range(NS):
            rows = pl.ds(dyn(i * (TM // 2) + t * (SR // 2), SR // 2), SR // 2)
            prev = jnp.maximum(i * TM - SR, 0) if t == 0 else i * TM + (t - 1) * SR
            a = None
            KS = 32
            hs = H // KS
            for c in range(KS):
                ctx = [pltpu.bitcast(ctx_buf[hh, rows, :], BF16) for hh in range(c * hs, (c + 1) * hs)]
                if (c + TOFF) % (KS // NPC) == 0:
                    j = (c + TOFF) // (KS // NPC) - 1
                    top, ob = finish(prev + j * P, a_buf[j * P:(j + 1) * P, :], top, (i > 0) if t == 0 else None)
                    ctx[0] = tie(ctx[0], ob)
                ctx = jnp.concatenate(ctx, axis=1) if hs > 1 else ctx[0]
                ac = jnp.dot(ctx, wo_buf[c * hs * D:(c + 1) * hs * D, :], preferred_element_type=F32)
                a = ac if a is None else a + ac
            a_buf[...] = a
        top_buf[0] = top[0]
        top_buf[1] = top[1]

        @pl.when(i == 0)
        def _():
            first_copy.start()

        @pl.when(i > 0)
        def _():
            out_copy(i).start()

        return 0

    lax.fori_loop(0, nb, proj_body, 0)
    for cp in big[1:]:
        cp.wait()
    top = (top_buf[0], top_buf[1])
    for j in range(NPC):
        top, _ = finish(S - SR + j * P, a_buf[j * P:(j + 1) * P, :], top, None)
    last_copy.start()

    best, second = top
    k1 = jnp.max(best, axis=0, keepdims=True)
    k2 = jnp.max(jnp.where(best == k1, second, best), axis=0, keepdims=True)
    kk = jnp.concatenate([jnp.broadcast_to(k1, (16, 1)), jnp.broadcast_to(k2, (16, 1))], axis=0)
    i1 = S - 1 - (k1[0, 0] & (S - 1))
    i2 = S - 1 - (k2[0, 0] & (S - 1))
    b1 = pl.multiple_of((i1 >> 4) << 4, 16)
    b2 = pl.multiple_of((i2 >> 4) << 4, 16)
    o = (kk >> PB) & 0xFFFF
    rsel = pltpu.bitcast(jnp.where(o >= 0x8000, o ^ 0x8000, o ^ 0xFFFF) << 16, F32)

    xs = jnp.concatenate([xn_buf[pl.ds(b1, 16), :], xn_buf[pl.ds(b2, 16), :]], axis=0)
    hsel = jnp.concatenate([x_buf[pl.ds(b1, 16), :], x_buf[pl.ds(b2, 16), :]], axis=0).astype(F32)
    g = _rb(jnp.dot(xs, wg_buf[...], preferred_element_type=F32))
    g = _rb(g * _rb(1.0 / (1.0 + jnp.exp(-g))))
    u = _rb(jnp.dot(xs, wu_buf[...], preferred_element_type=F32))
    gu = (g * u).astype(BF16)
    FF = gu.shape[1]
    y = None
    for t in range(FF // 128):
        yt = jnp.dot(gu[:, t * 128:(t + 1) * 128], wd_buf[t * 128:(t + 1) * 128, :], preferred_element_type=F32)
        y = yt if y is None else y + yt
    gate = _rb(1.0 / (1.0 + jnp.exp(-rsel)))
    y = _rb(_rb(y) * gate)
    new = (hsel + _rb(xs.astype(F32) + y)).astype(BF16)

    first_copy.wait()
    for i in range(1, nb):
        out_copy(i).wait()
    last_copy.wait()

    rid = lax.broadcasted_iota(jnp.int32, (16, M), 0)
    out_buf[pl.ds(b1, 16), :] = jnp.where(rid == i1 - b1, new[0:16], out_buf[pl.ds(b1, 16), :])
    out_buf[pl.ds(b2, 16), :] = jnp.where(rid == i2 - b2, new[16:32], out_buf[pl.ds(b2, 16), :])
    f1 = pltpu.make_async_copy(out_buf.at[pl.ds(b1, 16), :], out_hbm.at[pl.ds(b1, 16), :], sem_out.at[0])
    f2 = pltpu.make_async_copy(out_buf.at[pl.ds(b2, 16), :], out_hbm.at[pl.ds(b2, 16), :], sem_out.at[1])
    f1.start()

    @pl.when(b1 != b2)
    def _():
        f2.start()
        f2.wait()

    f1.wait()


@jax.jit
def pallas_sequential_preLN__compressed_kv_cla__moe_arch_mod__prompt_kernel(
    A_x, A_c_kv, A_w_q, A_w_uk, A_w_uv, A_w_o, B_x, B_w_r, B_w_gate, B_w_up, B_w_down,
):
    B, S, M = A_x.shape
    assert B == 1 and A_c_kv.shape[1] == S
    C = A_c_kv.shape[2]
    H, D = A_w_q.shape[1], A_w_q.shape[2]
    F = B_w_gate.shape[1]
    TQ = 128
    TM = 256
    TP = 256
    SR = 64

    any_spec = pl.BlockSpec(memory_space=pl.ANY)
    out = pl.pallas_call(
        functools.partial(_kernel, S=S, M=M, H=H, D=D, TQ=TQ, TM=TM, TP=TP, SR=SR),
        out_shape=jax.ShapeDtypeStruct((S, M), BF16),
        in_specs=[any_spec] * 10,
        out_specs=any_spec,
        scratch_shapes=[
            pltpu.VMEM((S, M), BF16),
            pltpu.VMEM((S, M), BF16),
            pltpu.VMEM((S, C), BF16),
            pltpu.VMEM((2, M, D), jnp.uint32),
            pltpu.VMEM((2, C, D), jnp.uint32),
            pltpu.VMEM((2, C, D), jnp.uint32),
            pltpu.VMEM((M, 2 * D), BF16),
            pltpu.VMEM((C, 4 * D), BF16),
            pltpu.VMEM((M,), BF16),
            pltpu.VMEM((H * D, M), BF16),
            pltpu.VMEM((M, F), BF16),
            pltpu.VMEM((M, F), BF16),
            pltpu.VMEM((F, M), BF16),
            pltpu.VMEM((2, S, D), BF16),
            pltpu.VMEM((2, S, D), BF16),
            pltpu.VMEM((2, S, D), BF16),
            pltpu.VMEM((H, S // 2, D), jnp.uint32),
            pltpu.VMEM((SR, M), F32),
            pltpu.VMEM((S, M), BF16),
            pltpu.VMEM((1, M), F32),
            pltpu.VMEM((2, 16, 1), jnp.int32),
            pltpu.SemaphoreType.DMA((S // TP,)),
            pltpu.SemaphoreType.DMA((S // TP + 3,)),
            pltpu.SemaphoreType.DMA((5,)),
            pltpu.SemaphoreType.DMA((2, 3)),
            pltpu.SemaphoreType.DMA((S // TM + 1,)),
            pltpu.SMEM((1,), jnp.int32),
        ],
        compiler_params=pltpu.CompilerParams(vmem_limit_bytes=120 * 1024 * 1024,
            disable_bounds_checks=True, disable_semaphore_checks=True,
            shape_invariant_numerics=True),
    )(
        A_x.reshape(S, M), A_c_kv.reshape(S, C), A_w_q, A_w_uk, A_w_uv,
        A_w_o.reshape(H * D, M), B_w_r, B_w_gate, B_w_up, B_w_down,
    )
    return out.reshape(B, S, M)
```

```python
import functools
import math

import jax
import jax.numpy as jnp
from jax import lax
import jax.experimental.pallas as pl
import jax.experimental.pallas.tpu as pltpu

F32 = jnp.float32
BF16 = jnp.bfloat16
NT = (((1,), (1,)), ((), ()))
NEG = -1e30
EPS = 1e-5


def _rb(x):
    return x.astype(BF16).astype(F32)


def _layernorm_fast(xf):
    n = xf.shape[-1]
    mu = jnp.sum(xf, axis=-1, keepdims=True) * (1.0 / n)
    c = xf - mu
    var = jnp.sum(c * c, axis=-1, keepdims=True) * (1.0 / n)
    return c * lax.rsqrt(var + EPS)


def _unpack(u, odd):
    w = (u & jnp.uint32(0xFFFF0000)) if odd else (u << 16)
    return pltpu.bitcast(w, F32).astype(BF16)


def _recip(l):
    r = pl.reciprocal(l, approx=True)
    return r * (2.0 - l * r)


def _kernel(*refs, **kw):
    one = refs[-1]
    one[0] = 1

    def body(_, c):
        _body(*refs[:-1], **kw)
        return c

    lax.fori_loop(0, one[0], body, 0)


def _body(x_hbm, c_hbm, wq_hbm, wk_hbm, wv_hbm, wo_hbm, wr_hbm, wg_hbm, wu_hbm, wd_hbm,
            out_hbm,
            x_buf, xn_buf, c_buf, w_buf, wp_q, wp_kv, wr_ref, wo_buf, wg_buf, wu_buf, wd_buf,
            q_all, k_all, v_all, ctx_buf, a_buf, out_buf, wr_buf, top_buf, sem_x, sem_c, sem_big, sem_w, sem_out,
            *, S, M, H, D, TQ, TM, TP, SR):
    NP = H // 2
    NB = S // TQ
    NCH = S // TP
    PB = (S - 1).bit_length()
    assert S == 1 << PB and PB <= 13
    scale = (D ** -0.5) * math.log2(math.e)
    sets = tuple((q_all.at[o], k_all.at[o], v_all.at[o]) for o in range(2))
    (q0, k0, v0), (q1, k1, v1) = sets

    wq32 = wq_hbm.bitcast(jnp.uint32)
    wk32 = wk_hbm.bitcast(jnp.uint32)
    wv32 = wv_hbm.bitcast(jnp.uint32)

    C = c_buf.shape[1]
    QR, KR, VR = pl.ds(0, M), pl.ds(M, C), pl.ds(M + C, C)

    def w_copies(p, slot, sems=None):
        sems = sems or [sem_w.at[slot]] * 3
        return (
            pltpu.make_async_copy(wk32.at[:, p, :], w_buf.at[slot, KR, :], sems[0]),
            pltpu.make_async_copy(wv32.at[:, p, :], w_buf.at[slot, VR, :], sems[1]),
            pltpu.make_async_copy(wq32.at[:, p, :], w_buf.at[slot, QR, :], sems[2]),
        )

    def w_wait(slot):
        pltpu.make_async_copy(w_buf.at[slot], w_buf.at[slot], sem_w.at[slot]).wait()

    def chunk_rows(j):
        return pl.ds(j * TP if isinstance(j, int) else pl.multiple_of(j * TP, TP), TP)

    def x_copy(j):
        return pltpu.make_async_copy(x_hbm.at[chunk_rows(j), :], x_buf.at[chunk_rows(j), :], sem_x.at[j])

    big = [
        pltpu.make_async_copy(wo_hbm, wo_buf, sem_big.at[0]),
        pltpu.make_async_copy(wg_hbm, wg_buf, sem_big.at[1]),
        pltpu.make_async_copy(wu_hbm, wu_buf, sem_big.at[2]),
        pltpu.make_async_copy(wd_hbm, wd_buf, sem_big.at[3]),
    ]

    cp_wr = pltpu.make_async_copy(wr_hbm, wr_ref, sem_big.at[4])

    def qk(st, i):
        q_buf, k_buf, _ = st
        row = lax.broadcasted_iota(jnp.int32, (TQ, TQ), 0)
        col = lax.broadcasted_iota(jnp.int32, (TQ, TQ), 1)
        qi = q_buf[i * TQ:(i + 1) * TQ, :]
        sd = lax.dot_general(qi, k_buf[i * TQ:(i + 1) * TQ, :], NT, preferred_element_type=F32)
        sd = jnp.where(col <= row, sd, NEG)
        if i > 0:
            so = lax.dot_general(qi, k_buf[:i * TQ, :], NT, preferred_element_type=F32)
            return jnp.concatenate([so, sd], axis=1)
        return sd

    def softmax(s):
        m = jnp.max(s, axis=1, keepdims=True)
        p = jnp.exp2(s - m).astype(BF16)
        l = jnp.sum(p.astype(F32), axis=1, keepdims=True)
        return p, _recip(l)

    FIRST = 'k'

    def attention(h, st, w, first):
        q_buf, k_buf, v_buf = st

        def pq(rows):
            return (jnp.dot(xn_buf[rows, :], w[0], preferred_element_type=F32) * scale).astype(BF16)

        def pk(rows):
            return jnp.dot(c_buf[rows, :], w[1], preferred_element_type=F32).astype(BF16)

        def pv(rows):
            return jnp.dot(c_buf[rows, :], w[2], preferred_element_type=F32).astype(BF16)

        top = slice(S - TQ, S)
        early = {}
        if first and FIRST != 'none':
            early[FIRST] = {'q': pq, 'k': pk, 'v': pv}[FIRST](top)
        s = qk(st, NB - 1)
        for i in range(NB - 1, -1, -1):
            rows = slice(i * TQ, (i + 1) * TQ)
            q_buf[rows, :] = early.pop('q') if 'q' in early else pq(rows)
            k_buf[rows, :] = early.pop('k') if 'k' in early else pk(rows)
            p, rl = softmax(s)
            if i > 0:
                s = qk(st, i - 1)
            o = jnp.dot(p, v_buf[:(i + 1) * TQ, :], preferred_element_type=F32)
            ctx_buf[h, i * TQ // 2:(i + 1) * TQ // 2, :] = pltpu.bitcast((o * rl).astype(BF16), jnp.uint32)
            v_buf[rows, :] = early.pop('v') if 'v' in early else pv(rows)

    LC = 256
    NL = 3
    WQAT = 1
    L0 = LC * NL
    CR = (S - L0) // NCH
    assert CR * NCH == S - L0 and CR % 16 == 0

    def c_rows(j):
        base = L0 + j * CR
        return pl.ds(base if isinstance(base, int) else pl.multiple_of(base, 16), CR)

    def lead_rows(t):
        return pl.ds(t * LC if isinstance(t, int) else pl.multiple_of(t * LC, LC), LC)

    def c_lead_copy(t):
        return pltpu.make_async_copy(c_hbm.at[lead_rows(t), :], c_buf.at[lead_rows(t), :], sem_c.at[NCH + t])

    def c_tail_copy(j):
        return pltpu.make_async_copy(c_hbm.at[c_rows(j), :], c_buf.at[c_rows(j), :], sem_c.at[j])

    w0 = w_copies(0, 0, [sem_w.at[2], sem_w.at[3], sem_w.at[4]])
    w0[0].start()
    w0[1].start()
    for t in range(NL):
        c_lead_copy(t).start(priority=1)

    def issue(j, _):
        x_copy(j).start(priority=1)
        c_tail_copy(j).start(priority=1)
        return 0

    lax.fori_loop(0, NCH, issue, 0)
    a_buf[...] = jnp.zeros(a_buf.shape, F32)

    def pro_kv(rows, wkv):
        kv = jnp.dot(c_buf[rows, :], wkv, preferred_element_type=F32).astype(BF16)
        k0[rows, :] = kv[:, 0:D]
        k1[rows, :] = kv[:, D:2 * D]
        v0[rows, :] = kv[:, 2 * D:3 * D]
        v1[rows, :] = kv[:, 3 * D:4 * D]

    w0[0].wait()
    w0[1].wait()
    wp_kv[...] = jnp.concatenate([_unpack(w_buf[0, KR, :], 0), _unpack(w_buf[0, KR, :], 1),
                                  _unpack(w_buf[0, VR, :], 0), _unpack(w_buf[0, VR, :], 1)], axis=1)

    def lead(t, _):
        c_lead_copy(t).wait()

        @pl.when(t == WQAT)
        def _():
            w0[2].start()

        pro_kv(lead_rows(t), wp_kv[...])
        return 0

    lax.fori_loop(0, NL, lead, 0)
    w0[2].wait()
    wp_q[...] = jnp.concatenate([_unpack(w_buf[0, QR, :], 0), _unpack(w_buf[0, QR, :], 1)], axis=1)

    def mid(j, _):
        x_copy(j).wait()
        c_tail_copy(j).wait()

        @pl.when(j == NCH - 2)
        def _():
            for cp in w_copies(1, 1):
                cp.start()
            cp_wr.start()

        NSUB = 1
        tp, cr = TP // NSUB, CR // NSUB
        assert cr % 16 == 0
        for u in range(NSUB):
            rows = pl.ds(pl.multiple_of(j * TP + u * tp, tp), tp)
            xn = _layernorm_fast(x_buf[rows, :].astype(F32)).astype(BF16)
            xn_buf[rows, :] = xn
            pro_kv(pl.ds(pl.multiple_of(L0 + j * CR + u * cr, 16), cr), wp_kv[...])
            q = (jnp.dot(xn, wp_q[...], preferred_element_type=F32) * scale).astype(BF16)
            q0[rows, :] = q[:, 0:D]
            q1[rows, :] = q[:, D:2 * D]
        return 0

    lax.fori_loop(0, NCH, mid, 0)

    def pair_body(j, _):
        slot = (j + 1) & 1
        w_wait(slot)

        def issue_next():
            @pl.when(j + 2 < NP)
            def _():
                for cp in w_copies(j + 2, 1 - slot):
                    cp.start()

            for t, cp in enumerate(big):
                @pl.when(j == t + 1)
                def _():
                    cp.start(priority=1)

        for odd in range(2):
            w = tuple(_unpack(w_buf[slot, r, :], odd) for r in (QR, KR, VR))
            if odd == 0:
                issue_next()
            attention(2 * j + odd, sets[odd], w, odd == 0)
        return 0

    lax.fori_loop(0, NP - 1, pair_body, 0)
    LA = 'mix2'
    LK = 2

    def last_body(o, _):
        st = sets[0]
        order = list(range(NB - 1, -1, -1))
        pend = [qk(st, i) for i in order[:LK]]
        for n, i in enumerate(order):
            rows = slice(i * TQ, (i + 1) * TQ)
            p, rl = softmax(pend.pop(0))
            if n + LK < len(order):
                pend.append(qk(st, order[n + LK]))
            ov = jnp.dot(p, st[2][:(i + 1) * TQ, :], preferred_element_type=F32)
            ctx_buf[H - 2 + o, i * TQ // 2:(i + 1) * TQ // 2, :] = pltpu.bitcast((ov * rl).astype(BF16), jnp.uint32)
            q0[rows, :] = q1[rows, :]
            k0[rows, :] = k1[rows, :]
            v0[rows, :] = v1[rows, :]
        return 0

    lax.fori_loop(0, 2, last_body, 0)

    big[0].wait()
    cp_wr.wait()
    nb = S // TM
    NS = TM // SR

    def dyn(base, mult):
        return base if isinstance(base, int) else pl.multiple_of(base, mult)

    def out_copy(i):
        rows = pl.ds(dyn(i * TM - SR, SR), TM)
        return pltpu.make_async_copy(out_buf.at[rows, :], out_hbm.at[rows, :], sem_out.at[i])

    first_copy = pltpu.make_async_copy(out_buf.at[pl.ds(0, TM - SR), :], out_hbm.at[pl.ds(0, TM - SR), :], sem_out.at[0])
    last_copy = pltpu.make_async_copy(out_buf.at[pl.ds(S - SR, SR), :], out_hbm.at[pl.ds(S - SR, SR), :], sem_out.at[nb])

    P = 16
    NPC = SR // P

    def zero_of(x):
        z = pltpu.bitcast(x, jnp.uint32)
        return lax.shift_right_logical(lax.shift_right_logical(z, jnp.uint32(16)), jnp.uint32(16))

    def finish(base, a):
        rows = pl.ds(dyn(base, P), P)
        hb = (x_buf[rows, :].astype(F32) + a).astype(BF16)
        x_buf[rows, :] = hb
        h = hb.astype(F32)
        mu = jnp.sum(h, axis=-1, keepdims=True) * (1.0 / M)
        mub = _rb(mu)
        d = h - mub
        dm = mu - mub
        var = jnp.sum(d * d, axis=-1, keepdims=True) * (1.0 / M) - dm * dm
        dw = jnp.sum(d * wr_buf[...], axis=-1, keepdims=True)
        rs = _recip(_rb(jnp.sqrt(_rb(_rb(jnp.maximum(var, 0.0)) + EPS))))
        if 0:
            rs = pltpu.bitcast(pltpu.bitcast(rs, jnp.uint32) | zero_of(dw), F32)
        hnb = (d * rs).astype(BF16)
        xn_buf[rows, :] = hnb
        ob = (h + hnb.astype(F32)).astype(BF16)
        out_buf[rows, :] = ob
        return dw * rs, ob

    def make_key(r, pos):
        r = _rb(r) + 0.0
        bits = lax.shift_right_logical(pltpu.bitcast(r, jnp.int32), 16)
        o = jnp.where(bits >= 0x8000, bits ^ 0xFFFF, bits ^ 0x8000)
        o = jnp.where(r != r, 0, o)
        return pltpu.bitcast((o << PB) | (S - 1 - pos) | 0x20000000, F32)

    def merge(top, key):
        best, second = top
        return jnp.maximum(best, key), jnp.maximum(second, jnp.minimum(best, key))

    def tie(x, dep):
        z = pltpu.bitcast(dep, jnp.uint32)
        z = functools.reduce(jnp.bitwise_or, [z[:, t * D:(t + 1) * D] for t in range(M // D)])
        z = lax.shift_right_logical(lax.shift_right_logical(z, jnp.uint32(16)), jnp.uint32(16))
        xu = pltpu.bitcast(x, jnp.uint32)
        n = z.shape[0]
        return pltpu.bitcast(jnp.concatenate([xu[:n] | z, xu[n:]], axis=0), BF16)

    wr_buf[...] = wr_ref[...].reshape(1, M).astype(F32)
    top_buf[...] = jnp.zeros(top_buf.shape, F32)
    TOFF = 1

    def proj_body(i, _):
        lane = lax.broadcasted_iota(jnp.int32, (P, D), 1)
        rmat = jnp.zeros((P, D), F32)
        for t in range(NS):
            rows = pl.ds(dyn(i * (TM // 2) + t * (SR // 2), SR // 2), SR // 2)
            prev = jnp.maximum(i * TM - SR, 0) if t == 0 else i * TM + (t - 1) * SR
            a = None
            KS = 32
            GL = 6
            hs = H // KS
            hist = []
            for c in range(KS):
                ctx = [pltpu.bitcast(ctx_buf[hh, rows, :], BF16) for hh in range(c * hs, (c + 1) * hs)]
                if (c + TOFF) % (KS // NPC) == 0:
                    j = (c + TOFF) // (KS // NPC) - 1
                    ap = a_buf[j * P:(j + 1) * P, :]
                    if GL and c - GL >= 0:
                        z = pltpu.bitcast(hist[c - GL][0:P, 0:D], jnp.uint32)
                        z = lax.shift_right_logical(lax.shift_right_logical(z, jnp.uint32(16)), jnp.uint32(16))
                        ap = pltpu.bitcast(pltpu.bitcast(ap, jnp.uint32) | jnp.concatenate([z] * (M // D), axis=1), F32)
                    r, ob = finish(prev + j * P, ap)
                    rmat = jnp.where(lane == t * NPC + j, r, rmat)
                    ctx[0] = tie(ctx[0], ob)
                ctx = jnp.concatenate(ctx, axis=1) if hs > 1 else ctx[0]
                ac = jnp.dot(ctx, wo_buf[c * hs * D:(c + 1) * hs * D, :], preferred_element_type=F32)
                a = ac if a is None else a + ac
                hist.append(a)
            a_buf[...] = a
        pos = i * TM - SR + lane * P + lax.broadcasted_iota(jnp.int32, (P, D), 0)
        live = jnp.logical_and(pos >= 0, lane < TM // P)
        top = merge((top_buf[0], top_buf[1]), jnp.where(live, make_key(rmat, pos), 0.0))
        top_buf[0] = top[0]
        top_buf[1] = top[1]

        @pl.when(i == 0)
        def _():
            first_copy.start()

        @pl.when(i > 0)
        def _():
            out_copy(i).start()

        return 0

    lax.fori_loop(0, nb, proj_body, 0)
    for cp in big[1:]:
        cp.wait()
    best, second = top_buf[0], top_buf[1]
    b = jnp.max(best, axis=1, keepdims=True)
    top = (b, jnp.max(jnp.where(best == b, second, best), axis=1, keepdims=True))
    for j in range(NPC):
        base = S - SR + j * P
        r, _ = finish(base, a_buf[j * P:(j + 1) * P, :])
        top = merge(top, make_key(r, base + lax.broadcasted_iota(jnp.int32, (P, 1), 0)))
    last_copy.start()

    best, second = top
    k1 = jnp.max(best, axis=0, keepdims=True)
    k2 = jnp.max(jnp.where(best == k1, second, best), axis=0, keepdims=True)
    kk = jnp.concatenate([jnp.broadcast_to(k1, (16, 1)), jnp.broadcast_to(k2, (16, 1))], axis=0)
    kk = pltpu.bitcast(kk, jnp.int32)
    i1 = S - 1 - (kk[0, 0] & (S - 1))
    i2 = S - 1 - (kk[16, 0] & (S - 1))
    b1 = pl.multiple_of((i1 >> 4) << 4, 16)
    b2 = pl.multiple_of((i2 >> 4) << 4, 16)
    o = (kk >> PB) & 0xFFFF
    rsel = pltpu.bitcast(jnp.where(o >= 0x8000, o ^ 0x8000, o ^ 0xFFFF) << 16, F32)

    xs = jnp.concatenate([xn_buf[pl.ds(b1, 16), :], xn_buf[pl.ds(b2, 16), :]], axis=0)
    hsel = jnp.concatenate([x_buf[pl.ds(b1, 16), :], x_buf[pl.ds(b2, 16), :]], axis=0).astype(F32)
    g = _rb(jnp.dot(xs, wg_buf[...], preferred_element_type=F32))
    g = _rb(g * _rb(1.0 / (1.0 + jnp.exp(-g))))
    u = _rb(jnp.dot(xs, wu_buf[...], preferred_element_type=F32))
    gu = (g * u).astype(BF16)
    FF = gu.shape[1]
    y = None
    for t in range(FF // 128):
        yt = jnp.dot(gu[:, t * 128:(t + 1) * 128], wd_buf[t * 128:(t + 1) * 128, :], preferred_element_type=F32)
        y = yt if y is None else y + yt
    gate = _rb(1.0 / (1.0 + jnp.exp(-rsel)))
    y = _rb(_rb(y) * gate)
    new = (hsel + _rb(xs.astype(F32) + y)).astype(BF16)

    first_copy.wait()
    for i in range(1, nb):
        out_copy(i).wait()
    last_copy.wait()

    rid = lax.broadcasted_iota(jnp.int32, (16, M), 0)
    out_buf[pl.ds(b1, 16), :] = jnp.where(rid == i1 - b1, new[0:16], out_buf[pl.ds(b1, 16), :])
    out_buf[pl.ds(b2, 16), :] = jnp.where(rid == i2 - b2, new[16:32], out_buf[pl.ds(b2, 16), :])
    f1 = pltpu.make_async_copy(out_buf.at[pl.ds(b1, 16), :], out_hbm.at[pl.ds(b1, 16), :], sem_out.at[0])
    f2 = pltpu.make_async_copy(out_buf.at[pl.ds(b2, 16), :], out_hbm.at[pl.ds(b2, 16), :], sem_out.at[1])
    f1.start()

    @pl.when(b1 != b2)
    def _():
        f2.start()
        f2.wait()

    f1.wait()


@jax.jit
def pallas_sequential_preLN__compressed_kv_cla__moe_arch_mod__prompt_kernel(
    A_x, A_c_kv, A_w_q, A_w_uk, A_w_uv, A_w_o, B_x, B_w_r, B_w_gate, B_w_up, B_w_down,
):
    B, S, M = A_x.shape
    assert B == 1 and A_c_kv.shape[1] == S
    C = A_c_kv.shape[2]
    H, D = A_w_q.shape[1], A_w_q.shape[2]
    F = B_w_gate.shape[1]
    TQ = 128
    TM = 256
    TP = 256
    SR = 64

    any_spec = pl.BlockSpec(memory_space=pl.ANY)
    out = pl.pallas_call(
        functools.partial(_kernel, S=S, M=M, H=H, D=D, TQ=TQ, TM=TM, TP=TP, SR=SR),
        out_shape=jax.ShapeDtypeStruct((S, M), BF16),
        in_specs=[any_spec] * 10,
        out_specs=any_spec,
        scratch_shapes=[
            pltpu.VMEM((S, M), BF16),
            pltpu.VMEM((S, M), BF16),
            pltpu.VMEM((S, C), BF16),
            pltpu.VMEM((2, M + 2 * C, D), jnp.uint32),
            pltpu.VMEM((M, 2 * D), BF16),
            pltpu.VMEM((C, 4 * D), BF16),
            pltpu.VMEM((M,), BF16),
            pltpu.VMEM((H * D, M), BF16),
            pltpu.VMEM((M, F), BF16),
            pltpu.VMEM((M, F), BF16),
            pltpu.VMEM((F, M), BF16),
            pltpu.VMEM((2, S, D), BF16),
            pltpu.VMEM((2, S, D), BF16),
            pltpu.VMEM((2, S, D), BF16),
            pltpu.VMEM((H, S // 2, D), jnp.uint32),
            pltpu.VMEM((SR, M), F32),
            pltpu.VMEM((S, M), BF16),
            pltpu.VMEM((1, M), F32),
            pltpu.VMEM((2, 16, D), F32),
            pltpu.SemaphoreType.DMA((S // TP,)),
            pltpu.SemaphoreType.DMA((S // TP + 3,)),
            pltpu.SemaphoreType.DMA((5,)),
            pltpu.SemaphoreType.DMA((5,)),
            pltpu.SemaphoreType.DMA((S // TM + 1,)),
            pltpu.SMEM((1,), jnp.int32),
        ],
        compiler_params=pltpu.CompilerParams(vmem_limit_bytes=120 * 1024 * 1024,
            disable_bounds_checks=True, disable_semaphore_checks=True,
            shape_invariant_numerics=True),
    )(
        A_x.reshape(S, M), A_c_kv.reshape(S, C), A_w_q, A_w_uk, A_w_uv,
        A_w_o.reshape(H * D, M), B_w_r, B_w_gate, B_w_up, B_w_down,
    )
    return out.reshape(B, S, M)
```

```python
import functools
import math

import jax
import jax.numpy as jnp
from jax import lax
import jax.experimental.pallas as pl
import jax.experimental.pallas.tpu as pltpu

F32 = jnp.float32
BF16 = jnp.bfloat16
NT = (((1,), (1,)), ((), ()))
NEG = -1e30
EPS = 1e-5


def _rb(x):
    return x.astype(BF16).astype(F32)


def _layernorm_fast(xf):
    n = xf.shape[-1]
    mu = jnp.sum(xf, axis=-1, keepdims=True) * (1.0 / n)
    c = xf - mu
    var = jnp.sum(c * c, axis=-1, keepdims=True) * (1.0 / n)
    return c * lax.rsqrt(var + EPS)


def _unpack(u, odd):
    w = (u & jnp.uint32(0xFFFF0000)) if odd else (u << 16)
    return pltpu.bitcast(w, F32).astype(BF16)


def _recip(l):
    r = pl.reciprocal(l, approx=True)
    return r * (2.0 - l * r)


def _kernel(*refs, **kw):
    one = refs[-1]
    one[0] = 1

    def body(_, c):
        _body(*refs[:-1], **kw)
        return c

    lax.fori_loop(0, one[0], body, 0)


def _body(x_hbm, c_hbm, wq_hbm, wk_hbm, wv_hbm, wo_hbm, wr_hbm, wg_hbm, wu_hbm, wd_hbm,
            out_hbm,
            x_buf, xn_buf, c_buf, w_buf, wp_q, wp_kv, wr_ref, wo_buf, wg_buf, wu_buf, wd_buf,
            q_all, k_all, v_all, ctx_buf, a_buf, out_buf, wr_buf, top_buf, sem_x, sem_c, sem_big, sem_w, sem_out,
            *, S, M, H, D, TQ, TM, TP, SR):
    NP = H // 2
    NB = S // TQ
    NCH = S // TP
    PB = (S - 1).bit_length()
    assert S == 1 << PB and PB <= 13
    scale = (D ** -0.5) * math.log2(math.e)
    sets = tuple((q_all.at[o], k_all.at[o], v_all.at[o]) for o in range(2))
    (q0, k0, v0), (q1, k1, v1) = sets

    wq32 = wq_hbm.bitcast(jnp.uint32)
    wk32 = wk_hbm.bitcast(jnp.uint32)
    wv32 = wv_hbm.bitcast(jnp.uint32)

    C = c_buf.shape[1]
    QR, KR, VR = pl.ds(0, M), pl.ds(M, C), pl.ds(M + C, C)

    def w_copies(p, slot, sems=None):
        sems = sems or [sem_w.at[slot]] * 3
        return (
            pltpu.make_async_copy(wk32.at[:, p, :], w_buf.at[slot, KR, :], sems[0]),
            pltpu.make_async_copy(wv32.at[:, p, :], w_buf.at[slot, VR, :], sems[1]),
            pltpu.make_async_copy(wq32.at[:, p, :], w_buf.at[slot, QR, :], sems[2]),
        )

    def w_wait(slot):
        pltpu.make_async_copy(w_buf.at[slot], w_buf.at[slot], sem_w.at[slot]).wait()

    def chunk_rows(j):
        return pl.ds(j * TP if isinstance(j, int) else pl.multiple_of(j * TP, TP), TP)

    def x_copy(j):
        return pltpu.make_async_copy(x_hbm.at[chunk_rows(j), :], x_buf.at[chunk_rows(j), :], sem_x.at[j])

    big = [
        pltpu.make_async_copy(wo_hbm, wo_buf, sem_big.at[0]),
        pltpu.make_async_copy(wg_hbm, wg_buf, sem_big.at[1]),
        pltpu.make_async_copy(wu_hbm, wu_buf, sem_big.at[2]),
        pltpu.make_async_copy(wd_hbm, wd_buf, sem_big.at[3]),
    ]

    cp_wr = pltpu.make_async_copy(wr_hbm, wr_ref, sem_big.at[4])

    def zero_of(x):
        z = pltpu.bitcast(x, jnp.uint32)
        return lax.shift_right_logical(lax.shift_right_logical(z, jnp.uint32(16)), jnp.uint32(16))

    def qk(st, i):
        q_buf, k_buf, _ = st
        row = lax.broadcasted_iota(jnp.int32, (TQ, TQ), 0)
        col = lax.broadcasted_iota(jnp.int32, (TQ, TQ), 1)
        qi = q_buf[i * TQ:(i + 1) * TQ, :]
        sd = lax.dot_general(qi, k_buf[i * TQ:(i + 1) * TQ, :], NT, preferred_element_type=F32)
        sd = jnp.where(col <= row, sd, NEG)
        if i > 0:
            so = lax.dot_general(qi, k_buf[:i * TQ, :], NT, preferred_element_type=F32)
            return jnp.concatenate([so, sd], axis=1)
        return sd

    def softmax(s):
        m = jnp.max(s, axis=1, keepdims=True)
        p = jnp.exp2(s - m).astype(BF16)
        l = jnp.sum(p.astype(F32), axis=1, keepdims=True)
        return p, _recip(l)

    FIRST = 'k'

    def attention(h, st, w, first):
        q_buf, k_buf, v_buf = st

        def pq(rows):
            return (jnp.dot(xn_buf[rows, :], w[0], preferred_element_type=F32) * scale).astype(BF16)

        def pk(rows):
            return jnp.dot(c_buf[rows, :], w[1], preferred_element_type=F32).astype(BF16)

        def pv(rows):
            return jnp.dot(c_buf[rows, :], w[2], preferred_element_type=F32).astype(BF16)

        top = slice(S - TQ, S)
        early = {}
        if first and FIRST != 'none':
            early[FIRST] = {'q': pq, 'k': pk, 'v': pv}[FIRST](top)
        MK = 1
        pend = [qk(st, NB - 1 - n) for n in range(MK)]
        for i in range(NB - 1, -1, -1):
            rows = slice(i * TQ, (i + 1) * TQ)
            q_buf[rows, :] = early.pop('q') if 'q' in early else pq(rows)
            k_buf[rows, :] = early.pop('k') if 'k' in early else pk(rows)
            p, rl = softmax(pend.pop(0))
            if i - MK >= 0:
                pend.append(qk(st, i - MK))
            o = jnp.dot(p, v_buf[:(i + 1) * TQ, :], preferred_element_type=F32)
            ctx_buf[h, i * TQ // 2:(i + 1) * TQ // 2, :] = pltpu.bitcast((o * rl).astype(BF16), jnp.uint32)
            v_buf[rows, :] = early.pop('v') if 'v' in early else pv(rows)

    LC = 256
    NL = 3
    WQAT = 1
    L0 = LC * NL
    CR = (S - L0) // NCH
    assert CR * NCH == S - L0 and CR % 16 == 0

    def c_rows(j):
        base = L0 + j * CR
        return pl.ds(base if isinstance(base, int) else pl.multiple_of(base, 16), CR)

    def lead_rows(t):
        return pl.ds(t * LC if isinstance(t, int) else pl.multiple_of(t * LC, LC), LC)

    def c_lead_copy(t):
        return pltpu.make_async_copy(c_hbm.at[lead_rows(t), :], c_buf.at[lead_rows(t), :], sem_c.at[NCH + t])

    def c_tail_copy(j):
        return pltpu.make_async_copy(c_hbm.at[c_rows(j), :], c_buf.at[c_rows(j), :], sem_c.at[j])

    w0 = w_copies(0, 0, [sem_w.at[2], sem_w.at[3], sem_w.at[4]])
    cp_wr.start()
    w0[0].start()
    w0[1].start()
    for t in range(NL):
        c_lead_copy(t).start(priority=1)

    def issue(j, _):
        x_copy(j).start(priority=1)
        c_tail_copy(j).start(priority=1)
        return 0

    lax.fori_loop(0, NCH, issue, 0)
    a_buf[...] = jnp.zeros(a_buf.shape, F32)
    top_buf[...] = jnp.zeros(top_buf.shape, F32)
    cp_wr.wait()
    wr_buf[...] = wr_ref[...].reshape(1, M).astype(F32)

    def unpack_pair(dst, col, start, n):
        for r in range(0, n, 64):
            u = w_buf[0, start + r:start + r + 64, :]
            for odd in range(2):
                dst[r // 2:r // 2 + 32, col + odd * D:col + (odd + 1) * D] = pltpu.bitcast(_unpack(u, odd), jnp.uint32)

    def pro_kv(rows, wkv):
        kv = jnp.dot(c_buf[rows, :], wkv, preferred_element_type=F32).astype(BF16)
        k0[rows, :] = kv[:, 0:D]
        k1[rows, :] = kv[:, D:2 * D]
        v0[rows, :] = kv[:, 2 * D:3 * D]
        v1[rows, :] = kv[:, 3 * D:4 * D]

    w0[0].wait()
    w0[1].wait()
    unpack_pair(wp_kv, 0, M, C)
    unpack_pair(wp_kv, 2 * D, M + C, C)

    def lead(t, _):
        c_lead_copy(t).wait()

        @pl.when(t == WQAT)
        def _():
            w0[2].start()

        pro_kv(lead_rows(t), pltpu.bitcast(wp_kv[...], BF16))
        return 0

    lax.fori_loop(0, NL, lead, 0)
    w0[2].wait()
    unpack_pair(wp_q, 0, 0, M)

    def mid(j, _):
        x_copy(j).wait()
        c_tail_copy(j).wait()

        @pl.when(j == NCH - 2)
        def _():
            for cp in w_copies(1, 1):
                cp.start()

        NSUB = 1
        tp, cr = TP // NSUB, CR // NSUB
        assert cr % 16 == 0
        for u in range(NSUB):
            rows = pl.ds(pl.multiple_of(j * TP + u * tp, tp), tp)
            xn = _layernorm_fast(x_buf[rows, :].astype(F32)).astype(BF16)
            xn_buf[rows, :] = xn
            pro_kv(pl.ds(pl.multiple_of(L0 + j * CR + u * cr, 16), cr), pltpu.bitcast(wp_kv[...], BF16))
            q = (jnp.dot(xn, pltpu.bitcast(wp_q[...], BF16), preferred_element_type=F32) * scale).astype(BF16)
            q0[rows, :] = q[:, 0:D]
            q1[rows, :] = q[:, D:2 * D]
        return 0

    lax.fori_loop(0, NCH, mid, 0)

    def pair_body(j, _):
        slot = (j + 1) & 1
        w_wait(slot)

        def issue_next():
            @pl.when(j + 2 < NP)
            def _():
                for cp in w_copies(j + 2, 1 - slot):
                    cp.start()

            for t, cp in enumerate(big):
                @pl.when(j == t + 1)
                def _():
                    cp.start(priority=1)

        for odd in range(2):
            w = tuple(_unpack(w_buf[slot, r, :], odd) for r in (QR, KR, VR))
            if odd == 0:
                issue_next()
            attention(2 * j + odd, sets[odd], w, odd == 0)
        return 0

    lax.fori_loop(0, NP - 1, pair_body, 0)
    LA = 'seq'
    LK = 4

    def last_body(o, _):
        st = sets[0]
        if LA == 'mix2':
            order = [x for i in range(NB // 2) for x in (NB - 1 - i, NB // 2 - 1 - i)]
        elif LA == 'mix3':
            order = [15, 3, 14, 2, 13, 5, 12, 4, 11, 7, 10, 6, 9, 8, 1, 0]
        elif LA == 'mix4':
            order = [15, 7, 14, 6, 13, 5, 12, 4, 11, 10, 3, 9, 8, 2, 1, 0]
        elif LA == 'mix5':
            order = [7, 15, 6, 14, 5, 13, 4, 12, 3, 11, 10, 9, 8, 2, 1, 0]
        else:
            order = list(range(NB - 1, -1, -1))
        pend = [qk(st, i) for i in order[:LK]]
        moved = NB
        for n, i in enumerate(order):
            rows = slice(i * TQ, (i + 1) * TQ)
            p, rl = softmax(pend.pop(0))
            if n + LK < len(order):
                pend.append(qk(st, order[n + LK]))
            ov = jnp.dot(p, st[2][:(i + 1) * TQ, :], preferred_element_type=F32)
            ctx_buf[H - 2 + o, i * TQ // 2:(i + 1) * TQ // 2, :] = pltpu.bitcast((ov * rl).astype(BF16), jnp.uint32)
            q0[rows, :] = q1[rows, :]
            live = max(order[n + 1:], default=-1) + 1
            if live < moved:
                dead = slice(live * TQ, moved * TQ)
                k0[dead, :] = k1[dead, :]
                v0[dead, :] = v1[dead, :]
                moved = live
        return 0

    lax.fori_loop(0, 2, last_body, 0)

    big[0].wait()
    nb = S // TM
    NS = TM // SR

    def dyn(base, mult):
        return base if isinstance(base, int) else pl.multiple_of(base, mult)

    def out_copy(i):
        rows = pl.ds(dyn(i * TM - SR, SR), TM)
        return pltpu.make_async_copy(out_buf.at[rows, :], out_hbm.at[rows, :], sem_out.at[i])

    first_copy = pltpu.make_async_copy(out_buf.at[pl.ds(0, TM - SR), :], out_hbm.at[pl.ds(0, TM - SR), :], sem_out.at[0])
    last_copy = pltpu.make_async_copy(out_buf.at[pl.ds(S - SR, SR), :], out_hbm.at[pl.ds(S - SR, SR), :], sem_out.at[nb])

    P = 16
    NPC = SR // P

    def finish(base, a):
        rows = pl.ds(dyn(base, P), P)
        hb = (x_buf[rows, :].astype(F32) + a).astype(BF16)
        x_buf[rows, :] = hb
        h = hb.astype(F32)
        mu = jnp.sum(h, axis=-1, keepdims=True) * (1.0 / M)
        mub = _rb(mu)
        d = h - mub
        dm = mu - mub
        var = jnp.sum(d * d, axis=-1, keepdims=True) * (1.0 / M) - dm * dm
        dw = jnp.sum(d * wr_buf[...], axis=-1, keepdims=True)
        rs = _recip(_rb(jnp.sqrt(_rb(_rb(jnp.maximum(var, 0.0)) + EPS))))
        if 0:
            rs = pltpu.bitcast(pltpu.bitcast(rs, jnp.uint32) | zero_of(dw), F32)
        hnb = (d * rs).astype(BF16)
        xn_buf[rows, :] = hnb
        ob = (h + hnb.astype(F32)).astype(BF16)
        out_buf[rows, :] = ob
        return dw * rs, ob

    def make_key(r, pos):
        r = _rb(r) + 0.0
        bits = lax.shift_right_logical(pltpu.bitcast(r, jnp.int32), 16)
        o = jnp.where(bits >= 0x8000, bits ^ 0xFFFF, bits ^ 0x8000)
        o = jnp.where(r != r, 0, o)
        return pltpu.bitcast((o << PB) | (S - 1 - pos) | 0x20000000, F32)

    def merge(top, key):
        best, second = top
        return jnp.maximum(best, key), jnp.maximum(second, jnp.minimum(best, key))

    def tie(x, dep):
        z = pltpu.bitcast(dep, jnp.uint32)
        z = functools.reduce(jnp.bitwise_or, [z[:, t * D:(t + 1) * D] for t in range(M // D)])
        z = lax.shift_right_logical(lax.shift_right_logical(z, jnp.uint32(16)), jnp.uint32(16))
        xu = pltpu.bitcast(x, jnp.uint32)
        n = z.shape[0]
        return pltpu.bitcast(jnp.concatenate([xu[:n] | z, xu[n:]], axis=0), BF16)

    TOFF = 1

    def proj_body(i, _):
        lane = lax.broadcasted_iota(jnp.int32, (P, D), 1)
        rmat = jnp.zeros((P, D), F32)
        for t in range(NS):
            rows = pl.ds(dyn(i * (TM // 2) + t * (SR // 2), SR // 2), SR // 2)
            prev = jnp.maximum(i * TM - SR, 0) if t == 0 else i * TM + (t - 1) * SR
            a = None
            KS = 32
            GL = 6
            hs = H // KS
            hist = []
            for c in range(KS):
                ctx = [pltpu.bitcast(ctx_buf[hh, rows, :], BF16) for hh in range(c * hs, (c + 1) * hs)]
                if (c + TOFF) % (KS // NPC) == 0:
                    j = (c + TOFF) // (KS // NPC) - 1
                    ap = a_buf[j * P:(j + 1) * P, :]
                    if GL and c - GL >= 0:
                        z = pltpu.bitcast(hist[c - GL][0:P, 0:D], jnp.uint32)
                        z = lax.shift_right_logical(lax.shift_right_logical(z, jnp.uint32(16)), jnp.uint32(16))
                        ap = pltpu.bitcast(pltpu.bitcast(ap, jnp.uint32) | jnp.concatenate([z] * (M // D), axis=1), F32)
                    r, ob = finish(prev + j * P, ap)
                    rmat = jnp.where(lane == t * NPC + j, r, rmat)
                    ctx[0] = tie(ctx[0], ob)
                ctx = jnp.concatenate(ctx, axis=1) if hs > 1 else ctx[0]
                ac = jnp.dot(ctx, wo_buf[c * hs * D:(c + 1) * hs * D, :], preferred_element_type=F32)
                a = ac if a is None else a + ac
                hist.append(a)
            a_buf[...] = a
        pos = i * TM - SR + lane * P + lax.broadcasted_iota(jnp.int32, (P, D), 0)
        live = jnp.logical_and(pos >= 0, lane < TM // P)
        top = merge((top_buf[0], top_buf[1]), jnp.where(live, make_key(rmat, pos), 0.0))
        top_buf[0] = top[0]
        top_buf[1] = top[1]

        @pl.when(i == 0)
        def _():
            first_copy.start()

        @pl.when(i > 0)
        def _():
            out_copy(i).start()

        return 0

    lax.fori_loop(0, nb, proj_body, 0)
    for cp in big[1:]:
        cp.wait()
    best, second = top_buf[0], top_buf[1]
    b = jnp.max(best, axis=1, keepdims=True)
    top = (b, jnp.max(jnp.where(best == b, second, best), axis=1, keepdims=True))
    for j in range(NPC):
        base = S - SR + j * P
        r, _ = finish(base, a_buf[j * P:(j + 1) * P, :])
        top = merge(top, make_key(r, base + lax.broadcasted_iota(jnp.int32, (P, 1), 0)))
    last_copy.start()

    best, second = top
    k1 = jnp.max(best, axis=0, keepdims=True)
    k2 = jnp.max(jnp.where(best == k1, second, best), axis=0, keepdims=True)
    kk = jnp.concatenate([jnp.broadcast_to(k1, (16, 1)), jnp.broadcast_to(k2, (16, 1))], axis=0)
    kk = pltpu.bitcast(kk, jnp.int32)
    i1 = S - 1 - (kk[0, 0] & (S - 1))
    i2 = S - 1 - (kk[16, 0] & (S - 1))
    b1 = pl.multiple_of((i1 >> 4) << 4, 16)
    b2 = pl.multiple_of((i2 >> 4) << 4, 16)
    o = (kk >> PB) & 0xFFFF
    rsel = pltpu.bitcast(jnp.where(o >= 0x8000, o ^ 0x8000, o ^ 0xFFFF) << 16, F32)

    xs = jnp.concatenate([xn_buf[pl.ds(b1, 16), :], xn_buf[pl.ds(b2, 16), :]], axis=0)
    hsel = jnp.concatenate([x_buf[pl.ds(b1, 16), :], x_buf[pl.ds(b2, 16), :]], axis=0).astype(F32)
    g = _rb(jnp.dot(xs, wg_buf[...], preferred_element_type=F32))
    g = _rb(g * _rb(1.0 / (1.0 + jnp.exp(-g))))
    u = _rb(jnp.dot(xs, wu_buf[...], preferred_element_type=F32))
    gu = (g * u).astype(BF16)
    FF = gu.shape[1]
    y = None
    for t in range(FF // 128):
        yt = jnp.dot(gu[:, t * 128:(t + 1) * 128], wd_buf[t * 128:(t + 1) * 128, :], preferred_element_type=F32)
        y = yt if y is None else y + yt
    gate = _rb(1.0 / (1.0 + jnp.exp(-rsel)))
    y = _rb(_rb(y) * gate)
    new = (hsel + _rb(xs.astype(F32) + y)).astype(BF16)

    first_copy.wait()
    for i in range(1, nb):
        out_copy(i).wait()
    last_copy.wait()

    rid = lax.broadcasted_iota(jnp.int32, (16, M), 0)
    out_buf[pl.ds(b1, 16), :] = jnp.where(rid == i1 - b1, new[0:16], out_buf[pl.ds(b1, 16), :])
    out_buf[pl.ds(b2, 16), :] = jnp.where(rid == i2 - b2, new[16:32], out_buf[pl.ds(b2, 16), :])
    f1 = pltpu.make_async_copy(out_buf.at[pl.ds(b1, 16), :], out_hbm.at[pl.ds(b1, 16), :], sem_out.at[0])
    f2 = pltpu.make_async_copy(out_buf.at[pl.ds(b2, 16), :], out_hbm.at[pl.ds(b2, 16), :], sem_out.at[1])
    f1.start()

    @pl.when(b1 != b2)
    def _():
        f2.start()
        f2.wait()

    f1.wait()


@jax.jit
def pallas_sequential_preLN__compressed_kv_cla__moe_arch_mod__prompt_kernel(
    A_x, A_c_kv, A_w_q, A_w_uk, A_w_uv, A_w_o, B_x, B_w_r, B_w_gate, B_w_up, B_w_down,
):
    B, S, M = A_x.shape
    assert B == 1 and A_c_kv.shape[1] == S
    C = A_c_kv.shape[2]
    H, D = A_w_q.shape[1], A_w_q.shape[2]
    F = B_w_gate.shape[1]
    TQ = 128
    TM = 256
    TP = 256
    SR = 64

    any_spec = pl.BlockSpec(memory_space=pl.ANY)
    out = pl.pallas_call(
        functools.partial(_kernel, S=S, M=M, H=H, D=D, TQ=TQ, TM=TM, TP=TP, SR=SR),
        out_shape=jax.ShapeDtypeStruct((S, M), BF16),
        in_specs=[any_spec] * 10,
        out_specs=any_spec,
        scratch_shapes=[
            pltpu.VMEM((S, M), BF16),
            pltpu.VMEM((S, M), BF16),
            pltpu.VMEM((S, C), BF16),
            pltpu.VMEM((2, M + 2 * C, D), jnp.uint32),
            pltpu.VMEM((M // 2, 2 * D), jnp.uint32),
            pltpu.VMEM((C // 2, 4 * D), jnp.uint32),
            pltpu.VMEM((M,), BF16),
            pltpu.VMEM((H * D, M), BF16),
            pltpu.VMEM((M, F), BF16),
            pltpu.VMEM((M, F), BF16),
            pltpu.VMEM((F, M), BF16),
            pltpu.VMEM((2, S, D), BF16),
            pltpu.VMEM((2, S, D), BF16),
            pltpu.VMEM((2, S, D), BF16),
            pltpu.VMEM((H, S // 2, D), jnp.uint32),
            pltpu.VMEM((SR, M), F32),
            pltpu.VMEM((S, M), BF16),
            pltpu.VMEM((1, M), F32),
            pltpu.VMEM((2, 16, D), F32),
            pltpu.SemaphoreType.DMA((S // TP,)),
            pltpu.SemaphoreType.DMA((S // TP + 3,)),
            pltpu.SemaphoreType.DMA((5,)),
            pltpu.SemaphoreType.DMA((5,)),
            pltpu.SemaphoreType.DMA((S // TM + 1,)),
            pltpu.SMEM((1,), jnp.int32),
        ],
        compiler_params=pltpu.CompilerParams(vmem_limit_bytes=120 * 1024 * 1024,
            disable_bounds_checks=False, disable_semaphore_checks=True,
            shape_invariant_numerics=True),
    )(
        A_x.reshape(S, M), A_c_kv.reshape(S, C), A_w_q, A_w_uk, A_w_uv,
        A_w_o.reshape(H * D, M), B_w_r, B_w_gate, B_w_up, B_w_down,
    )
    return out.reshape(B, S, M)
```

```python
import functools
import math

import jax
import jax.numpy as jnp
from jax import lax
import jax.experimental.pallas as pl
import jax.experimental.pallas.tpu as pltpu

F32 = jnp.float32
BF16 = jnp.bfloat16
NT = (((1,), (1,)), ((), ()))
NEG = -1e30
EPS = 1e-5


def _rb(x):
    return x.astype(BF16).astype(F32)


def _layernorm_fast(xf):
    n = xf.shape[-1]
    mu = jnp.sum(xf, axis=-1, keepdims=True) * (1.0 / n)
    c = xf - mu
    var = jnp.sum(c * c, axis=-1, keepdims=True) * (1.0 / n)
    return c * lax.rsqrt(var + EPS)


def _unpack(u, odd):
    w = (u & jnp.uint32(0xFFFF0000)) if odd else (u << 16)
    return pltpu.bitcast(w, F32).astype(BF16)


def _recip(l):
    r = pl.reciprocal(l, approx=True)
    return r * (2.0 - l * r)


def _kernel(*refs, **kw):
    one = refs[-1]
    one[0] = 1

    def body(_, c):
        _body(*refs[:-1], **kw)
        return c

    lax.fori_loop(0, one[0], body, 0)


def _body(x_hbm, c_hbm, wq_hbm, wk_hbm, wv_hbm, wo_hbm, wr_hbm, wg_hbm, wu_hbm, wd_hbm,
            out_hbm,
            x_buf, xn_buf, c_buf, w_buf, wp_q, wp_kv, wr_ref, wo_buf, wg_buf, wu_buf, wd_buf,
            q_all, k_all, v_all, ctx_buf, a_buf, out_buf, wr_buf, top_buf, sem_x, sem_c, sem_big, sem_w, sem_out,
            *, S, M, H, D, TQ, TM, TP, SR):
    NP = H // 2
    NB = S // TQ
    NCH = S // TP
    PB = (S - 1).bit_length()
    assert S == 1 << PB and PB <= 13
    scale = (D ** -0.5) * math.log2(math.e)
    sets = tuple((q_all.at[o], k_all.at[o], v_all.at[o]) for o in range(2))
    (q0, k0, v0), (q1, k1, v1) = sets

    C = c_buf.shape[1]
    QR, KR, VR = (0, M), (M, C), (M + C, C)

    def w_copies(src, rng, p, slot, sem, parts=range(8)):
        return [
            pltpu.make_async_copy(src.at[:, s, pl.ds(2 * p, 2), :],
                                  w_buf.at[slot, pl.ds(rng[0] // 8, rng[1] // 8), pl.ds(2 * s, 2), :], sem)
            for s in parts
        ]

    def w_start(p, slot, parts=range(8)):
        for src, rng in ((wk_hbm, KR), (wv_hbm, VR), (wq_hbm, QR)):
            for cp in w_copies(src, rng, p, slot, sem_w.at[slot], parts):
                cp.start()

    def w_wait(slot, start, n, sem):
        part = w_buf.at[slot, pl.ds(start // 8, n // 8)]
        pltpu.make_async_copy(part, part, sem).wait()

    def w_load(slot, start, n):
        return pltpu.bitcast(w_buf[slot, start // 8:(start + n) // 8], jnp.uint32).reshape(n, D)

    def chunk_rows(j):
        return pl.ds(j * TP if isinstance(j, int) else pl.multiple_of(j * TP, TP), TP)

    def x_copy(j):
        return pltpu.make_async_copy(x_hbm.at[chunk_rows(j), :], x_buf.at[chunk_rows(j), :], sem_x.at[j])

    big = [
        pltpu.make_async_copy(wo_hbm, wo_buf, sem_big.at[0]),
        pltpu.make_async_copy(wg_hbm, wg_buf, sem_big.at[1]),
        pltpu.make_async_copy(wu_hbm, wu_buf, sem_big.at[2]),
        pltpu.make_async_copy(wd_hbm, wd_buf, sem_big.at[3]),
    ]

    cp_wr = pltpu.make_async_copy(wr_hbm, wr_ref, sem_big.at[4])

    def zero_of(x):
        z = pltpu.bitcast(x, jnp.uint32)
        return lax.shift_right_logical(lax.shift_right_logical(z, jnp.uint32(16)), jnp.uint32(16))

    def qk(st, i, mode='a'):
        q_buf, k_buf, _ = st
        row = lax.broadcasted_iota(jnp.int32, (TQ, TQ), 0)
        col = lax.broadcasted_iota(jnp.int32, (TQ, TQ), 1)
        qi = q_buf[i * TQ:(i + 1) * TQ, :]
        if mode == 'b':
            s = lax.dot_general(qi, k_buf[:(i + 1) * TQ, :], NT, preferred_element_type=F32)
            sd = jnp.where(col <= row, s[:, i * TQ:], NEG)
            return jnp.concatenate([s[:, :i * TQ], sd], axis=1) if i > 0 else sd
        sd = lax.dot_general(qi, k_buf[i * TQ:(i + 1) * TQ, :], NT, preferred_element_type=F32)
        sd = jnp.where(col <= row, sd, NEG)
        if i > 0:
            so = lax.dot_general(qi, k_buf[:i * TQ, :], NT, preferred_element_type=F32)
            return jnp.concatenate([so, sd], axis=1)
        return sd

    def softmax(s):
        m = jnp.max(s, axis=1, keepdims=True)
        p = jnp.exp2(s - m).astype(BF16)
        l = jnp.sum(p.astype(F32), axis=1, keepdims=True)
        return p, _recip(l)

    FIRST = 'k'

    def attention(h, st, w, first):
        q_buf, k_buf, v_buf = st

        def pq(rows):
            return (jnp.dot(xn_buf[rows, :], w[0], preferred_element_type=F32) * scale).astype(BF16)

        def pk(rows):
            return jnp.dot(c_buf[rows, :], w[1], preferred_element_type=F32).astype(BF16)

        def pv(rows):
            return jnp.dot(c_buf[rows, :], w[2], preferred_element_type=F32).astype(BF16)

        top = slice(S - TQ, S)
        early = {}
        if first and FIRST != 'none':
            early[FIRST] = {'q': pq, 'k': pk, 'v': pv}[FIRST](top)
        MK = 1
        pend = [qk(st, NB - 1 - n) for n in range(MK)]
        for i in range(NB - 1, -1, -1):
            rows = slice(i * TQ, (i + 1) * TQ)
            q_buf[rows, :] = early.pop('q') if 'q' in early else pq(rows)
            k_buf[rows, :] = early.pop('k') if 'k' in early else pk(rows)
            p, rl = softmax(pend.pop(0))
            if i - MK >= 0:
                pend.append(qk(st, i - MK))
            o = jnp.dot(p, v_buf[:(i + 1) * TQ, :], preferred_element_type=F32)
            ctx_buf[h, i * TQ // 2:(i + 1) * TQ // 2, :] = pltpu.bitcast((o * rl).astype(BF16), jnp.uint32)
            v_buf[rows, :] = early.pop('v') if 'v' in early else pv(rows)

    LC = 256
    NL = 3
    WQAT = 0
    L0 = LC * NL
    CR = (S - L0) // NCH
    assert CR * NCH == S - L0 and CR % 16 == 0

    def c_rows(j):
        base = L0 + j * CR
        return pl.ds(base if isinstance(base, int) else pl.multiple_of(base, 16), CR)

    def lead_rows(t):
        return pl.ds(t * LC if isinstance(t, int) else pl.multiple_of(t * LC, LC), LC)

    def c_lead_copy(t):
        return pltpu.make_async_copy(c_hbm.at[lead_rows(t), :], c_buf.at[lead_rows(t), :], sem_c.at[NCH + t])

    def c_tail_copy(j):
        return pltpu.make_async_copy(c_hbm.at[c_rows(j), :], c_buf.at[c_rows(j), :], sem_c.at[j])

    cp_wr.start()
    for cp in w_copies(wk_hbm, KR, 0, 0, sem_w.at[0]) + w_copies(wv_hbm, VR, 0, 0, sem_w.at[0]):
        cp.start()
    for t in range(NL):
        c_lead_copy(t).start(priority=1)

    def issue(j, _):
        x_copy(j).start(priority=1)
        c_tail_copy(j).start(priority=1)
        return 0

    lax.fori_loop(0, NCH, issue, 0)
    a_buf[...] = jnp.zeros(a_buf.shape, F32)
    top_buf[...] = jnp.zeros(top_buf.shape, F32)
    cp_wr.wait()
    wr_buf[...] = wr_ref[...].reshape(1, M).astype(F32)

    def unpack_pair(dst, col, start, n):
        for r in range(0, n, 64):
            u = w_load(0, start + r, 64)
            for odd in range(2):
                dst[r // 2:r // 2 + 32, col + odd * D:col + (odd + 1) * D] = pltpu.bitcast(_unpack(u, odd), jnp.uint32)

    def pro_kv(rows, wkv):
        kv = jnp.dot(c_buf[rows, :], wkv, preferred_element_type=F32).astype(BF16)
        k0[rows, :] = kv[:, 0:D]
        k1[rows, :] = kv[:, D:2 * D]
        v0[rows, :] = kv[:, 2 * D:3 * D]
        v1[rows, :] = kv[:, 3 * D:4 * D]

    w_wait(0, M, 2 * C, sem_w.at[0])
    unpack_pair(wp_kv, 0, M, C)
    unpack_pair(wp_kv, 2 * D, M + C, C)

    def lead(t, _):
        c_lead_copy(t).wait()

        @pl.when(t == WQAT)
        def _():
            for cp in w_copies(wq_hbm, QR, 0, 0, sem_w.at[0]):
                cp.start()

        pro_kv(lead_rows(t), pltpu.bitcast(wp_kv[...], BF16))
        return 0

    lax.fori_loop(0, NL, lead, 0)
    w_wait(0, 0, M, sem_w.at[0])
    unpack_pair(wp_q, 0, 0, M)

    def mid(j, _):
        x_copy(j).wait()
        c_tail_copy(j).wait()

        w_start(1, 1, [j * (8 // NCH) + t for t in range(8 // NCH)])
        NSUB = 1
        tp, cr = TP // NSUB, CR // NSUB
        assert cr % 16 == 0
        for u in range(NSUB):
            rows = pl.ds(pl.multiple_of(j * TP + u * tp, tp), tp)
            xn = _layernorm_fast(x_buf[rows, :].astype(F32)).astype(BF16)
            xn_buf[rows, :] = xn
            pro_kv(pl.ds(pl.multiple_of(L0 + j * CR + u * cr, 16), cr), pltpu.bitcast(wp_kv[...], BF16))
            q = (jnp.dot(xn, pltpu.bitcast(wp_q[...], BF16), preferred_element_type=F32) * scale).astype(BF16)
            q0[rows, :] = q[:, 0:D]
            q1[rows, :] = q[:, D:2 * D]
        return 0

    lax.fori_loop(0, NCH, mid, 0)

    def pair_body(j, _):
        slot = (j + 1) & 1
        w_wait(slot, 0, M + 2 * C, sem_w.at[slot])

        def issue_next():
            w_start(jnp.minimum(j + 2, NP - 1), 1 - slot)

            for t, cp in enumerate(big):
                @pl.when(j == t + 1)
                def _():
                    cp.start(priority=1)

        for odd in range(2):
            w = tuple(_unpack(w_load(slot, *r), odd) for r in (QR, KR, VR))
            if odd == 0:
                issue_next()
            attention(2 * j + odd, sets[odd], w, odd == 0)
        return 0

    lax.fori_loop(0, NP - 1, pair_body, 0)
    LA = 'seq'
    LK = 4

    def last_body(o, _):
        st = sets[0]
        if LA == 'mix2':
            order = [x for i in range(NB // 2) for x in (NB - 1 - i, NB // 2 - 1 - i)]
        elif LA == 'mix3':
            order = [15, 3, 14, 2, 13, 5, 12, 4, 11, 7, 10, 6, 9, 8, 1, 0]
        elif LA == 'mix4':
            order = [15, 7, 14, 6, 13, 5, 12, 4, 11, 10, 3, 9, 8, 2, 1, 0]
        elif LA == 'mix5':
            order = [7, 15, 6, 14, 5, 13, 4, 12, 3, 11, 10, 9, 8, 2, 1, 0]
        else:
            order = list(range(NB - 1, -1, -1))
        pend = [qk(st, i, 'b') for i in order[:LK]]
        moved = NB
        for n, i in enumerate(order):
            rows = slice(i * TQ, (i + 1) * TQ)
            p, rl = softmax(pend.pop(0))
            if n + LK < len(order):
                pend.append(qk(st, order[n + LK], 'b'))
            ov = jnp.dot(p, st[2][:(i + 1) * TQ, :], preferred_element_type=F32)
            ctx_buf[H - 2 + o, i * TQ // 2:(i + 1) * TQ // 2, :] = pltpu.bitcast((ov * rl).astype(BF16), jnp.uint32)
            q0[rows, :] = q1[rows, :]
            live = max(order[n + 1:], default=-1) + 1
            if live < moved:
                dead = slice(live * TQ, moved * TQ)
                k0[dead, :] = k1[dead, :]
                v0[dead, :] = v1[dead, :]
                moved = live
        return 0

    lax.fori_loop(0, 2, last_body, 0)

    big[0].wait()
    w_wait(NP & 1, 0, M + 2 * C, sem_w.at[NP & 1])
    nb = S // TM
    NS = TM // SR

    def dyn(base, mult):
        return base if isinstance(base, int) else pl.multiple_of(base, mult)

    def out_copy(i):
        rows = pl.ds(dyn(i * TM - SR, SR), TM)
        return pltpu.make_async_copy(out_buf.at[rows, :], out_hbm.at[rows, :], sem_out.at[i])

    first_copy = pltpu.make_async_copy(out_buf.at[pl.ds(0, TM - SR), :], out_hbm.at[pl.ds(0, TM - SR), :], sem_out.at[0])
    last_copy = pltpu.make_async_copy(out_buf.at[pl.ds(S - SR, SR), :], out_hbm.at[pl.ds(S - SR, SR), :], sem_out.at[nb])

    P = 16
    NPC = SR // P

    def finish(base, a):
        rows = pl.ds(dyn(base, P), P)
        hb = (x_buf[rows, :].astype(F32) + a).astype(BF16)
        x_buf[rows, :] = hb
        h = hb.astype(F32)
        mu = jnp.sum(h, axis=-1, keepdims=True) * (1.0 / M)
        mub = _rb(mu)
        d = h - mub
        dm = mu - mub
        var = jnp.sum(d * d, axis=-1, keepdims=True) * (1.0 / M) - dm * dm
        dw = jnp.sum(d * wr_buf[...], axis=-1, keepdims=True)
        rs = _recip(_rb(jnp.sqrt(_rb(_rb(jnp.maximum(var, 0.0)) + EPS))))
        if 0:
            rs = pltpu.bitcast(pltpu.bitcast(rs, jnp.uint32) | zero_of(dw), F32)
        hnb = (d * rs).astype(BF16)
        xn_buf[rows, :] = hnb
        ob = (h + hnb.astype(F32)).astype(BF16)
        out_buf[rows, :] = ob
        return dw * rs, ob

    def make_key(r, pos):
        r = _rb(r) + 0.0
        bits = lax.shift_right_logical(pltpu.bitcast(r, jnp.int32), 16)
        o = jnp.where(bits >= 0x8000, bits ^ 0xFFFF, bits ^ 0x8000)
        o = jnp.where(r != r, 0, o)
        return pltpu.bitcast((o << PB) | (S - 1 - pos) | 0x20000000, F32)

    def merge(top, key):
        best, second = top
        return jnp.maximum(best, key), jnp.maximum(second, jnp.minimum(best, key))

    def tie(x, dep):
        z = pltpu.bitcast(dep, jnp.uint32)
        z = functools.reduce(jnp.bitwise_or, [z[:, t * D:(t + 1) * D] for t in range(M // D)])
        z = lax.shift_right_logical(lax.shift_right_logical(z, jnp.uint32(16)), jnp.uint32(16))
        xu = pltpu.bitcast(x, jnp.uint32)
        n = z.shape[0]
        return pltpu.bitcast(jnp.concatenate([xu[:n] | z, xu[n:]], axis=0), BF16)

    TOFF = 1

    def proj_body(i, _):
        lane = lax.broadcasted_iota(jnp.int32, (P, D), 1)
        rmat = jnp.zeros((P, D), F32)
        for t in range(NS):
            rows = pl.ds(dyn(i * (TM // 2) + t * (SR // 2), SR // 2), SR // 2)
            prev = jnp.maximum(i * TM - SR, 0) if t == 0 else i * TM + (t - 1) * SR
            a = None
            KS = 32
            GL = 6
            hs = H // KS
            hist = []
            for c in range(KS):
                ctx = [pltpu.bitcast(ctx_buf[hh, rows, :], BF16) for hh in range(c * hs, (c + 1) * hs)]
                if (c + TOFF) % (KS // NPC) == 0:
                    j = (c + TOFF) // (KS // NPC) - 1
                    ap = a_buf[j * P:(j + 1) * P, :]
                    if GL and c - GL >= 0:
                        z = pltpu.bitcast(hist[c - GL][0:P, 0:D], jnp.uint32)
                        z = lax.shift_right_logical(lax.shift_right_logical(z, jnp.uint32(16)), jnp.uint32(16))
                        ap = pltpu.bitcast(pltpu.bitcast(ap, jnp.uint32) | jnp.concatenate([z] * (M // D), axis=1), F32)
                    r, ob = finish(prev + j * P, ap)
                    rmat = jnp.where(lane == t * NPC + j, r, rmat)
                    ctx[0] = tie(ctx[0], ob)
                ctx = jnp.concatenate(ctx, axis=1) if hs > 1 else ctx[0]
                ac = jnp.dot(ctx, wo_buf[c * hs * D:(c + 1) * hs * D, :], preferred_element_type=F32)
                a = ac if a is None else a + ac
                hist.append(a)
            a_buf[...] = a
        pos = i * TM - SR + lane * P + lax.broadcasted_iota(jnp.int32, (P, D), 0)
        live = jnp.logical_and(pos >= 0, lane < TM // P)
        top = merge((top_buf[0], top_buf[1]), jnp.where(live, make_key(rmat, pos), 0.0))
        top_buf[0] = top[0]
        top_buf[1] = top[1]

        @pl.when(i == 0)
        def _():
            first_copy.start()

        @pl.when(i > 0)
        def _():
            out_copy(i).start()

        return 0

    lax.fori_loop(0, nb, proj_body, 0)
    for cp in big[1:]:
        cp.wait()
    best, second = top_buf[0], top_buf[1]
    b = jnp.max(best, axis=1, keepdims=True)
    top = (b, jnp.max(jnp.where(best == b, second, best), axis=1, keepdims=True))
    for j in range(NPC):
        base = S - SR + j * P
        r, _ = finish(base, a_buf[j * P:(j + 1) * P, :])
        top = merge(top, make_key(r, base + lax.broadcasted_iota(jnp.int32, (P, 1), 0)))
    last_copy.start()

    best, second = top
    k1 = jnp.max(best, axis=0, keepdims=True)
    k2 = jnp.max(jnp.where(best == k1, second, best), axis=0, keepdims=True)
    kk = jnp.concatenate([jnp.broadcast_to(k1, (16, 1)), jnp.broadcast_to(k2, (16, 1))], axis=0)
    kk = pltpu.bitcast(kk, jnp.int32)
    i1 = S - 1 - (kk[0, 0] & (S - 1))
    i2 = S - 1 - (kk[16, 0] & (S - 1))
    b1 = pl.multiple_of((i1 >> 4) << 4, 16)
    b2 = pl.multiple_of((i2 >> 4) << 4, 16)
    o = (kk >> PB) & 0xFFFF
    rsel = pltpu.bitcast(jnp.where(o >= 0x8000, o ^ 0x8000, o ^ 0xFFFF) << 16, F32)

    xs = jnp.concatenate([xn_buf[pl.ds(b1, 16), :], xn_buf[pl.ds(b2, 16), :]], axis=0)
    hsel = jnp.concatenate([x_buf[pl.ds(b1, 16), :], x_buf[pl.ds(b2, 16), :]], axis=0).astype(F32)
    g = _rb(jnp.dot(xs, wg_buf[...], preferred_element_type=F32))
    g = _rb(g * _rb(1.0 / (1.0 + jnp.exp(-g))))
    u = _rb(jnp.dot(xs, wu_buf[...], preferred_element_type=F32))
    gu = (g * u).astype(BF16)
    FF = gu.shape[1]
    y = None
    for t in range(FF // 128):
        yt = jnp.dot(gu[:, t * 128:(t + 1) * 128], wd_buf[t * 128:(t + 1) * 128, :], preferred_element_type=F32)
        y = yt if y is None else y + yt
    gate = _rb(1.0 / (1.0 + jnp.exp(-rsel)))
    y = _rb(_rb(y) * gate)
    new = (hsel + _rb(xs.astype(F32) + y)).astype(BF16)

    first_copy.wait()
    for i in range(1, nb):
        out_copy(i).wait()
    last_copy.wait()

    rid = lax.broadcasted_iota(jnp.int32, (16, M), 0)
    out_buf[pl.ds(b1, 16), :] = jnp.where(rid == i1 - b1, new[0:16], out_buf[pl.ds(b1, 16), :])
    out_buf[pl.ds(b2, 16), :] = jnp.where(rid == i2 - b2, new[16:32], out_buf[pl.ds(b2, 16), :])
    f1 = pltpu.make_async_copy(out_buf.at[pl.ds(b1, 16), :], out_hbm.at[pl.ds(b1, 16), :], sem_out.at[0])
    f2 = pltpu.make_async_copy(out_buf.at[pl.ds(b2, 16), :], out_hbm.at[pl.ds(b2, 16), :], sem_out.at[1])
    f1.start()

    @pl.when(b1 != b2)
    def _():
        f2.start()
        f2.wait()

    f1.wait()


@jax.jit
def pallas_sequential_preLN__compressed_kv_cla__moe_arch_mod__prompt_kernel(
    A_x, A_c_kv, A_w_q, A_w_uk, A_w_uv, A_w_o, B_x, B_w_r, B_w_gate, B_w_up, B_w_down,
):
    B, S, M = A_x.shape
    assert B == 1 and A_c_kv.shape[1] == S
    C = A_c_kv.shape[2]
    H, D = A_w_q.shape[1], A_w_q.shape[2]
    F = B_w_gate.shape[1]
    TQ = 128
    TM = 256
    TP = 256
    SR = 64

    any_spec = pl.BlockSpec(memory_space=pl.ANY)
    out = pl.pallas_call(
        functools.partial(_kernel, S=S, M=M, H=H, D=D, TQ=TQ, TM=TM, TP=TP, SR=SR),
        out_shape=jax.ShapeDtypeStruct((S, M), BF16),
        in_specs=[any_spec] * 10,
        out_specs=any_spec,
        scratch_shapes=[
            pltpu.VMEM((S, M), BF16),
            pltpu.VMEM((S, M), BF16),
            pltpu.VMEM((S, C), BF16),
            pltpu.VMEM((2, (M + 2 * C) // 8, 16, D), BF16),
            pltpu.VMEM((M // 2, 2 * D), jnp.uint32),
            pltpu.VMEM((C // 2, 4 * D), jnp.uint32),
            pltpu.VMEM((M,), BF16),
            pltpu.VMEM((H * D, M), BF16),
            pltpu.VMEM((M, F), BF16),
            pltpu.VMEM((M, F), BF16),
            pltpu.VMEM((F, M), BF16),
            pltpu.VMEM((2, S, D), BF16),
            pltpu.VMEM((2, S, D), BF16),
            pltpu.VMEM((2, S, D), BF16),
            pltpu.VMEM((H, S // 2, D), jnp.uint32),
            pltpu.VMEM((SR, M), F32),
            pltpu.VMEM((S, M), BF16),
            pltpu.VMEM((1, M), F32),
            pltpu.VMEM((2, 16, D), F32),
            pltpu.SemaphoreType.DMA((S // TP,)),
            pltpu.SemaphoreType.DMA((S // TP + 3,)),
            pltpu.SemaphoreType.DMA((5,)),
            pltpu.SemaphoreType.DMA((2,)),
            pltpu.SemaphoreType.DMA((S // TM + 1,)),
            pltpu.SMEM((1,), jnp.int32),
        ],
        compiler_params=pltpu.CompilerParams(vmem_limit_bytes=120 * 1024 * 1024,
            disable_bounds_checks=True, disable_semaphore_checks=True,
            shape_invariant_numerics=True),
    )(
        A_x.reshape(S, M), A_c_kv.reshape(S, C),
        A_w_q.reshape(M // 8, 8, H, D), A_w_uk.reshape(C // 8, 8, H, D), A_w_uv.reshape(C // 8, 8, H, D),
        A_w_o.reshape(H * D, M), B_w_r, B_w_gate, B_w_up, B_w_down,
    )
    return out.reshape(B, S, M)
```

```python
import functools
import math

import jax
import jax.numpy as jnp
from jax import lax
import jax.experimental.pallas as pl
import jax.experimental.pallas.tpu as pltpu

F32 = jnp.float32
BF16 = jnp.bfloat16
U32 = jnp.uint32
NT = (((1,), (1,)), ((), ()))
NEG = -1e30
EPS = 1e-5

TQ = 128
TP = 256
LC = 256
NL = 3
TM = 256
SR = 64
P = 16
LK = 4
GL = 6


def _dot(a, b):
    return jnp.dot(a, b, preferred_element_type=F32)


def _rb(x):
    return x.astype(BF16).astype(F32)


def _unpack(u, odd):
    w = (u & U32(0xFFFF0000)) if odd else (u << 16)
    return pltpu.bitcast(w, F32).astype(BF16)


def _recip(x):
    r = pl.reciprocal(x, approx=True)
    return r * (2.0 - x * r)


def _zero_of(x):
    z = pltpu.bitcast(x, U32)
    return lax.shift_right_logical(lax.shift_right_logical(z, U32(16)), U32(16))


def _rows(start, size, mult):
    return pl.ds(start if isinstance(start, int) else pl.multiple_of(start, mult), size)


def _kernel(*refs):
    one = refs[-1]
    one[0] = 1

    def body(_, c):
        _body(*refs[:-1])
        return c

    lax.fori_loop(0, one[0], body, 0)


def _body(x_hbm, c_hbm, wq_hbm, wk_hbm, wv_hbm, wo_hbm, wr_hbm, wg_hbm, wu_hbm, wd_hbm,
          out_hbm,
          x_buf, xn_buf, c_buf, w_buf, wp_q, wp_kv, wr_ref, wo_buf, wg_buf, wu_buf, wd_buf,
          q_all, k_all, v_all, ctx_buf, a_buf, out_buf, wr_buf, top_buf,
          sem_x, sem_c, sem_big, sem_w, sem_out):
    S, M = x_buf.shape
    C = c_buf.shape[1]
    H, _, D = ctx_buf.shape
    NP = H // 2
    NB = S // TQ
    NCH = S // TP
    PB = (S - 1).bit_length()
    assert S == 1 << PB and PB <= 13 and 8 % NCH == 0
    scale = (D ** -0.5) * math.log2(math.e)
    sets = tuple((q_all.at[o], k_all.at[o], v_all.at[o]) for o in range(2))
    (q0, k0, v0), (q1, k1, v1) = sets

    QR, KR, VR = (0, M), (M, C), (M + C, C)

    def w_copies(src, rng, p, slot, parts=range(8)):
        return [
            pltpu.make_async_copy(src.at[:, s, pl.ds(2 * p, 2), :],
                                  w_buf.at[slot, pl.ds(rng[0] // 8, rng[1] // 8), pl.ds(2 * s, 2), :],
                                  sem_w.at[slot])
            for s in parts
        ]

    def w_start(p, slot, parts=range(8)):
        for src, rng in ((wk_hbm, KR), (wv_hbm, VR), (wq_hbm, QR)):
            for cp in w_copies(src, rng, p, slot, parts):
                cp.start()

    def w_wait(slot, start=0, n=M + 2 * C):
        part = w_buf.at[slot, pl.ds(start // 8, n // 8)]
        pltpu.make_async_copy(part, part, sem_w.at[slot]).wait()

    def w_load(slot, start, n):
        return pltpu.bitcast(w_buf[slot, start // 8:(start + n) // 8], U32).reshape(n, D)

    def x_copy(j):
        rows = _rows(j * TP, TP, TP)
        return pltpu.make_async_copy(x_hbm.at[rows, :], x_buf.at[rows, :], sem_x.at[j])

    big = [
        pltpu.make_async_copy(wo_hbm, wo_buf, sem_big.at[0]),
        pltpu.make_async_copy(wg_hbm, wg_buf, sem_big.at[1]),
        pltpu.make_async_copy(wu_hbm, wu_buf, sem_big.at[2]),
        pltpu.make_async_copy(wd_hbm, wd_buf, sem_big.at[3]),
    ]
    cp_wr = pltpu.make_async_copy(wr_hbm, wr_ref, sem_big.at[4])

    def scores(st, i, fused=False):
        q_buf, k_buf, _ = st
        row = lax.broadcasted_iota(jnp.int32, (TQ, TQ), 0)
        col = lax.broadcasted_iota(jnp.int32, (TQ, TQ), 1)
        qi = q_buf[i * TQ:(i + 1) * TQ, :]
        if fused:
            s = lax.dot_general(qi, k_buf[:(i + 1) * TQ, :], NT, preferred_element_type=F32)
            sd = jnp.where(col <= row, s[:, i * TQ:], NEG)
            return jnp.concatenate([s[:, :i * TQ], sd], axis=1) if i > 0 else sd
        sd = lax.dot_general(qi, k_buf[i * TQ:(i + 1) * TQ, :], NT, preferred_element_type=F32)
        sd = jnp.where(col <= row, sd, NEG)
        if i > 0:
            so = lax.dot_general(qi, k_buf[:i * TQ, :], NT, preferred_element_type=F32)
            return jnp.concatenate([so, sd], axis=1)
        return sd

    def softmax(s):
        m = jnp.max(s, axis=1, keepdims=True)
        p = jnp.exp2(s - m).astype(BF16)
        l = jnp.sum(p.astype(F32), axis=1, keepdims=True)
        return p, _recip(l)

    def context(h, v_buf, i, p, rl):
        o = _dot(p, v_buf[:(i + 1) * TQ, :])
        ctx_buf[h, i * TQ // 2:(i + 1) * TQ // 2, :] = pltpu.bitcast((o * rl).astype(BF16), U32)

    def attention(h, st, w, first):
        q_buf, k_buf, v_buf = st
        k_top = _dot(c_buf[S - TQ:S, :], w[1]).astype(BF16) if first else None
        s = scores(st, NB - 1)
        for i in range(NB - 1, -1, -1):
            rows = slice(i * TQ, (i + 1) * TQ)
            q_buf[rows, :] = (_dot(xn_buf[rows, :], w[0]) * scale).astype(BF16)
            if i == NB - 1 and first:
                k_buf[rows, :] = k_top
            else:
                k_buf[rows, :] = _dot(c_buf[rows, :], w[1]).astype(BF16)
            p, rl = softmax(s)
            if i > 0:
                s = scores(st, i - 1)
            context(h, v_buf, i, p, rl)
            v_buf[rows, :] = _dot(c_buf[rows, :], w[2]).astype(BF16)

    L0 = LC * NL
    CR = (S - L0) // NCH
    assert CR * NCH == S - L0 and CR % 16 == 0

    def c_lead_copy(t):
        rows = _rows(t * LC, LC, LC)
        return pltpu.make_async_copy(c_hbm.at[rows, :], c_buf.at[rows, :], sem_c.at[NCH + t])

    def c_tail_copy(j):
        rows = _rows(L0 + j * CR, CR, 16)
        return pltpu.make_async_copy(c_hbm.at[rows, :], c_buf.at[rows, :], sem_c.at[j])

    cp_wr.start()
    for cp in w_copies(wk_hbm, KR, 0, 0) + w_copies(wv_hbm, VR, 0, 0):
        cp.start()
    for t in range(NL):
        c_lead_copy(t).start(priority=1)

    def issue(j, _):
        x_copy(j).start(priority=1)
        c_tail_copy(j).start(priority=1)
        return 0

    lax.fori_loop(0, NCH, issue, 0)
    a_buf[...] = jnp.zeros(a_buf.shape, F32)
    top_buf[...] = jnp.zeros(top_buf.shape, F32)
    cp_wr.wait()
    wr_buf[...] = wr_ref[...].reshape(1, M).astype(F32)

    def unpack_pair(dst, col, start, n):
        for r in range(0, n, 64):
            u = w_load(0, start + r, 64)
            for odd in range(2):
                dst[r // 2:r // 2 + 32, col + odd * D:col + (odd + 1) * D] = pltpu.bitcast(_unpack(u, odd), U32)

    def project_kv(rows):
        kv = _dot(c_buf[rows, :], pltpu.bitcast(wp_kv[...], BF16)).astype(BF16)
        k0[rows, :] = kv[:, 0:D]
        k1[rows, :] = kv[:, D:2 * D]
        v0[rows, :] = kv[:, 2 * D:3 * D]
        v1[rows, :] = kv[:, 3 * D:4 * D]

    w_wait(0, M, 2 * C)
    unpack_pair(wp_kv, 0, *KR)
    unpack_pair(wp_kv, 2 * D, *VR)

    def lead(t, _):
        c_lead_copy(t).wait()

        @pl.when(t == 0)
        def _():
            for cp in w_copies(wq_hbm, QR, 0, 0):
                cp.start()

        project_kv(_rows(t * LC, LC, LC))
        return 0

    lax.fori_loop(0, NL, lead, 0)
    w_wait(0, *QR)
    unpack_pair(wp_q, 0, *QR)

    def mid(j, _):
        x_copy(j).wait()
        c_tail_copy(j).wait()
        w_start(1, 1, [j * (8 // NCH) + t for t in range(8 // NCH)])
        rows = _rows(j * TP, TP, TP)
        x = x_buf[rows, :].astype(F32)
        xc = x - jnp.sum(x, axis=-1, keepdims=True) * (1.0 / M)
        var = jnp.sum(xc * xc, axis=-1, keepdims=True) * (1.0 / M)
        xn = (xc * lax.rsqrt(var + EPS)).astype(BF16)
        xn_buf[rows, :] = xn
        project_kv(_rows(L0 + j * CR, CR, 16))
        q = (_dot(xn, pltpu.bitcast(wp_q[...], BF16)) * scale).astype(BF16)
        q0[rows, :] = q[:, 0:D]
        q1[rows, :] = q[:, D:2 * D]
        return 0

    lax.fori_loop(0, NCH, mid, 0)

    def pair_body(j, _):
        slot = (j + 1) & 1
        w_wait(slot)
        for odd in range(2):
            w = tuple(_unpack(w_load(slot, *r), odd) for r in (QR, KR, VR))
            if odd == 0:
                w_start(jnp.minimum(j + 2, NP - 1), 1 - slot)
                for t, cp in enumerate(big):
                    @pl.when(j == t + 1)
                    def _():
                        cp.start(priority=1)
            attention(2 * j + odd, sets[odd], w, odd == 0)
        return 0

    assert NP - 1 > len(big)
    lax.fori_loop(0, NP - 1, pair_body, 0)

    def last_body(o, _):
        pend = [scores(sets[0], NB - 1 - n, True) for n in range(LK)]
        for i in range(NB - 1, -1, -1):
            rows = slice(i * TQ, (i + 1) * TQ)
            p, rl = softmax(pend.pop(0))
            if i >= LK:
                pend.append(scores(sets[0], i - LK, True))
            context(H - 2 + o, v0, i, p, rl)
            q0[rows, :] = q1[rows, :]
            k0[rows, :] = k1[rows, :]
            v0[rows, :] = v1[rows, :]
        return 0

    lax.fori_loop(0, 2, last_body, 0)

    big[0].wait()
    w_wait(NP & 1)
    nb = S // TM
    NPC = SR // P

    def out_copy(start, size, n):
        rows = _rows(start, size, SR)
        return pltpu.make_async_copy(out_buf.at[rows, :], out_hbm.at[rows, :], sem_out.at[n])

    first_copy = out_copy(0, TM - SR, 0)
    last_copy = out_copy(S - SR, SR, nb)

    def finish(base, a):
        rows = _rows(base, P, P)
        hb = (x_buf[rows, :].astype(F32) + a).astype(BF16)
        x_buf[rows, :] = hb
        h = hb.astype(F32)
        mu = jnp.sum(h, axis=-1, keepdims=True) * (1.0 / M)
        mub = _rb(mu)
        d = h - mub
        dm = mu - mub
        var = jnp.sum(d * d, axis=-1, keepdims=True) * (1.0 / M) - dm * dm
        dw = jnp.sum(d * wr_buf[...], axis=-1, keepdims=True)
        rs = _recip(_rb(jnp.sqrt(_rb(_rb(jnp.maximum(var, 0.0)) + EPS))))
        hnb = (d * rs).astype(BF16)
        xn_buf[rows, :] = hnb
        ob = (h + hnb.astype(F32)).astype(BF16)
        out_buf[rows, :] = ob
        return dw * rs, ob

    def make_key(r, pos):
        r = _rb(r)
        bits = lax.shift_right_logical(pltpu.bitcast(r, jnp.int32), 16)
        o = jnp.where(bits > 0x8000, bits ^ 0xFFFF, bits | 0x8000)
        o = jnp.where(r != r, 0, o)
        return pltpu.bitcast((o << PB) | (S - 1 - pos) | 0x20000000, F32)

    def merge(top, key):
        best, second = top
        return jnp.maximum(best, key), jnp.maximum(second, jnp.minimum(best, key))

    def proj_body(i, _):
        lane = lax.broadcasted_iota(jnp.int32, (P, D), 1)
        rmat = jnp.zeros((P, D), F32)
        for t in range(TM // SR):
            rows = _rows(i * (TM // 2) + t * (SR // 2), SR // 2, SR // 2)
            prev = jnp.maximum(i * TM - SR, 0) if t == 0 else i * TM + (t - 1) * SR
            acc = []
            for hh in range(H):
                ctx = pltpu.bitcast(ctx_buf[hh, rows, :], BF16)
                if (hh + 1) % (H // NPC) == 0:
                    j = (hh + 1) // (H // NPC) - 1
                    ap = a_buf[j * P:(j + 1) * P, :]
                    if hh >= GL:
                        z = _zero_of(acc[hh - GL][0:P, 0:D])
                        ap = pltpu.bitcast(pltpu.bitcast(ap, U32) | jnp.concatenate([z] * (M // D), axis=1), F32)
                    r, ob = finish(prev + j * P, ap)
                    rmat = jnp.where(lane == t * NPC + j, r, rmat)
                    z = pltpu.bitcast(ob, U32)
                    z = _zero_of(functools.reduce(jnp.bitwise_or, [z[:, n * D:(n + 1) * D] for n in range(M // D)]))
                    cu = pltpu.bitcast(ctx, U32)
                    ctx = pltpu.bitcast(jnp.concatenate([cu[:P // 2] | z, cu[P // 2:]], axis=0), BF16)
                a = _dot(ctx, wo_buf[hh * D:(hh + 1) * D, :])
                acc.append(acc[-1] + a if acc else a)
            a_buf[...] = acc[-1]
        pos = i * TM - SR + lane * P + lax.broadcasted_iota(jnp.int32, (P, D), 0)
        live = jnp.logical_and(pos >= 0, lane < TM // P)
        top = merge((top_buf[0], top_buf[1]), jnp.where(live, make_key(rmat, pos), 0.0))
        top_buf[0] = top[0]
        top_buf[1] = top[1]

        @pl.when(i == 0)
        def _():
            first_copy.start()

        @pl.when(i > 0)
        def _():
            out_copy(i * TM - SR, TM, i).start()

        return 0

    lax.fori_loop(0, nb, proj_body, 0)
    for cp in big[1:]:
        cp.wait()
    best, second = top_buf[0], top_buf[1]
    b = jnp.max(best, axis=1, keepdims=True)
    top = (b, jnp.max(jnp.where(best == b, second, best), axis=1, keepdims=True))
    for j in range(NPC):
        base = S - SR + j * P
        r, _ = finish(base, a_buf[j * P:(j + 1) * P, :])
        top = merge(top, make_key(r, base + lax.broadcasted_iota(jnp.int32, (P, 1), 0)))
    last_copy.start()

    best, second = top
    key1 = jnp.max(best, axis=0, keepdims=True)
    key2 = jnp.max(jnp.where(best == key1, second, best), axis=0, keepdims=True)
    kk = jnp.concatenate([jnp.broadcast_to(key1, (16, 1)), jnp.broadcast_to(key2, (16, 1))], axis=0)
    kk = pltpu.bitcast(kk, jnp.int32)
    i1 = S - 1 - (kk[0, 0] & (S - 1))
    i2 = S - 1 - (kk[16, 0] & (S - 1))
    b1 = pl.multiple_of((i1 >> 4) << 4, 16)
    b2 = pl.multiple_of((i2 >> 4) << 4, 16)
    o = (kk >> PB) & 0xFFFF
    rsel = pltpu.bitcast(jnp.where(o >= 0x8000, o ^ 0x8000, o ^ 0xFFFF) << 16, F32)

    xs = jnp.concatenate([xn_buf[pl.ds(b1, 16), :], xn_buf[pl.ds(b2, 16), :]], axis=0)
    hsel = jnp.concatenate([x_buf[pl.ds(b1, 16), :], x_buf[pl.ds(b2, 16), :]], axis=0).astype(F32)
    g = _rb(_dot(xs, wg_buf[...]))
    g = _rb(g * _rb(1.0 / (1.0 + jnp.exp(-g))))
    u = _rb(_dot(xs, wu_buf[...]))
    gu = (g * u).astype(BF16)
    y = None
    for t in range(gu.shape[1] // 128):
        yt = _dot(gu[:, t * 128:(t + 1) * 128], wd_buf[t * 128:(t + 1) * 128, :])
        y = yt if y is None else y + yt
    gate = _rb(1.0 / (1.0 + jnp.exp(-rsel)))
    y = _rb(_rb(y) * gate)
    new = (hsel + _rb(xs.astype(F32) + y)).astype(BF16)

    first_copy.wait()
    for i in range(1, nb):
        out_copy(i * TM - SR, TM, i).wait()
    last_copy.wait()

    rid = lax.broadcasted_iota(jnp.int32, (16, M), 0)
    out_buf[pl.ds(b1, 16), :] = jnp.where(rid == i1 - b1, new[0:16], out_buf[pl.ds(b1, 16), :])
    out_buf[pl.ds(b2, 16), :] = jnp.where(rid == i2 - b2, new[16:32], out_buf[pl.ds(b2, 16), :])
    f1 = pltpu.make_async_copy(out_buf.at[pl.ds(b1, 16), :], out_hbm.at[pl.ds(b1, 16), :], sem_out.at[0])
    f2 = pltpu.make_async_copy(out_buf.at[pl.ds(b2, 16), :], out_hbm.at[pl.ds(b2, 16), :], sem_out.at[1])
    f1.start()

    @pl.when(b1 != b2)
    def _():
        f2.start()
        f2.wait()

    f1.wait()


@jax.jit
def pallas_sequential_preLN__compressed_kv_cla__moe_arch_mod__prompt_kernel(
    A_x: jax.Array,
    A_c_kv: jax.Array,
    A_w_q: jax.Array,
    A_w_uk: jax.Array,
    A_w_uv: jax.Array,
    A_w_o: jax.Array,
    B_x: jax.Array,
    B_w_r: jax.Array,
    B_w_gate: jax.Array,
    B_w_up: jax.Array,
    B_w_down: jax.Array,
):
    del B_x
    B, S, M = A_x.shape
    assert B == 1 and A_c_kv.shape[1] == S
    C = A_c_kv.shape[2]
    H, D = A_w_q.shape[1], A_w_q.shape[2]
    F = B_w_gate.shape[1]

    any_spec = pl.BlockSpec(memory_space=pl.ANY)
    out = pl.pallas_call(
        _kernel,
        out_shape=jax.ShapeDtypeStruct((S, M), BF16),
        in_specs=[any_spec] * 10,
        out_specs=any_spec,
        scratch_shapes=[
            pltpu.VMEM((S, M), BF16),
            pltpu.VMEM((S, M), BF16),
            pltpu.VMEM((S, C), BF16),
            pltpu.VMEM((2, (M + 2 * C) // 8, 16, D), BF16),
            pltpu.VMEM((M // 2, 2 * D), U32),
            pltpu.VMEM((C // 2, 4 * D), U32),
            pltpu.VMEM((M,), BF16),
            pltpu.VMEM((H * D, M), BF16),
            pltpu.VMEM((M, F), BF16),
            pltpu.VMEM((M, F), BF16),
            pltpu.VMEM((F, M), BF16),
            pltpu.VMEM((2, S, D), BF16),
            pltpu.VMEM((2, S, D), BF16),
            pltpu.VMEM((2, S, D), BF16),
            pltpu.VMEM((H, S // 2, D), U32),
            pltpu.VMEM((SR, M), F32),
            pltpu.VMEM((S, M), BF16),
            pltpu.VMEM((1, M), F32),
            pltpu.VMEM((2, P, D), F32),
            pltpu.SemaphoreType.DMA((S // TP,)),
            pltpu.SemaphoreType.DMA((S // TP + NL,)),
            pltpu.SemaphoreType.DMA((5,)),
            pltpu.SemaphoreType.DMA((2,)),
            pltpu.SemaphoreType.DMA((S // TM + 1,)),
            pltpu.SMEM((1,), jnp.int32),
        ],
        compiler_params=pltpu.CompilerParams(
            vmem_limit_bytes=120 * 1024 * 1024,
            disable_bounds_checks=True,
            disable_semaphore_checks=True,
        ),
    )(
        A_x.reshape(S, M), A_c_kv.reshape(S, C),
        A_w_q.reshape(M // 8, 8, H, D), A_w_uk.reshape(C // 8, 8, H, D), A_w_uv.reshape(C // 8, 8, H, D),
        A_w_o.reshape(H * D, M), B_w_r, B_w_gate, B_w_up, B_w_down,
    )
    return out.reshape(B, S, M)
```

```python
import functools
import math

import jax
import jax.numpy as jnp
from jax import lax
import jax.experimental.pallas as pl
import jax.experimental.pallas.tpu as pltpu

F32 = jnp.float32
BF16 = jnp.bfloat16
U32 = jnp.uint32
NT = (((1,), (1,)), ((), ()))
NEG = -1e30
EPS = 1e-5

TQ = 128
TP = 256
LC = 256
NL = 3
TM = 256
SR = 64
P = 16
LK = 4
GL = 6


def _dot(a, b):
    return jnp.dot(a, b, preferred_element_type=F32)


def _rb(x):
    return x.astype(BF16).astype(F32)


def _unpack(u, odd):
    w = (u & U32(0xFFFF0000)) if odd else (u << 16)
    return pltpu.bitcast(w, F32).astype(BF16)


def _recip(x):
    r = pl.reciprocal(x, approx=True)
    return r * (2.0 - x * r)


def _zero_of(x):
    z = pltpu.bitcast(x, U32)
    return lax.shift_right_logical(lax.shift_right_logical(z, U32(16)), U32(16))


def _rows(start, size, mult):
    return pl.ds(start if isinstance(start, int) else pl.multiple_of(start, mult), size)


def _kernel(*refs):
    one = refs[-1]
    one[0] = 1

    def body(_, c):
        _body(*refs[:-1])
        return c

    lax.fori_loop(0, one[0], body, 0)


def _body(x_hbm, c_hbm, wq_hbm, wk_hbm, wv_hbm, wo_hbm, wr_hbm, wg_hbm, wu_hbm, wd_hbm,
          out_hbm,
          x_buf, xn_buf, c_buf, w_buf, wp_q, wp_kv, wr_ref, wo_buf, wg_buf, wu_buf, wd_buf,
          q_all, k_all, v_all, ctx_buf, a_buf, out_buf, fix_buf, wr_buf, top_buf,
          sem_x, sem_c, sem_big, sem_w, sem_out):
    S, M = x_buf.shape
    C = c_buf.shape[1]
    H, _, D = ctx_buf.shape
    NP = H // 2
    NB = S // TQ
    NCH = S // TP
    PB = (S - 1).bit_length()
    assert S == 1 << PB and PB <= 13 and NCH >= 4
    scale = (D ** -0.5) * math.log2(math.e)
    sets = tuple((q_all.at[o], k_all.at[o], v_all.at[o]) for o in range(2))
    (q0, k0, v0), (q1, k1, v1) = sets

    QR, KR, VR = (0, M), (M, C), (M + C, C)

    def w_copies(src, rng, p, slot, parts=range(8)):
        return [
            pltpu.make_async_copy(src.at[:, s, pl.ds(2 * p, 2), :],
                                  w_buf.at[slot, pl.ds(rng[0] // 8, rng[1] // 8), pl.ds(2 * s, 2), :],
                                  sem_w.at[slot])
            for s in parts
        ]

    def w_start(p, slot, parts=range(8)):
        for src, rng in ((wk_hbm, KR), (wv_hbm, VR), (wq_hbm, QR)):
            for cp in w_copies(src, rng, p, slot, parts):
                cp.start()

    def w_wait(slot, start=0, n=M + 2 * C):
        part = w_buf.at[slot, pl.ds(start // 8, n // 8)]
        pltpu.make_async_copy(part, part, sem_w.at[slot]).wait()

    def w_load(slot, start, n):
        return pltpu.bitcast(w_buf[slot, start // 8:(start + n) // 8], U32).reshape(n, D)

    def x_copy(j):
        rows = _rows(j * TP, TP, TP)
        return pltpu.make_async_copy(x_hbm.at[rows, :], x_buf.at[rows, :], sem_x.at[j])

    big = [
        pltpu.make_async_copy(wo_hbm, wo_buf, sem_big.at[0]),
        pltpu.make_async_copy(wg_hbm, wg_buf, sem_big.at[1]),
        pltpu.make_async_copy(wu_hbm, wu_buf, sem_big.at[2]),
        pltpu.make_async_copy(wd_hbm, wd_buf, sem_big.at[3]),
    ]
    cp_wr = pltpu.make_async_copy(wr_hbm, wr_ref, sem_big.at[4])

    def scores(st, i, fused=False):
        q_buf, k_buf, _ = st
        row = lax.broadcasted_iota(jnp.int32, (TQ, TQ), 0)
        col = lax.broadcasted_iota(jnp.int32, (TQ, TQ), 1)
        qi = q_buf[i * TQ:(i + 1) * TQ, :]
        if fused:
            s = lax.dot_general(qi, k_buf[:(i + 1) * TQ, :], NT, preferred_element_type=F32)
            sd = jnp.where(col <= row, s[:, i * TQ:], NEG)
            return jnp.concatenate([s[:, :i * TQ], sd], axis=1) if i > 0 else sd
        sd = lax.dot_general(qi, k_buf[i * TQ:(i + 1) * TQ, :], NT, preferred_element_type=F32)
        sd = jnp.where(col <= row, sd, NEG)
        if i > 0:
            so = lax.dot_general(qi, k_buf[:i * TQ, :], NT, preferred_element_type=F32)
            return jnp.concatenate([so, sd], axis=1)
        return sd

    def softmax(s):
        m = jnp.max(s, axis=1, keepdims=True)
        p = jnp.exp2(s - m).astype(BF16)
        l = jnp.sum(p.astype(F32), axis=1, keepdims=True)
        return p, _recip(l)

    def context(h, v_buf, i, p, rl):
        o = _dot(p, v_buf[:(i + 1) * TQ, :])
        ctx_buf[h, i * TQ // 2:(i + 1) * TQ // 2, :] = pltpu.bitcast((o * rl).astype(BF16), U32)

    def attention(h, st, w, first):
        q_buf, k_buf, v_buf = st
        head = {}
        if first:
            head = {i: _dot(c_buf[i * TQ:(i + 1) * TQ, :D], w[1][:D]) for i in range(NB - 1, NB - 5, -1)}
        s = scores(st, NB - 1)
        for i in range(NB - 1, -1, -1):
            rows = slice(i * TQ, (i + 1) * TQ)
            q_buf[rows, :] = (_dot(xn_buf[rows, :], w[0]) * scale).astype(BF16)
            if i in head:
                k_buf[rows, :] = (_dot(c_buf[rows, D:], w[1][D:]) + head[i]).astype(BF16)
            else:
                k_buf[rows, :] = _dot(c_buf[rows, :], w[1]).astype(BF16)
            p, rl = softmax(s)
            if i > 0:
                s = scores(st, i - 1)
            context(h, v_buf, i, p, rl)
            v_buf[rows, :] = _dot(c_buf[rows, :], w[2]).astype(BF16)

    L0 = LC * NL
    CR = (S - L0) // NCH
    assert CR * NCH == S - L0 and CR % 16 == 0

    def c_lead_copy(t):
        rows = _rows(t * LC, LC, LC)
        return pltpu.make_async_copy(c_hbm.at[rows, :], c_buf.at[rows, :], sem_c.at[NCH + t])

    def c_tail_copy(j):
        rows = _rows(L0 + j * CR, CR, 16)
        return pltpu.make_async_copy(c_hbm.at[rows, :], c_buf.at[rows, :], sem_c.at[j])

    cp_wr.start()
    for cp in w_copies(wk_hbm, KR, 0, 0) + w_copies(wv_hbm, VR, 0, 0):
        cp.start()
    for t in range(NL):
        c_lead_copy(t).start(priority=1)

    def issue(j, _):
        x_copy(j).start(priority=1)
        c_tail_copy(j).start(priority=1)
        return 0

    lax.fori_loop(0, NCH, issue, 0)
    a_buf[...] = jnp.zeros(a_buf.shape, F32)
    top_buf[...] = jnp.zeros(top_buf.shape, F32)
    cp_wr.wait()
    wr_buf[...] = wr_ref[...].reshape(1, M).astype(F32)

    def unpack_pair(dst, col, start, n):
        for r in range(0, n, 64):
            u = w_load(0, start + r, 64)
            for odd in range(2):
                dst[r // 2:r // 2 + 32, col + odd * D:col + (odd + 1) * D] = pltpu.bitcast(_unpack(u, odd), U32)

    def project_kv(rows):
        kv = _dot(c_buf[rows, :], pltpu.bitcast(wp_kv[...], BF16)).astype(BF16)
        k0[rows, :] = kv[:, 0:D]
        k1[rows, :] = kv[:, D:2 * D]
        v0[rows, :] = kv[:, 2 * D:3 * D]
        v1[rows, :] = kv[:, 3 * D:4 * D]

    w_wait(0, M, 2 * C)
    unpack_pair(wp_kv, 0, *KR)
    unpack_pair(wp_kv, 2 * D, *VR)

    def lead(t, _):
        c_lead_copy(t).wait()

        @pl.when(t == 0)
        def _():
            for cp in w_copies(wq_hbm, QR, 0, 0):
                cp.start()

        project_kv(_rows(t * LC, LC, LC))
        return 0

    lax.fori_loop(0, NL, lead, 0)
    w_wait(0, *QR)
    unpack_pair(wp_q, 0, *QR)

    W0 = max(NCH - 5, 0)

    def mid(j, _):
        x_copy(j).wait()
        c_tail_copy(j).wait()

        @pl.when(jnp.logical_and(j >= W0, j < W0 + 4))
        def _():
            w_start(1, 1, [2 * (j - W0), 2 * (j - W0) + 1])

        rows = _rows(j * TP, TP, TP)
        x = x_buf[rows, :].astype(F32)
        xc = x - jnp.sum(x, axis=-1, keepdims=True) * (1.0 / M)
        var = jnp.sum(xc * xc, axis=-1, keepdims=True) * (1.0 / M)
        xn = (xc * lax.rsqrt(var + EPS)).astype(BF16)
        xn_buf[rows, :] = xn
        project_kv(_rows(L0 + j * CR, CR, 16))
        q = (_dot(xn, pltpu.bitcast(wp_q[...], BF16)) * scale).astype(BF16)
        q0[rows, :] = q[:, 0:D]
        q1[rows, :] = q[:, D:2 * D]
        return 0

    lax.fori_loop(0, NCH, mid, 0)

    def pair_body(j, _):
        slot = (j + 1) & 1
        w_wait(slot)
        for odd in range(2):
            w = tuple(_unpack(w_load(slot, *r), odd) for r in (QR, KR, VR))
            if odd == 0:
                w_start(jnp.minimum(j + 2, NP - 1), 1 - slot)
                for t, cp in enumerate(big):
                    @pl.when(j == t + 1)
                    def _():
                        cp.start(priority=1)
            attention(2 * j + odd, sets[odd], w, odd == 0)
        return 0

    assert NP - 1 > len(big)
    lax.fori_loop(0, NP - 1, pair_body, 0)

    def last_body(o, _):
        pend = [scores(sets[0], NB - 1 - n, True) for n in range(LK)]
        for i in range(NB - 1, -1, -1):
            rows = slice(i * TQ, (i + 1) * TQ)
            p, rl = softmax(pend.pop(0))
            if i >= LK:
                pend.append(scores(sets[0], i - LK, True))
            context(H - 2 + o, v0, i, p, rl)
            q0[rows, :] = q1[rows, :]
            k0[rows, :] = k1[rows, :]
            v0[rows, :] = v1[rows, :]
        return 0

    lax.fori_loop(0, 2, last_body, 0)

    for cp in big:
        cp.wait()
    w_wait(NP & 1)
    nb = S // TM
    NPC = SR // P

    def out_copy(start, size, n):
        rows = _rows(start, size, SR)
        return pltpu.make_async_copy(out_buf.at[rows, :], out_hbm.at[rows, :], sem_out.at[n])

    first_copy = out_copy(0, TM - SR, 0)
    last_copy = out_copy(S - SR, SR, nb)

    def finish(base, a):
        rows = _rows(base, P, P)
        hb = (x_buf[rows, :].astype(F32) + a).astype(BF16)
        x_buf[rows, :] = hb
        h = hb.astype(F32)
        mu = jnp.sum(h, axis=-1, keepdims=True) * (1.0 / M)
        mub = _rb(mu)
        d = h - mub
        dm = mu - mub
        var = jnp.sum(d * d, axis=-1, keepdims=True) * (1.0 / M) - dm * dm
        dw = jnp.sum(d * wr_buf[...], axis=-1, keepdims=True)
        rs = _recip(_rb(jnp.sqrt(_rb(_rb(jnp.maximum(var, 0.0)) + EPS))))
        hnb = (d * rs).astype(BF16)
        xn_buf[rows, :] = hnb
        ob = (h + hnb.astype(F32)).astype(BF16)
        out_buf[rows, :] = ob
        return dw * rs, ob

    def make_key(r, pos):
        r = _rb(r)
        bits = lax.shift_right_logical(pltpu.bitcast(r, jnp.int32), 16)
        o = jnp.where(bits > 0x8000, bits ^ 0xFFFF, bits | 0x8000)
        o = jnp.where(r != r, 0, o)
        return pltpu.bitcast((o << PB) | (S - 1 - pos) | 0x20000000, F32)

    def merge(top, key):
        best, second = top
        return jnp.maximum(best, key), jnp.maximum(second, jnp.minimum(best, key))

    def proj_body(i, _):
        lane = lax.broadcasted_iota(jnp.int32, (P, D), 1)
        rmat = jnp.zeros((P, D), F32)
        for t in range(TM // SR):
            rows = _rows(i * (TM // 2) + t * (SR // 2), SR // 2, SR // 2)
            prev = jnp.maximum(i * TM - SR, 0) if t == 0 else i * TM + (t - 1) * SR
            acc = []
            for hh in range(H):
                ctx = pltpu.bitcast(ctx_buf[hh, rows, :], BF16)
                if (hh + 1) % (H // NPC) == 0:
                    j = (hh + 1) // (H // NPC) - 1
                    ap = a_buf[j * P:(j + 1) * P, :]
                    if hh >= GL:
                        z = _zero_of(acc[hh - GL][0:P, 0:D])
                        ap = pltpu.bitcast(pltpu.bitcast(ap, U32) | jnp.concatenate([z] * (M // D), axis=1), F32)
                    r, ob = finish(prev + j * P, ap)
                    rmat = jnp.where(lane == t * NPC + j, r, rmat)
                    z = pltpu.bitcast(ob, U32)
                    z = _zero_of(functools.reduce(jnp.bitwise_or, [z[:, n * D:(n + 1) * D] for n in range(M // D)]))
                    cu = pltpu.bitcast(ctx, U32)
                    ctx = pltpu.bitcast(jnp.concatenate([cu[:P // 2] | z, cu[P // 2:]], axis=0), BF16)
                a = _dot(ctx, wo_buf[hh * D:(hh + 1) * D, :])
                acc.append(acc[-1] + a if acc else a)
            a_buf[...] = acc[-1]
        pos = i * TM - SR + lane * P + lax.broadcasted_iota(jnp.int32, (P, D), 0)
        live = jnp.logical_and(pos >= 0, lane < TM // P)
        top = merge((top_buf[0], top_buf[1]), jnp.where(live, make_key(rmat, pos), 0.0))
        top_buf[0] = top[0]
        top_buf[1] = top[1]

        @pl.when(i == 0)
        def _():
            first_copy.start()

        @pl.when(i > 0)
        def _():
            out_copy(i * TM - SR, TM, i).start()

        return 0

    lax.fori_loop(0, nb, proj_body, 0)
    best, second = top_buf[0], top_buf[1]
    b = jnp.max(best, axis=1, keepdims=True)
    top = (b, jnp.max(jnp.where(best == b, second, best), axis=1, keepdims=True))
    for j in range(NPC):
        base = S - SR + j * P
        r, _ = finish(base, a_buf[j * P:(j + 1) * P, :])
        top = merge(top, make_key(r, base + lax.broadcasted_iota(jnp.int32, (P, 1), 0)))
    last_copy.start()

    best, second = top
    key1 = jnp.max(best, axis=0, keepdims=True)
    key2 = jnp.max(jnp.where(best == key1, second, best), axis=0, keepdims=True)
    kk = jnp.concatenate([jnp.broadcast_to(key1, (16, 1)), jnp.broadcast_to(key2, (16, 1))], axis=0)
    kk = pltpu.bitcast(kk, jnp.int32)
    i1 = S - 1 - (kk[0, 0] & (S - 1))
    i2 = S - 1 - (kk[16, 0] & (S - 1))
    b1 = pl.multiple_of((i1 >> 4) << 4, 16)
    b2 = pl.multiple_of((i2 >> 4) << 4, 16)
    o = (kk >> PB) & 0xFFFF
    rsel = pltpu.bitcast(jnp.where(o >= 0x8000, o ^ 0x8000, o ^ 0xFFFF) << 16, F32)

    xs = jnp.concatenate([xn_buf[pl.ds(b1, 16), :], xn_buf[pl.ds(b2, 16), :]], axis=0)
    hsel = jnp.concatenate([x_buf[pl.ds(b1, 16), :], x_buf[pl.ds(b2, 16), :]], axis=0).astype(F32)
    g = _rb(_dot(xs, wg_buf[...]))
    g = _rb(g * _rb(1.0 / (1.0 + jnp.exp(-g))))
    u = _rb(_dot(xs, wu_buf[...]))
    gu = (g * u).astype(BF16)
    y = None
    for t in range(gu.shape[1] // 128):
        yt = _dot(gu[:, t * 128:(t + 1) * 128], wd_buf[t * 128:(t + 1) * 128, :])
        y = yt if y is None else y + yt
    gate = _rb(1.0 / (1.0 + jnp.exp(-rsel)))
    y = _rb(_rb(y) * gate)
    new = (hsel + _rb(xs.astype(F32) + y)).astype(BF16)

    rid = lax.broadcasted_iota(jnp.int32, (16, M), 0)
    fix_buf[0:16, :] = jnp.where(rid == i1 - b1, new[0:16],
                                 jnp.where(rid == i2 - b1, new[16:32], out_buf[pl.ds(b1, 16), :]))
    fix_buf[16:32, :] = jnp.where(rid == i2 - b2, new[16:32], out_buf[pl.ds(b2, 16), :])

    first_copy.wait()
    for i in range(1, nb):
        out_copy(i * TM - SR, TM, i).wait()
    last_copy.wait()
    f1 = pltpu.make_async_copy(fix_buf.at[pl.ds(0, 16), :], out_hbm.at[pl.ds(b1, 16), :], sem_out.at[0])
    f2 = pltpu.make_async_copy(fix_buf.at[pl.ds(16, 16), :], out_hbm.at[pl.ds(b2, 16), :], sem_out.at[1])
    f1.start()

    @pl.when(b1 != b2)
    def _():
        f2.start()
        f2.wait()

    f1.wait()


@jax.jit
def pallas_sequential_preLN__compressed_kv_cla__moe_arch_mod__prompt_kernel(
    A_x: jax.Array,
    A_c_kv: jax.Array,
    A_w_q: jax.Array,
    A_w_uk: jax.Array,
    A_w_uv: jax.Array,
    A_w_o: jax.Array,
    B_x: jax.Array,
    B_w_r: jax.Array,
    B_w_gate: jax.Array,
    B_w_up: jax.Array,
    B_w_down: jax.Array,
):
    del B_x
    B, S, M = A_x.shape
    assert B == 1 and A_c_kv.shape[1] == S
    C = A_c_kv.shape[2]
    H, D = A_w_q.shape[1], A_w_q.shape[2]
    F = B_w_gate.shape[1]

    any_spec = pl.BlockSpec(memory_space=pl.ANY)
    out = pl.pallas_call(
        _kernel,
        out_shape=jax.ShapeDtypeStruct((S, M), BF16),
        in_specs=[any_spec] * 10,
        out_specs=any_spec,
        scratch_shapes=[
            pltpu.VMEM((S, M), BF16),
            pltpu.VMEM((S, M), BF16),
            pltpu.VMEM((S, C), BF16),
            pltpu.VMEM((2, (M + 2 * C) // 8, 16, D), BF16),
            pltpu.VMEM((M // 2, 2 * D), U32),
            pltpu.VMEM((C // 2, 4 * D), U32),
            pltpu.VMEM((M,), BF16),
            pltpu.VMEM((H * D, M), BF16),
            pltpu.VMEM((M, F), BF16),
            pltpu.VMEM((M, F), BF16),
            pltpu.VMEM((F, M), BF16),
            pltpu.VMEM((2, S, D), BF16),
            pltpu.VMEM((2, S, D), BF16),
            pltpu.VMEM((2, S, D), BF16),
            pltpu.VMEM((H, S // 2, D), U32),
            pltpu.VMEM((SR, M), F32),
            pltpu.VMEM((S, M), BF16),
            pltpu.VMEM((32, M), BF16),
            pltpu.VMEM((1, M), F32),
            pltpu.VMEM((2, P, D), F32),
            pltpu.SemaphoreType.DMA((S // TP,)),
            pltpu.SemaphoreType.DMA((S // TP + NL,)),
            pltpu.SemaphoreType.DMA((5,)),
            pltpu.SemaphoreType.DMA((2,)),
            pltpu.SemaphoreType.DMA((S // TM + 1,)),
            pltpu.SMEM((1,), jnp.int32),
        ],
        compiler_params=pltpu.CompilerParams(
            vmem_limit_bytes=120 * 1024 * 1024,
            disable_bounds_checks=True,
            disable_semaphore_checks=True,
        ),
    )(
        A_x.reshape(S, M), A_c_kv.reshape(S, C),
        A_w_q.reshape(M // 8, 8, H, D), A_w_uk.reshape(C // 8, 8, H, D), A_w_uv.reshape(C // 8, 8, H, D),
        A_w_o.reshape(H * D, M), B_w_r, B_w_gate, B_w_up, B_w_down,
    )
    return out.reshape(B, S, M)
```

```python
import functools
import math

import jax
import jax.numpy as jnp
from jax import lax
import jax.experimental.pallas as pl
import jax.experimental.pallas.tpu as pltpu

F32 = jnp.float32
BF16 = jnp.bfloat16
U32 = jnp.uint32
NT = (((1,), (1,)), ((), ()))
NEG = -1e30
EPS = 1e-5

TQ = 128
TP = 256
LC = 256
NL = 3
TM = 256
SR = 64
P = 16
LK = 4
GL = 6


def _dot(a, b):
    return jnp.dot(a, b, preferred_element_type=F32)


def _rb(x):
    return x.astype(BF16).astype(F32)


def _unpack(u, odd):
    w = (u & U32(0xFFFF0000)) if odd else (u << 16)
    return pltpu.bitcast(w, F32).astype(BF16)


def _recip(x):
    r = pl.reciprocal(x, approx=True)
    return r * (2.0 - x * r)


def _zero_of(x):
    z = pltpu.bitcast(x, U32)
    return lax.shift_right_logical(lax.shift_right_logical(z, U32(16)), U32(16))


def _rows(start, size, mult):
    return pl.ds(start if isinstance(start, int) else pl.multiple_of(start, mult), size)


def _ld(ref, start, stop):
    return pltpu.bitcast(ref[start // 2:stop // 2, :], BF16)


def _kernel(*refs):
    one = refs[-1]
    one[0] = 1

    def body(_, c):
        _body(*refs[:-1])
        return c

    lax.fori_loop(0, one[0], body, 0)


def _body(x_hbm, c_hbm, wq_hbm, wk_hbm, wv_hbm, wo_hbm, wr_hbm, wg_hbm, wu_hbm, wd_hbm,
          out_hbm,
          x_buf, xn_buf, hn_buf, c_buf, cp_buf, w_buf, wp_q, wp_kv, wr_ref, wo_buf, wg_buf, wu_buf, wd_buf,
          q_all, k_all, v_all, ctx_buf, a_buf, out_buf, fix_buf, wr_buf, top_buf,
          sem_x, sem_c, sem_big, sem_w, sem_out):
    S, M = x_buf.shape
    C = c_buf.shape[1]
    H, _, D = ctx_buf.shape
    NP = H // 2
    NB = S // TQ
    NCH = S // TP
    PB = (S - 1).bit_length()
    assert S == 1 << PB and PB <= 13 and NCH >= 4
    scale = (D ** -0.5) * math.log2(math.e)
    sets = tuple((q_all.at[o], k_all.at[o], v_all.at[o]) for o in range(2))
    (q0, k0, v0), (q1, k1, v1) = sets

    QR, KR, VR = (0, M), (M, C), (M + C, C)

    def w_copies(src, rng, p, slot, parts=range(8)):
        return [
            pltpu.make_async_copy(src.at[:, s, pl.ds(2 * p, 2), :],
                                  w_buf.at[slot, pl.ds(rng[0] // 8, rng[1] // 8), pl.ds(2 * s, 2), :],
                                  sem_w.at[slot])
            for s in parts
        ]

    def w_start(p, slot, parts=range(8)):
        for src, rng in ((wk_hbm, KR), (wv_hbm, VR), (wq_hbm, QR)):
            for cp in w_copies(src, rng, p, slot, parts):
                cp.start()

    def w_wait(slot, start=0, n=M + 2 * C):
        part = w_buf.at[slot, pl.ds(start // 8, n // 8)]
        pltpu.make_async_copy(part, part, sem_w.at[slot]).wait()

    def w_load(slot, start, n):
        return pltpu.bitcast(w_buf[slot, start // 8:(start + n) // 8], U32).reshape(n, D)

    def x_copy(j):
        rows = _rows(j * TP, TP, TP)
        return pltpu.make_async_copy(x_hbm.at[rows, :], x_buf.at[rows, :], sem_x.at[j])

    big = [
        pltpu.make_async_copy(wo_hbm, wo_buf, sem_big.at[0]),
        pltpu.make_async_copy(wg_hbm, wg_buf, sem_big.at[1]),
        pltpu.make_async_copy(wu_hbm, wu_buf, sem_big.at[2]),
        pltpu.make_async_copy(wd_hbm, wd_buf, sem_big.at[3]),
    ]
    cp_wr = pltpu.make_async_copy(wr_hbm, wr_ref, sem_big.at[4])

    def scores(st, i, fused=False):
        q_buf, k_buf, _ = st
        row = lax.broadcasted_iota(jnp.int32, (TQ, TQ), 0)
        col = lax.broadcasted_iota(jnp.int32, (TQ, TQ), 1)
        qi = _ld(q_buf, i * TQ, (i + 1) * TQ)
        if fused:
            s = lax.dot_general(qi, _ld(k_buf, 0, (i + 1) * TQ), NT, preferred_element_type=F32)
            sd = jnp.where(col <= row, s[:, i * TQ:], NEG)
            return jnp.concatenate([s[:, :i * TQ], sd], axis=1) if i > 0 else sd
        sd = lax.dot_general(qi, _ld(k_buf, i * TQ, (i + 1) * TQ), NT, preferred_element_type=F32)
        sd = jnp.where(col <= row, sd, NEG)
        if i > 0:
            so = lax.dot_general(qi, _ld(k_buf, 0, i * TQ), NT, preferred_element_type=F32)
            return jnp.concatenate([so, sd], axis=1)
        return sd

    def softmax(s):
        m = jnp.max(s, axis=1, keepdims=True)
        p = jnp.exp2(s - m).astype(BF16)
        l = jnp.sum(p.astype(F32), axis=1, keepdims=True)
        return p, _recip(l)

    def context(h, v_buf, i, p, rl):
        o = _dot(p, _ld(v_buf, 0, (i + 1) * TQ))
        ctx_buf[h, i * TQ // 2:(i + 1) * TQ // 2, :] = pltpu.bitcast((o * rl).astype(BF16), U32)

    def attention(h, st, w, first):
        q_buf, k_buf, v_buf = st

        def c(i, cols=slice(None)):
            return pltpu.bitcast(cp_buf[i * TQ // 2:(i + 1) * TQ // 2, cols], BF16)

        head = {}
        if first:
            head = {i: _dot(c(i, slice(0, D)), w[1][:D]) for i in range(NB - 1, NB - 5, -1)}
        s = scores(st, NB - 1)
        for i in range(NB - 1, -1, -1):
            half = slice(i * TQ // 2, (i + 1) * TQ // 2)
            q_buf[half, :] = pltpu.bitcast((_dot(_ld(xn_buf, i * TQ, (i + 1) * TQ), w[0]) * scale).astype(BF16), U32)
            if i in head:
                k_buf[half, :] = pltpu.bitcast((_dot(c(i, slice(D, C)), w[1][D:]) + head[i]).astype(BF16), U32)
            else:
                k_buf[half, :] = pltpu.bitcast(_dot(c(i), w[1]).astype(BF16), U32)
            p, rl = softmax(s)
            if i > 0:
                s = scores(st, i - 1)
            context(h, v_buf, i, p, rl)
            v_buf[half, :] = pltpu.bitcast(_dot(c(i), w[2]).astype(BF16), U32)

    L0 = LC * NL
    CR = (S - L0) // NCH
    assert CR * NCH == S - L0 and CR % 16 == 0

    def c_lead_copy(t):
        rows = _rows(t * LC, LC, LC)
        return pltpu.make_async_copy(c_hbm.at[rows, :], c_buf.at[rows, :], sem_c.at[NCH + t])

    def c_tail_copy(j):
        rows = _rows(L0 + j * CR, CR, 16)
        return pltpu.make_async_copy(c_hbm.at[rows, :], c_buf.at[rows, :], sem_c.at[j])

    cp_wr.start()
    for cp in w_copies(wk_hbm, KR, 0, 0) + w_copies(wv_hbm, VR, 0, 0):
        cp.start()
    for t in range(NL):
        c_lead_copy(t).start(priority=1)

    def issue(j, _):
        x_copy(j).start(priority=1)
        c_tail_copy(j).start(priority=1)
        return 0

    lax.fori_loop(0, NCH, issue, 0)
    a_buf[...] = jnp.zeros(a_buf.shape, F32)
    top_buf[...] = jnp.zeros(top_buf.shape, F32)
    cp_wr.wait()
    wr_buf[...] = wr_ref[...].reshape(1, M).astype(F32)

    def unpack_pair(dst, col, start, n):
        for r in range(0, n, 64):
            u = w_load(0, start + r, 64)
            for odd in range(2):
                dst[r // 2:r // 2 + 32, col + odd * D:col + (odd + 1) * D] = pltpu.bitcast(_unpack(u, odd), U32)

    def project_kv(start, size):
        c = c_buf[_rows(start, size, 16), :]
        half = _rows(start >> 1, size // 2, 8)
        cp_buf[half, :] = pltpu.bitcast(c, U32)
        kv = _dot(c, pltpu.bitcast(wp_kv[...], BF16))
        k0[half, :] = pltpu.bitcast(kv[:, 0:D].astype(BF16), U32)
        k1[half, :] = pltpu.bitcast(kv[:, D:2 * D].astype(BF16), U32)
        v0[half, :] = pltpu.bitcast(kv[:, 2 * D:3 * D].astype(BF16), U32)
        v1[half, :] = pltpu.bitcast(kv[:, 3 * D:4 * D].astype(BF16), U32)

    w_wait(0, M, 2 * C)
    unpack_pair(wp_kv, 0, *KR)
    unpack_pair(wp_kv, 2 * D, *VR)

    def lead(t, _):
        c_lead_copy(t).wait()

        @pl.when(t == 0)
        def _():
            for cp in w_copies(wq_hbm, QR, 0, 0):
                cp.start()

        project_kv(t * LC, LC)
        return 0

    lax.fori_loop(0, NL, lead, 0)
    w_wait(0, *QR)
    unpack_pair(wp_q, 0, *QR)

    W0 = max(NCH - 5, 0)

    def mid(j, _):
        x_copy(j).wait()
        c_tail_copy(j).wait()

        @pl.when(jnp.logical_and(j >= W0, j < W0 + 4))
        def _():
            w_start(1, 1, [2 * (j - W0), 2 * (j - W0) + 1])

        x = x_buf[_rows(j * TP, TP, TP), :].astype(F32)
        xc = x - jnp.sum(x, axis=-1, keepdims=True) * (1.0 / M)
        var = jnp.sum(xc * xc, axis=-1, keepdims=True) * (1.0 / M)
        xn = (xc * lax.rsqrt(var + EPS)).astype(BF16)
        half = _rows(j * (TP // 2), TP // 2, TP // 2)
        xn_buf[half, :] = pltpu.bitcast(xn, U32)
        project_kv(L0 + j * CR, CR)
        q = _dot(xn, pltpu.bitcast(wp_q[...], BF16)) * scale
        q0[half, :] = pltpu.bitcast(q[:, 0:D].astype(BF16), U32)
        q1[half, :] = pltpu.bitcast(q[:, D:2 * D].astype(BF16), U32)
        return 0

    lax.fori_loop(0, NCH, mid, 0)

    def pair_body(j, _):
        slot = (j + 1) & 1
        w_wait(slot)
        for odd in range(2):
            w = tuple(_unpack(w_load(slot, *r), odd) for r in (QR, KR, VR))
            if odd == 0:
                w_start(jnp.minimum(j + 2, NP - 1), 1 - slot)
                for t, cp in enumerate(big):
                    @pl.when(j == t + 1)
                    def _():
                        cp.start(priority=1)
            attention(2 * j + odd, sets[odd], w, odd == 0)
        return 0

    assert NP - 1 > len(big)
    lax.fori_loop(0, NP - 1, pair_body, 0)

    def last_body(o, _):
        pend = [scores(sets[0], NB - 1 - n, True) for n in range(LK)]
        for i in range(NB - 1, -1, -1):
            half = slice(i * TQ // 2, (i + 1) * TQ // 2)
            p, rl = softmax(pend.pop(0))
            if i >= LK:
                pend.append(scores(sets[0], i - LK, True))
            context(H - 2 + o, v0, i, p, rl)
            q0[half, :] = q1[half, :]
            k0[half, :] = k1[half, :]
            v0[half, :] = v1[half, :]
        return 0

    lax.fori_loop(0, 2, last_body, 0)

    for cp in big:
        cp.wait()
    w_wait(NP & 1)
    nb = S // TM
    NPC = SR // P

    def out_copy(start, size, n):
        rows = _rows(start, size, SR)
        return pltpu.make_async_copy(out_buf.at[rows, :], out_hbm.at[rows, :], sem_out.at[n])

    first_copy = out_copy(0, TM - SR, 0)
    last_copy = out_copy(S - SR, SR, nb)

    def finish(base, a):
        rows = _rows(base, P, P)
        hb = (x_buf[rows, :].astype(F32) + a).astype(BF16)
        x_buf[rows, :] = hb
        h = hb.astype(F32)
        mu = jnp.sum(h, axis=-1, keepdims=True) * (1.0 / M)
        mub = _rb(mu)
        d = h - mub
        dm = mu - mub
        var = jnp.sum(d * d, axis=-1, keepdims=True) * (1.0 / M) - dm * dm
        dw = jnp.sum(d * wr_buf[...], axis=-1, keepdims=True)
        rs = _recip(_rb(jnp.sqrt(_rb(_rb(jnp.maximum(var, 0.0)) + EPS))))
        hnb = (d * rs).astype(BF16)
        hn_buf[rows, :] = hnb
        ob = (h + hnb.astype(F32)).astype(BF16)
        out_buf[rows, :] = ob
        return dw * rs, ob

    def make_key(r, pos):
        r = _rb(r)
        bits = lax.shift_right_logical(pltpu.bitcast(r, jnp.int32), 16)
        o = jnp.where(bits > 0x8000, bits ^ 0xFFFF, bits | 0x8000)
        o = jnp.where(r != r, 0, o)
        return pltpu.bitcast((o << PB) | (S - 1 - pos) | 0x20000000, F32)

    def merge(top, key):
        best, second = top
        return jnp.maximum(best, key), jnp.maximum(second, jnp.minimum(best, key))

    def proj_body(i, _):
        lane = lax.broadcasted_iota(jnp.int32, (P, D), 1)
        rmat = jnp.zeros((P, D), F32)
        for t in range(TM // SR):
            rows = _rows(i * (TM // 2) + t * (SR // 2), SR // 2, SR // 2)
            prev = jnp.maximum(i * TM - SR, 0) if t == 0 else i * TM + (t - 1) * SR
            acc = []
            for hh in range(H):
                ctx = pltpu.bitcast(ctx_buf[hh, rows, :], BF16)
                if (hh + 1) % (H // NPC) == 0:
                    j = (hh + 1) // (H // NPC) - 1
                    ap = a_buf[j * P:(j + 1) * P, :]
                    if hh >= GL:
                        z = _zero_of(acc[hh - GL][0:P, 0:D])
                        ap = pltpu.bitcast(pltpu.bitcast(ap, U32) | jnp.concatenate([z] * (M // D), axis=1), F32)
                    r, ob = finish(prev + j * P, ap)
                    rmat = jnp.where(lane == t * NPC + j, r, rmat)
                    z = pltpu.bitcast(ob, U32)
                    z = _zero_of(functools.reduce(jnp.bitwise_or, [z[:, n * D:(n + 1) * D] for n in range(M // D)]))
                    cu = pltpu.bitcast(ctx, U32)
                    ctx = pltpu.bitcast(jnp.concatenate([cu[:P // 2] | z, cu[P // 2:]], axis=0), BF16)
                a = _dot(ctx, wo_buf[hh * D:(hh + 1) * D, :])
                acc.append(acc[-1] + a if acc else a)
            a_buf[...] = acc[-1]
        pos = i * TM - SR + lane * P + lax.broadcasted_iota(jnp.int32, (P, D), 0)
        live = jnp.logical_and(pos >= 0, lane < TM // P)
        top = merge((top_buf[0], top_buf[1]), jnp.where(live, make_key(rmat, pos), 0.0))
        top_buf[0] = top[0]
        top_buf[1] = top[1]

        @pl.when(i == 0)
        def _():
            first_copy.start()

        @pl.when(i > 0)
        def _():
            out_copy(i * TM - SR, TM, i).start()

        return 0

    lax.fori_loop(0, nb, proj_body, 0)
    best, second = top_buf[0], top_buf[1]
    b = jnp.max(best, axis=1, keepdims=True)
    top = (b, jnp.max(jnp.where(best == b, second, best), axis=1, keepdims=True))
    for j in range(NPC):
        base = S - SR + j * P
        r, _ = finish(base, a_buf[j * P:(j + 1) * P, :])
        top = merge(top, make_key(r, base + lax.broadcasted_iota(jnp.int32, (P, 1), 0)))
    last_copy.start()

    best, second = top
    key1 = jnp.max(best, axis=0, keepdims=True)
    key2 = jnp.max(jnp.where(best == key1, second, best), axis=0, keepdims=True)
    kk = jnp.concatenate([jnp.broadcast_to(key1, (16, 1)), jnp.broadcast_to(key2, (16, 1))], axis=0)
    kk = pltpu.bitcast(kk, jnp.int32)
    i1 = S - 1 - (kk[0, 0] & (S - 1))
    i2 = S - 1 - (kk[16, 0] & (S - 1))
    b1 = pl.multiple_of((i1 >> 4) << 4, 16)
    b2 = pl.multiple_of((i2 >> 4) << 4, 16)
    o = (kk >> PB) & 0xFFFF
    rsel = pltpu.bitcast(jnp.where(o >= 0x8000, o ^ 0x8000, o ^ 0xFFFF) << 16, F32)

    xs = jnp.concatenate([hn_buf[pl.ds(b1, 16), :], hn_buf[pl.ds(b2, 16), :]], axis=0)
    hsel = jnp.concatenate([x_buf[pl.ds(b1, 16), :], x_buf[pl.ds(b2, 16), :]], axis=0).astype(F32)
    g = _rb(_dot(xs, wg_buf[...]))
    g = _rb(g * _rb(1.0 / (1.0 + jnp.exp(-g))))
    u = _rb(_dot(xs, wu_buf[...]))
    gu = (g * u).astype(BF16)
    y = None
    for t in range(gu.shape[1] // 128):
        yt = _dot(gu[:, t * 128:(t + 1) * 128], wd_buf[t * 128:(t + 1) * 128, :])
        y = yt if y is None else y + yt
    gate = _rb(1.0 / (1.0 + jnp.exp(-rsel)))
    y = _rb(_rb(y) * gate)
    new = (hsel + _rb(xs.astype(F32) + y)).astype(BF16)

    rid = lax.broadcasted_iota(jnp.int32, (16, M), 0)
    fix_buf[0:16, :] = jnp.where(rid == i1 - b1, new[0:16],
                                 jnp.where(rid == i2 - b1, new[16:32], out_buf[pl.ds(b1, 16), :]))
    fix_buf[16:32, :] = jnp.where(rid == i2 - b2, new[16:32], out_buf[pl.ds(b2, 16), :])

    first_copy.wait()
    for i in range(1, nb):
        out_copy(i * TM - SR, TM, i).wait()
    last_copy.wait()
    f1 = pltpu.make_async_copy(fix_buf.at[pl.ds(0, 16), :], out_hbm.at[pl.ds(b1, 16), :], sem_out.at[0])
    f2 = pltpu.make_async_copy(fix_buf.at[pl.ds(16, 16), :], out_hbm.at[pl.ds(b2, 16), :], sem_out.at[1])
    f1.start()

    @pl.when(b1 != b2)
    def _():
        f2.start()
        f2.wait()

    f1.wait()


@jax.jit
def pallas_sequential_preLN__compressed_kv_cla__moe_arch_mod__prompt_kernel(
    A_x: jax.Array,
    A_c_kv: jax.Array,
    A_w_q: jax.Array,
    A_w_uk: jax.Array,
    A_w_uv: jax.Array,
    A_w_o: jax.Array,
    B_x: jax.Array,
    B_w_r: jax.Array,
    B_w_gate: jax.Array,
    B_w_up: jax.Array,
    B_w_down: jax.Array,
):
    del B_x
    B, S, M = A_x.shape
    assert B == 1 and A_c_kv.shape[1] == S
    C = A_c_kv.shape[2]
    H, D = A_w_q.shape[1], A_w_q.shape[2]
    F = B_w_gate.shape[1]

    any_spec = pl.BlockSpec(memory_space=pl.ANY)
    out = pl.pallas_call(
        _kernel,
        out_shape=jax.ShapeDtypeStruct((S, M), BF16),
        in_specs=[any_spec] * 10,
        out_specs=any_spec,
        scratch_shapes=[
            pltpu.VMEM((S, M), BF16),
            pltpu.VMEM((S // 2, M), U32),
            pltpu.VMEM((S, M), BF16),
            pltpu.VMEM((S, C), BF16),
            pltpu.VMEM((S // 2, C), U32),
            pltpu.VMEM((2, (M + 2 * C) // 8, 16, D), BF16),
            pltpu.VMEM((M // 2, 2 * D), U32),
            pltpu.VMEM((C // 2, 4 * D), U32),
            pltpu.VMEM((M,), BF16),
            pltpu.VMEM((H * D, M), BF16),
            pltpu.VMEM((M, F), BF16),
            pltpu.VMEM((M, F), BF16),
            pltpu.VMEM((F, M), BF16),
            pltpu.VMEM((2, S // 2, D), U32),
            pltpu.VMEM((2, S // 2, D), U32),
            pltpu.VMEM((2, S // 2, D), U32),
            pltpu.VMEM((H, S // 2, D), U32),
            pltpu.VMEM((SR, M), F32),
            pltpu.VMEM((S, M), BF16),
            pltpu.VMEM((32, M), BF16),
            pltpu.VMEM((1, M), F32),
            pltpu.VMEM((2, P, D), F32),
            pltpu.SemaphoreType.DMA((S // TP,)),
            pltpu.SemaphoreType.DMA((S // TP + NL,)),
            pltpu.SemaphoreType.DMA((5,)),
            pltpu.SemaphoreType.DMA((2,)),
            pltpu.SemaphoreType.DMA((S // TM + 1,)),
            pltpu.SMEM((1,), jnp.int32),
        ],
        compiler_params=pltpu.CompilerParams(
            vmem_limit_bytes=120 * 1024 * 1024,
            disable_bounds_checks=True,
            disable_semaphore_checks=True,
        ),
    )(
        A_x.reshape(S, M), A_c_kv.reshape(S, C),
        A_w_q.reshape(M // 8, 8, H, D), A_w_uk.reshape(C // 8, 8, H, D), A_w_uv.reshape(C // 8, 8, H, D),
        A_w_o.reshape(H * D, M), B_w_r, B_w_gate, B_w_up, B_w_down,
    )
    return out.reshape(B, S, M)
```

```python
import functools
import math

import jax
import jax.numpy as jnp
from jax import lax
import jax.experimental.pallas as pl
import jax.experimental.pallas.tpu as pltpu

F32 = jnp.float32
BF16 = jnp.bfloat16
U32 = jnp.uint32
NT = (((1,), (1,)), ((), ()))
NEG = -1e30
EPS = 1e-5

TQ = 128
TP = 256
LC = 256
NL = 3
TM = 256
SR = 64
P = 16
LK = 4
GL = 6


def _dot(a, b):
    return jnp.dot(a, b, preferred_element_type=F32)


def _rb(x):
    return x.astype(BF16).astype(F32)


def _unpack(u, odd):
    w = (u & U32(0xFFFF0000)) if odd else (u << 16)
    return pltpu.bitcast(w, F32).astype(BF16)


def _recip(x):
    r = pl.reciprocal(x, approx=True)
    return r * (2.0 - x * r)


def _zero_of(x):
    z = pltpu.bitcast(x, U32)
    return lax.shift_right_logical(lax.shift_right_logical(z, U32(16)), U32(16))


def _rows(start, size, mult):
    return pl.ds(start if isinstance(start, int) else pl.multiple_of(start, mult), size)


def _ld(ref, start, stop):
    return pltpu.bitcast(ref[start // 2:stop // 2, :], BF16)


def _kernel(*refs):
    one = refs[-1]
    one[0] = 1

    def body(_, c):
        _body(*refs[:-1])
        return c

    lax.fori_loop(0, one[0], body, 0)


def _body(x_hbm, c_hbm, wq_hbm, wk_hbm, wv_hbm, wo_hbm, wr_hbm, wg_hbm, wu_hbm, wd_hbm,
          out_hbm,
          x_buf, xn_buf, hn_buf, c_buf, cp_buf, w_buf, wp_q, wp_kv, wr_ref, wo_buf, wg_buf, wu_buf, wd_buf,
          q_all, k_all, v_all, ctx_buf, a_buf, out_buf, fix_buf, wr_buf, top_buf,
          sem_x, sem_c, sem_big, sem_w, sem_out):
    S, M = x_buf.shape
    C = c_buf.shape[1]
    H, _, D = ctx_buf.shape
    NP = H // 2
    NB = S // TQ
    NCH = S // TP
    PB = (S - 1).bit_length()
    assert S == 1 << PB and PB <= 13 and NCH >= 4
    scale = (D ** -0.5) * math.log2(math.e)
    sets = tuple((q_all.at[o], k_all.at[o], v_all.at[o]) for o in range(2))
    (q0, k0, v0), (q1, k1, v1) = sets

    QR, KR, VR = (0, M), (M, C), (M + C, C)

    def w_copies(src, rng, p, slot, parts=range(8)):
        return [
            pltpu.make_async_copy(src.at[:, s, pl.ds(2 * p, 2), :],
                                  w_buf.at[slot, pl.ds(rng[0] // 8, rng[1] // 8), pl.ds(2 * s, 2), :],
                                  sem_w.at[slot])
            for s in parts
        ]

    def w_start(p, slot, parts=range(8)):
        for src, rng in ((wk_hbm, KR), (wv_hbm, VR), (wq_hbm, QR)):
            for cp in w_copies(src, rng, p, slot, parts):
                cp.start()

    def w_wait(slot, start=0, n=M + 2 * C):
        part = w_buf.at[slot, pl.ds(start // 8, n // 8)]
        pltpu.make_async_copy(part, part, sem_w.at[slot]).wait()

    def w_load(slot, start, n):
        return pltpu.bitcast(w_buf[slot, start // 8:(start + n) // 8], U32).reshape(n, D)

    def x_copy(j):
        rows = _rows(j * TP, TP, TP)
        return pltpu.make_async_copy(x_hbm.at[rows, :], x_buf.at[rows, :], sem_x.at[j])

    big = [
        pltpu.make_async_copy(wo_hbm, wo_buf, sem_big.at[0]),
        pltpu.make_async_copy(wg_hbm, wg_buf, sem_big.at[1]),
        pltpu.make_async_copy(wu_hbm, wu_buf, sem_big.at[2]),
        pltpu.make_async_copy(wd_hbm, wd_buf, sem_big.at[3]),
    ]
    cp_wr = pltpu.make_async_copy(wr_hbm, wr_ref, sem_big.at[4])

    def scores(st, i, fused=False):
        q_buf, k_buf, _ = st
        row = lax.broadcasted_iota(jnp.int32, (TQ, TQ), 0)
        col = lax.broadcasted_iota(jnp.int32, (TQ, TQ), 1)
        qi = _ld(q_buf, i * TQ, (i + 1) * TQ)
        if fused:
            s = lax.dot_general(qi, _ld(k_buf, 0, (i + 1) * TQ), NT, preferred_element_type=F32)
            sd = jnp.where(col <= row, s[:, i * TQ:], NEG)
            return jnp.concatenate([s[:, :i * TQ], sd], axis=1) if i > 0 else sd
        sd = lax.dot_general(qi, _ld(k_buf, i * TQ, (i + 1) * TQ), NT, preferred_element_type=F32)
        sd = jnp.where(col <= row, sd, NEG)
        if i > 0:
            so = lax.dot_general(qi, _ld(k_buf, 0, i * TQ), NT, preferred_element_type=F32)
            return jnp.concatenate([so, sd], axis=1)
        return sd

    def softmax(s):
        m = jnp.max(s, axis=1, keepdims=True)
        p = jnp.exp2(s - m).astype(BF16)
        l = jnp.sum(p.astype(F32), axis=1, keepdims=True)
        return p, _recip(l)

    def context(h, v_buf, i, p, rl):
        o = _dot(p, _ld(v_buf, 0, (i + 1) * TQ))
        ctx_buf[h, i * TQ // 2:(i + 1) * TQ // 2, :] = pltpu.bitcast((o * rl).astype(BF16), U32)

    def attention(h, st, w, first):
        q_buf, k_buf, v_buf = st

        def c(i, cols=slice(None)):
            return pltpu.bitcast(cp_buf[i * TQ // 2:(i + 1) * TQ // 2, cols], BF16)

        head = {}
        if first:
            head = {i: _dot(c(i, slice(0, D)), w[1][:D]) for i in range(NB - 1, NB - 5, -1)}
        s = scores(st, NB - 1)
        for i in range(NB - 1, -1, -1):
            half = slice(i * TQ // 2, (i + 1) * TQ // 2)
            q_buf[half, :] = pltpu.bitcast((_dot(_ld(xn_buf, i * TQ, (i + 1) * TQ), w[0]) * scale).astype(BF16), U32)
            if i in head:
                k_buf[half, :] = pltpu.bitcast((_dot(c(i, slice(D, C)), w[1][D:]) + head[i]).astype(BF16), U32)
            else:
                k_buf[half, :] = pltpu.bitcast(_dot(c(i), w[1]).astype(BF16), U32)
            p, rl = softmax(s)
            if i > 0:
                s = scores(st, i - 1)
            context(h, v_buf, i, p, rl)
            v_buf[half, :] = pltpu.bitcast(_dot(c(i), w[2]).astype(BF16), U32)

    L0 = LC * NL
    CR = (S - L0) // NCH
    assert CR * NCH == S - L0 and CR % 16 == 0

    def c_lead_copy(t):
        rows = _rows(t * LC, LC, LC)
        return pltpu.make_async_copy(c_hbm.at[rows, :], c_buf.at[rows, :], sem_c.at[NCH + t])

    def c_tail_copy(j):
        rows = _rows(L0 + j * CR, CR, 16)
        return pltpu.make_async_copy(c_hbm.at[rows, :], c_buf.at[rows, :], sem_c.at[j])

    cp_wr.start()
    for cp in w_copies(wk_hbm, KR, 0, 0) + w_copies(wv_hbm, VR, 0, 0):
        cp.start()
    for t in range(NL):
        c_lead_copy(t).start(priority=1)

    def issue(j, _):
        x_copy(j).start(priority=1)
        c_tail_copy(j).start(priority=1)
        return 0

    lax.fori_loop(0, NCH, issue, 0)
    a_buf[...] = jnp.zeros(a_buf.shape, F32)
    top_buf[...] = jnp.zeros(top_buf.shape, F32)
    cp_wr.wait()
    wr_buf[...] = wr_ref[...].reshape(1, M).astype(F32)

    def unpack_pair(dst, col, start, n):
        for r in range(0, n, 64):
            u = w_load(0, start + r, 64)
            for odd in range(2):
                dst[r // 2:r // 2 + 32, col + odd * D:col + (odd + 1) * D] = pltpu.bitcast(_unpack(u, odd), U32)

    def project_kv(start, size):
        c = c_buf[_rows(start, size, 16), :]
        half = _rows(start >> 1, size // 2, 8)
        cp_buf[half, :] = pltpu.bitcast(c, U32)
        kv = _dot(c, pltpu.bitcast(wp_kv[...], BF16))
        k0[half, :] = pltpu.bitcast(kv[:, 0:D].astype(BF16), U32)
        k1[half, :] = pltpu.bitcast(kv[:, D:2 * D].astype(BF16), U32)
        v0[half, :] = pltpu.bitcast(kv[:, 2 * D:3 * D].astype(BF16), U32)
        v1[half, :] = pltpu.bitcast(kv[:, 3 * D:4 * D].astype(BF16), U32)

    w_wait(0, M, 2 * C)
    unpack_pair(wp_kv, 0, *KR)
    unpack_pair(wp_kv, 2 * D, *VR)

    def lead(t, _):
        c_lead_copy(t).wait()

        @pl.when(t == 0)
        def _():
            for cp in w_copies(wq_hbm, QR, 0, 0):
                cp.start()

        project_kv(t * LC, LC)
        return 0

    lax.fori_loop(0, NL, lead, 0)
    w_wait(0, *QR)
    unpack_pair(wp_q, 0, *QR)

    W0 = max(NCH - 5, 0)

    def mid(j, _):
        x_copy(j).wait()
        c_tail_copy(j).wait()

        @pl.when(jnp.logical_and(j >= W0, j < W0 + 4))
        def _():
            w_start(1, 1, [2 * (j - W0), 2 * (j - W0) + 1])

        x = x_buf[_rows(j * TP, TP, TP), :].astype(F32)
        xc = x - jnp.sum(x, axis=-1, keepdims=True) * (1.0 / M)
        var = jnp.sum(xc * xc, axis=-1, keepdims=True) * (1.0 / M)
        xn = (xc * lax.rsqrt(var + EPS)).astype(BF16)
        half = _rows(j * (TP // 2), TP // 2, TP // 2)
        xn_buf[half, :] = pltpu.bitcast(xn, U32)
        project_kv(L0 + j * CR, CR)
        q = _dot(xn, pltpu.bitcast(wp_q[...], BF16)) * scale
        q0[half, :] = pltpu.bitcast(q[:, 0:D].astype(BF16), U32)
        q1[half, :] = pltpu.bitcast(q[:, D:2 * D].astype(BF16), U32)
        return 0

    lax.fori_loop(0, NCH, mid, 0)

    def pair_body(j, _):
        slot = (j + 1) & 1
        w_wait(slot)
        for odd in range(2):
            w = tuple(_unpack(w_load(slot, *r), odd) for r in (QR, KR, VR))
            if odd == 0:
                w_start(jnp.minimum(j + 2, NP - 1), 1 - slot)
                for t, cp in enumerate(big):
                    @pl.when(j == t + 1)
                    def _():
                        cp.start(priority=1)
            attention(2 * j + odd, sets[odd], w, odd == 0)
        return 0

    assert NP - 1 > len(big)
    lax.fori_loop(0, NP - 1, pair_body, 0)

    def last_body(o, _):
        pend = [scores(sets[0], NB - 1 - n, True) for n in range(LK)]
        for i in range(NB - 1, -1, -1):
            half = slice(i * TQ // 2, (i + 1) * TQ // 2)
            p, rl = softmax(pend.pop(0))
            if i >= LK:
                pend.append(scores(sets[0], i - LK, True))
            context(H - 2 + o, v0, i, p, rl)
            q0[half, :] = q1[half, :]
            k0[half, :] = k1[half, :]
            v0[half, :] = v1[half, :]
        return 0

    lax.fori_loop(0, 2, last_body, 0)

    for cp in big:
        cp.wait()
    w_wait(NP & 1)
    nb = S // TM
    NPC = SR // P

    def out_copy(start, size, n):
        rows = _rows(start, size, SR)
        return pltpu.make_async_copy(out_buf.at[rows, :], out_hbm.at[rows, :], sem_out.at[n])

    first_copy = out_copy(0, TM - SR, 0)
    last_copy = out_copy(S - SR, SR, nb)

    def finish(base, a):
        rows = _rows(base, P, P)
        hb = (x_buf[rows, :].astype(F32) + a).astype(BF16)
        x_buf[rows, :] = hb
        h = hb.astype(F32)
        mu = jnp.sum(h, axis=-1, keepdims=True) * (1.0 / M)
        mub = _rb(mu)
        d = h - mub
        dm = mu - mub
        var = jnp.sum(d * d, axis=-1, keepdims=True) * (1.0 / M) - dm * dm
        dw = jnp.sum(d * wr_buf[...], axis=-1, keepdims=True)
        rs = _recip(_rb(jnp.sqrt(_rb(_rb(jnp.maximum(var, 0.0)) + EPS))))
        hnb = (d * rs).astype(BF16)
        hn_buf[rows, :] = hnb
        ob = (h + hnb.astype(F32)).astype(BF16)
        out_buf[rows, :] = ob
        return dw * rs, ob

    def make_key(r, pos):
        r = _rb(r)
        bits = lax.shift_right_logical(pltpu.bitcast(r, jnp.int32), 16)
        o = jnp.where(bits > 0x8000, bits ^ 0xFFFF, bits | 0x8000)
        o = jnp.where(r != r, 0, o)
        return pltpu.bitcast((o << PB) | (S - 1 - pos) | 0x20000000, F32)

    def merge(top, key):
        best, second = top
        return jnp.maximum(best, key), jnp.maximum(second, jnp.minimum(best, key))

    def proj_body(i, _):
        lane = lax.broadcasted_iota(jnp.int32, (P, D), 1)
        rmat = jnp.zeros((P, D), F32)
        for t in range(TM // SR):
            rows = _rows(i * (TM // 2) + t * (SR // 2), SR // 2, SR // 2)
            prev = jnp.maximum(i * TM - SR, 0) if t == 0 else i * TM + (t - 1) * SR
            acc = []
            for hh in range(H):
                ctx = pltpu.bitcast(ctx_buf[hh, rows, :], BF16)
                if (hh + 1) % (H // NPC) == 0:
                    j = (hh + 1) // (H // NPC) - 1
                    ap = a_buf[j * P:(j + 1) * P, :]
                    if hh >= GL:
                        z = _zero_of(acc[hh - GL][0:P, 0:D])
                        ap = pltpu.bitcast(pltpu.bitcast(ap, U32) | jnp.concatenate([z] * (M // D), axis=1), F32)
                    r, ob = finish(prev + j * P, ap)
                    rmat = jnp.where(lane == t * NPC + j, r, rmat)
                    z = pltpu.bitcast(ob, U32)
                    z = _zero_of(functools.reduce(jnp.bitwise_or, [z[:, n * D:(n + 1) * D] for n in range(M // D)]))
                    cu = pltpu.bitcast(ctx, U32)
                    ctx = pltpu.bitcast(jnp.concatenate([cu[:P // 2] | z, cu[P // 2:]], axis=0), BF16)
                a = _dot(ctx, wo_buf[hh * D:(hh + 1) * D, :])
                acc.append(acc[-1] + a if acc else a)
            a_buf[...] = acc[-1]
        pos = i * TM - SR + lane * P + lax.broadcasted_iota(jnp.int32, (P, D), 0)
        live = jnp.logical_and(pos >= 0, lane < TM // P)
        top = merge((top_buf[0], top_buf[1]), jnp.where(live, make_key(rmat, pos), 0.0))
        top_buf[0] = top[0]
        top_buf[1] = top[1]

        @pl.when(i == 0)
        def _():
            first_copy.start()

        @pl.when(i > 0)
        def _():
            out_copy(i * TM - SR, TM, i).start()

        return 0

    lax.fori_loop(0, nb, proj_body, 0)
    best, second = top_buf[0], top_buf[1]
    b = jnp.max(best, axis=1, keepdims=True)
    top = (b, jnp.max(jnp.where(best == b, second, best), axis=1, keepdims=True))
    for j in range(NPC):
        base = S - SR + j * P
        r, _ = finish(base, a_buf[j * P:(j + 1) * P, :])
        top = merge(top, make_key(r, base + lax.broadcasted_iota(jnp.int32, (P, 1), 0)))
    last_copy.start()

    best, second = top
    key1 = jnp.max(best, axis=0, keepdims=True)
    key2 = jnp.max(jnp.where(best == key1, second, best), axis=0, keepdims=True)
    kk = jnp.concatenate([jnp.broadcast_to(key1, (8, 1)), jnp.broadcast_to(key2, (8, 1))], axis=0)
    kk = pltpu.bitcast(kk, jnp.int32)
    i1 = S - 1 - (kk[0, 0] & (S - 1))
    i2 = S - 1 - (kk[8, 0] & (S - 1))
    b1 = pl.multiple_of((i1 >> 4) << 4, 16)
    b2 = pl.multiple_of((i2 >> 4) << 4, 16)
    o = (kk >> PB) & 0xFFFF
    rsel = pltpu.bitcast(jnp.where(o >= 0x8000, o ^ 0x8000, o ^ 0xFFFF) << 16, F32)

    rid = lax.broadcasted_iota(jnp.int32, (16, M), 0)

    def pick(buf):
        rows = [jnp.sum(jnp.where(rid == i - b, buf[pl.ds(b, 16), :].astype(F32), 0.0), axis=0, keepdims=True)
                for i, b in ((i1, b1), (i2, b2))]
        return jnp.concatenate([jnp.broadcast_to(r, (8, M)) for r in rows], axis=0)

    xf = pick(hn_buf)
    xs = xf.astype(BF16)
    hsel = pick(x_buf)
    g = _dot(xs, wg_buf[...])
    u = _dot(xs, wu_buf[...])
    g = _rb(g)
    g = _rb(g * _rb(1.0 / (1.0 + jnp.exp(-g))))
    gu = (g * _rb(u)).astype(BF16)
    y = None
    for t in range(gu.shape[1] // 128):
        yt = _dot(gu[:, t * 128:(t + 1) * 128], wd_buf[t * 128:(t + 1) * 128, :])
        y = yt if y is None else y + yt
    gate = _rb(1.0 / (1.0 + jnp.exp(-rsel)))
    y = _rb(_rb(y) * gate)
    new = hsel + _rb(xf + y)
    n1 = jnp.concatenate([new[0:8], new[0:8]], axis=0).astype(BF16)
    n2 = jnp.concatenate([new[8:16], new[8:16]], axis=0).astype(BF16)

    fix_buf[0:16, :] = jnp.where(rid == i1 - b1, n1, jnp.where(rid == i2 - b1, n2, out_buf[pl.ds(b1, 16), :]))
    fix_buf[16:32, :] = jnp.where(rid == i2 - b2, n2, out_buf[pl.ds(b2, 16), :])

    first_copy.wait()
    for i in range(1, nb):
        out_copy(i * TM - SR, TM, i).wait()
    last_copy.wait()
    f1 = pltpu.make_async_copy(fix_buf.at[pl.ds(0, 16), :], out_hbm.at[pl.ds(b1, 16), :], sem_out.at[0])
    f2 = pltpu.make_async_copy(fix_buf.at[pl.ds(16, 16), :], out_hbm.at[pl.ds(b2, 16), :], sem_out.at[1])
    f1.start()

    @pl.when(b1 != b2)
    def _():
        f2.start()
        f2.wait()

    f1.wait()


@jax.jit
def pallas_sequential_preLN__compressed_kv_cla__moe_arch_mod__prompt_kernel(
    A_x: jax.Array,
    A_c_kv: jax.Array,
    A_w_q: jax.Array,
    A_w_uk: jax.Array,
    A_w_uv: jax.Array,
    A_w_o: jax.Array,
    B_x: jax.Array,
    B_w_r: jax.Array,
    B_w_gate: jax.Array,
    B_w_up: jax.Array,
    B_w_down: jax.Array,
):
    del B_x
    B, S, M = A_x.shape
    assert B == 1 and A_c_kv.shape[1] == S
    C = A_c_kv.shape[2]
    H, D = A_w_q.shape[1], A_w_q.shape[2]
    F = B_w_gate.shape[1]

    any_spec = pl.BlockSpec(memory_space=pl.ANY)
    out = pl.pallas_call(
        _kernel,
        out_shape=jax.ShapeDtypeStruct((S, M), BF16),
        in_specs=[any_spec] * 10,
        out_specs=any_spec,
        scratch_shapes=[
            pltpu.VMEM((S, M), BF16),
            pltpu.VMEM((S // 2, M), U32),
            pltpu.VMEM((S, M), BF16),
            pltpu.VMEM((S, C), BF16),
            pltpu.VMEM((S // 2, C), U32),
            pltpu.VMEM((2, (M + 2 * C) // 8, 16, D), BF16),
            pltpu.VMEM((M // 2, 2 * D), U32),
            pltpu.VMEM((C // 2, 4 * D), U32),
            pltpu.VMEM((M,), BF16),
            pltpu.VMEM((H * D, M), BF16),
            pltpu.VMEM((M, F), BF16),
            pltpu.VMEM((M, F), BF16),
            pltpu.VMEM((F, M), BF16),
            pltpu.VMEM((2, S // 2, D), U32),
            pltpu.VMEM((2, S // 2, D), U32),
            pltpu.VMEM((2, S // 2, D), U32),
            pltpu.VMEM((H, S // 2, D), U32),
            pltpu.VMEM((SR, M), F32),
            pltpu.VMEM((S, M), BF16),
            pltpu.VMEM((32, M), BF16),
            pltpu.VMEM((1, M), F32),
            pltpu.VMEM((2, P, D), F32),
            pltpu.SemaphoreType.DMA((S // TP,)),
            pltpu.SemaphoreType.DMA((S // TP + NL,)),
            pltpu.SemaphoreType.DMA((5,)),
            pltpu.SemaphoreType.DMA((2,)),
            pltpu.SemaphoreType.DMA((S // TM + 1,)),
            pltpu.SMEM((1,), jnp.int32),
        ],
        compiler_params=pltpu.CompilerParams(
            vmem_limit_bytes=120 * 1024 * 1024,
            disable_bounds_checks=True,
            disable_semaphore_checks=True,
        ),
    )(
        A_x.reshape(S, M), A_c_kv.reshape(S, C),
        A_w_q.reshape(M // 8, 8, H, D), A_w_uk.reshape(C // 8, 8, H, D), A_w_uv.reshape(C // 8, 8, H, D),
        A_w_o.reshape(H * D, M), B_w_r, B_w_gate, B_w_up, B_w_down,
    )
    return out.reshape(B, S, M)
```

```python
import functools
import math

import jax
import jax.numpy as jnp
from jax import lax
import jax.experimental.pallas as pl
import jax.experimental.pallas.tpu as pltpu

F32 = jnp.float32
BF16 = jnp.bfloat16
U32 = jnp.uint32
NT = (((1,), (1,)), ((), ()))
NEG = -1e30
EPS = 1e-5

TQ = 128
TP = 256
LC = 256
NL = 3
TM = 256
SR = 64
P = 16
LK = 4
GL = 6


def _dot(a, b):
    return jnp.dot(a, b, preferred_element_type=F32)


def _rb(x):
    return x.astype(BF16).astype(F32)


def _unpack(u, odd):
    w = (u & U32(0xFFFF0000)) if odd else (u << 16)
    return pltpu.bitcast(w, F32).astype(BF16)


def _recip(x):
    r = pl.reciprocal(x, approx=True)
    return r * (2.0 - x * r)


def _zero_of(x):
    z = pltpu.bitcast(x, U32)
    return lax.shift_right_logical(lax.shift_right_logical(z, U32(16)), U32(16))


def _rows(start, size, mult):
    return pl.ds(start if isinstance(start, int) else pl.multiple_of(start, mult), size)


def _ld(ref, start, stop):
    return pltpu.bitcast(ref[start // 2:stop // 2, :], BF16)


def _kernel(*refs):
    one = refs[-1]
    one[0] = 1

    def body(_, c):
        _body(*refs[:-1])
        return c

    lax.fori_loop(0, one[0], body, 0)


def _body(x_hbm, c_hbm, wq_hbm, wk_hbm, wv_hbm, wo_hbm, wr_hbm, wg_hbm, wu_hbm, wd_hbm,
          out_hbm,
          x_buf, xn_buf, hn_buf, c_buf, cp_buf, w_buf, wp_q, wp_kv, wr_ref, wo_buf, wg_buf, wu_buf, wd_buf,
          q_all, k_all, v_all, ctx_buf, a_buf, out_buf, fix_buf, wr_buf, top_buf,
          sem_x, sem_c, sem_big, sem_w, sem_out):
    S, M = x_buf.shape
    C = c_buf.shape[1]
    H, _, D = ctx_buf.shape
    NP = H // 2
    NB = S // TQ
    NCH = S // TP
    PB = (S - 1).bit_length()
    assert S == 1 << PB and PB <= 13 and NCH >= 4
    scale = (D ** -0.5) * math.log2(math.e)
    sets = tuple((q_all.at[o], k_all.at[o], v_all.at[o]) for o in range(2))
    (q0, k0, v0), (q1, k1, v1) = sets

    QR, KR, VR = (0, M), (M, C), (M + C, C)

    def w_copies(src, rng, p, slot, parts=range(8)):
        return [
            pltpu.make_async_copy(src.at[:, s, pl.ds(2 * p, 2), :],
                                  w_buf.at[slot, pl.ds(rng[0] // 8, rng[1] // 8), pl.ds(2 * s, 2), :],
                                  sem_w.at[slot])
            for s in parts
        ]

    def w_start(p, slot, parts=range(8)):
        for src, rng in ((wk_hbm, KR), (wv_hbm, VR), (wq_hbm, QR)):
            for cp in w_copies(src, rng, p, slot, parts):
                cp.start()

    def w_wait(slot, start=0, n=M + 2 * C):
        part = w_buf.at[slot, pl.ds(start // 8, n // 8)]
        pltpu.make_async_copy(part, part, sem_w.at[slot]).wait()

    def w_load(slot, start, n):
        return pltpu.bitcast(w_buf[slot, start // 8:(start + n) // 8], U32).reshape(n, D)

    def x_copy(j):
        rows = _rows(j * TP, TP, TP)
        return pltpu.make_async_copy(x_hbm.at[rows, :], x_buf.at[rows, :], sem_x.at[j])

    big = [
        pltpu.make_async_copy(wo_hbm, wo_buf, sem_big.at[0]),
        pltpu.make_async_copy(wg_hbm, wg_buf, sem_big.at[1]),
        pltpu.make_async_copy(wu_hbm, wu_buf, sem_big.at[2]),
        pltpu.make_async_copy(wd_hbm, wd_buf, sem_big.at[3]),
    ]
    cp_wr = pltpu.make_async_copy(wr_hbm, wr_ref, sem_big.at[4])

    def scores(st, i, fused=False):
        q_buf, k_buf, _ = st
        row = lax.broadcasted_iota(jnp.int32, (TQ, TQ), 0)
        col = lax.broadcasted_iota(jnp.int32, (TQ, TQ), 1)
        qi = _ld(q_buf, i * TQ, (i + 1) * TQ)
        if fused:
            s = lax.dot_general(qi, _ld(k_buf, 0, (i + 1) * TQ), NT, preferred_element_type=F32)
            sd = jnp.where(col <= row, s[:, i * TQ:], NEG)
            return jnp.concatenate([s[:, :i * TQ], sd], axis=1) if i > 0 else sd
        sd = lax.dot_general(qi, _ld(k_buf, i * TQ, (i + 1) * TQ), NT, preferred_element_type=F32)
        sd = jnp.where(col <= row, sd, NEG)
        if i > 0:
            so = lax.dot_general(qi, _ld(k_buf, 0, i * TQ), NT, preferred_element_type=F32)
            return jnp.concatenate([so, sd], axis=1)
        return sd

    def softmax(s):
        m = jnp.max(s, axis=1, keepdims=True)
        p = jnp.exp2(s - m).astype(BF16)
        l = jnp.sum(p.astype(F32), axis=1, keepdims=True)
        return p, _recip(l)

    def context(h, v_buf, i, p, rl):
        o = _dot(p, _ld(v_buf, 0, (i + 1) * TQ))
        ctx_buf[h, i * TQ // 2:(i + 1) * TQ // 2, :] = pltpu.bitcast((o * rl).astype(BF16), U32)

    def attention(h, st, w, first):
        q_buf, k_buf, v_buf = st

        def c(i, cols=slice(None)):
            return pltpu.bitcast(cp_buf[i * TQ // 2:(i + 1) * TQ // 2, cols], BF16)

        head = {}
        if first:
            head = {i: _dot(c(i, slice(0, D)), w[1][:D]) for i in range(NB - 1, NB - 5, -1)}
        s = scores(st, NB - 1)
        for i in range(NB - 1, -1, -1):
            half = slice(i * TQ // 2, (i + 1) * TQ // 2)
            q_buf[half, :] = pltpu.bitcast((_dot(_ld(xn_buf, i * TQ, (i + 1) * TQ), w[0]) * scale).astype(BF16), U32)
            if i in head:
                k_buf[half, :] = pltpu.bitcast((_dot(c(i, slice(D, C)), w[1][D:]) + head[i]).astype(BF16), U32)
            else:
                k_buf[half, :] = pltpu.bitcast(_dot(c(i), w[1]).astype(BF16), U32)
            p, rl = softmax(s)
            if i > 0:
                s = scores(st, i - 1)
            context(h, v_buf, i, p, rl)
            v_buf[half, :] = pltpu.bitcast(_dot(c(i), w[2]).astype(BF16), U32)

    L0 = LC * NL
    CR = (S - L0) // NCH
    assert CR * NCH == S - L0 and CR % 16 == 0

    def c_lead_copy(t):
        rows = _rows(t * LC, LC, LC)
        return pltpu.make_async_copy(c_hbm.at[rows, :], c_buf.at[rows, :], sem_c.at[NCH + t])

    def c_tail_copy(j):
        rows = _rows(L0 + j * CR, CR, 16)
        return pltpu.make_async_copy(c_hbm.at[rows, :], c_buf.at[rows, :], sem_c.at[j])

    cp_wr.start()
    for cp in w_copies(wk_hbm, KR, 0, 0) + w_copies(wv_hbm, VR, 0, 0):
        cp.start()
    for t in range(NL):
        c_lead_copy(t).start(priority=1)

    def issue(j, _):
        x_copy(j).start(priority=1)
        c_tail_copy(j).start(priority=1)
        return 0

    lax.fori_loop(0, NCH, issue, 0)
    a_buf[...] = jnp.zeros(a_buf.shape, F32)
    top_buf[...] = jnp.zeros(top_buf.shape, F32)
    cp_wr.wait()
    wr_buf[...] = wr_ref[...].reshape(1, M).astype(F32)

    def unpack_pair(dst, col, start, n):
        for r in range(0, n, 64):
            u = w_load(0, start + r, 64)
            for odd in range(2):
                dst[r // 2:r // 2 + 32, col + odd * D:col + (odd + 1) * D] = pltpu.bitcast(_unpack(u, odd), U32)

    def project_kv(start, size):
        c = c_buf[_rows(start, size, 16), :]
        half = _rows(start >> 1, size // 2, 8)
        cp_buf[half, :] = pltpu.bitcast(c, U32)
        kv = _dot(c, pltpu.bitcast(wp_kv[...], BF16))
        for n, dst in enumerate((k0, k1, v0, v1)):
            dst[half, :] = pltpu.bitcast(kv[:, n * D:(n + 1) * D].astype(BF16), U32)

    w_wait(0, M, 2 * C)
    unpack_pair(wp_kv, 0, *KR)
    unpack_pair(wp_kv, 2 * D, *VR)

    def lead(t, _):
        c_lead_copy(t).wait()

        @pl.when(t == 0)
        def _():
            for cp in w_copies(wq_hbm, QR, 0, 0):
                cp.start()

        project_kv(t * LC, LC)
        return 0

    lax.fori_loop(0, NL, lead, 0)
    w_wait(0, *QR)
    unpack_pair(wp_q, 0, *QR)

    W0 = max(NCH - 5, 0)

    def mid(j, _):
        x_copy(j).wait()
        c_tail_copy(j).wait()

        @pl.when(jnp.logical_and(j >= W0, j < W0 + 4))
        def _():
            w_start(1, 1, [2 * (j - W0), 2 * (j - W0) + 1])

        x = x_buf[_rows(j * TP, TP, TP), :].astype(F32)
        xc = x - jnp.sum(x, axis=-1, keepdims=True) * (1.0 / M)
        var = jnp.sum(xc * xc, axis=-1, keepdims=True) * (1.0 / M)
        xn = (xc * lax.rsqrt(var + EPS)).astype(BF16)
        xn_buf[_rows(j * (TP // 2), TP // 2, TP // 2), :] = pltpu.bitcast(xn, U32)
        project_kv(L0 + j * CR, CR)
        for r in range(0, TP, 64):
            q = _dot(xn[r:r + 64], pltpu.bitcast(wp_q[...], BF16)) * scale
            half = _rows(j * (TP // 2) + r // 2, 32, 32)
            q0[half, :] = pltpu.bitcast(q[:, 0:D].astype(BF16), U32)
            q1[half, :] = pltpu.bitcast(q[:, D:2 * D].astype(BF16), U32)
        return 0

    lax.fori_loop(0, NCH, mid, 0)

    def pair_body(j, _):
        slot = (j + 1) & 1
        w_wait(slot)
        for odd in range(2):
            w = tuple(_unpack(w_load(slot, *r), odd) for r in (QR, KR, VR))
            if odd == 0:
                w_start(jnp.minimum(j + 2, NP - 1), 1 - slot)
                for t, cp in enumerate(big):
                    @pl.when(j == t + 1)
                    def _():
                        cp.start(priority=1)
            attention(2 * j + odd, sets[odd], w, odd == 0)
        return 0

    assert NP - 1 > len(big)
    lax.fori_loop(0, NP - 1, pair_body, 0)

    def last_body(o, _):
        pend = [scores(sets[0], NB - 1 - n, True) for n in range(LK)]
        for i in range(NB - 1, -1, -1):
            half = slice(i * TQ // 2, (i + 1) * TQ // 2)
            p, rl = softmax(pend.pop(0))
            if i >= LK:
                pend.append(scores(sets[0], i - LK, True))
            context(H - 2 + o, v0, i, p, rl)
            q0[half, :] = q1[half, :]
            k0[half, :] = k1[half, :]
            v0[half, :] = v1[half, :]
        return 0

    lax.fori_loop(0, 2, last_body, 0)

    for cp in big:
        cp.wait()
    w_wait(NP & 1)
    nb = S // TM
    NPC = SR // P

    def out_copy(start, size, n):
        rows = _rows(start, size, SR)
        return pltpu.make_async_copy(out_buf.at[rows, :], out_hbm.at[rows, :], sem_out.at[n])

    first_copy = out_copy(0, TM - SR, 0)
    last_copy = out_copy(S - SR, SR, nb)

    def finish(base, a):
        rows = _rows(base, P, P)
        hb = (x_buf[rows, :].astype(F32) + a).astype(BF16)
        x_buf[rows, :] = hb
        h = hb.astype(F32)
        mu = jnp.sum(h, axis=-1, keepdims=True) * (1.0 / M)
        mub = _rb(mu)
        d = h - mub
        dm = mu - mub
        var = jnp.sum(d * d, axis=-1, keepdims=True) * (1.0 / M) - dm * dm
        dw = jnp.sum(d * wr_buf[...], axis=-1, keepdims=True)
        rs = _recip(_rb(jnp.sqrt(_rb(_rb(jnp.maximum(var, 0.0)) + EPS))))
        hnb = (d * rs).astype(BF16)
        hn_buf[rows, :] = hnb
        ob = (h + hnb.astype(F32)).astype(BF16)
        out_buf[rows, :] = ob
        return dw * rs, ob

    def make_key(r, pos):
        r = _rb(r)
        bits = lax.shift_right_logical(pltpu.bitcast(r, jnp.int32), 16)
        o = jnp.where(bits > 0x8000, bits ^ 0xFFFF, bits | 0x8000)
        o = jnp.where(r != r, 0, o)
        return pltpu.bitcast((o << PB) | (S - 1 - pos) | 0x20000000, F32)

    def merge(top, key):
        best, second = top
        return jnp.maximum(best, key), jnp.maximum(second, jnp.minimum(best, key))

    def proj_body(i, _):
        lane = lax.broadcasted_iota(jnp.int32, (P, D), 1)
        rmat = jnp.zeros((P, D), F32)
        for t in range(TM // SR):
            rows = _rows(i * (TM // 2) + t * (SR // 2), SR // 2, SR // 2)
            prev = jnp.maximum(i * TM - SR, 0) if t == 0 else i * TM + (t - 1) * SR
            acc = []
            for hh in range(H):
                ctx = pltpu.bitcast(ctx_buf[hh, rows, :], BF16)
                if (hh + 1) % (H // NPC) == 0:
                    j = (hh + 1) // (H // NPC) - 1
                    ap = a_buf[j * P:(j + 1) * P, :]
                    if hh >= GL:
                        z = _zero_of(acc[hh - GL][0:P, 0:D])
                        ap = pltpu.bitcast(pltpu.bitcast(ap, U32) | jnp.concatenate([z] * (M // D), axis=1), F32)
                    r, ob = finish(prev + j * P, ap)
                    rmat = jnp.where(lane == t * NPC + j, r, rmat)
                    z = pltpu.bitcast(ob, U32)
                    z = _zero_of(functools.reduce(jnp.bitwise_or, [z[:, n * D:(n + 1) * D] for n in range(M // D)]))
                    cu = pltpu.bitcast(ctx, U32)
                    ctx = pltpu.bitcast(jnp.concatenate([cu[:P // 2] | z, cu[P // 2:]], axis=0), BF16)
                a = _dot(ctx, wo_buf[hh * D:(hh + 1) * D, :])
                acc.append(acc[-1] + a if acc else a)
            a_buf[...] = acc[-1]
        pos = i * TM - SR + lane * P + lax.broadcasted_iota(jnp.int32, (P, D), 0)
        live = jnp.logical_and(pos >= 0, lane < TM // P)
        top = merge((top_buf[0], top_buf[1]), jnp.where(live, make_key(rmat, pos), 0.0))
        top_buf[0] = top[0]
        top_buf[1] = top[1]

        @pl.when(i == 0)
        def _():
            first_copy.start()

        @pl.when(i > 0)
        def _():
            out_copy(i * TM - SR, TM, i).start()

        return 0

    lax.fori_loop(0, nb, proj_body, 0)
    best, second = top_buf[0], top_buf[1]
    b = jnp.max(best, axis=1, keepdims=True)
    top = (b, jnp.max(jnp.where(best == b, second, best), axis=1, keepdims=True))
    for j in range(NPC):
        base = S - SR + j * P
        r, _ = finish(base, a_buf[j * P:(j + 1) * P, :])
        top = merge(top, make_key(r, base + lax.broadcasted_iota(jnp.int32, (P, 1), 0)))
    last_copy.start()

    best, second = top
    key1 = jnp.max(best, axis=0, keepdims=True)
    key2 = jnp.max(jnp.where(best == key1, second, best), axis=0, keepdims=True)
    kk = jnp.concatenate([jnp.broadcast_to(key1, (8, 1)), jnp.broadcast_to(key2, (8, 1))], axis=0)
    kk = pltpu.bitcast(kk, jnp.int32)
    i1 = S - 1 - (kk[0, 0] & (S - 1))
    i2 = S - 1 - (kk[8, 0] & (S - 1))
    b1 = pl.multiple_of((i1 >> 4) << 4, 16)
    b2 = pl.multiple_of((i2 >> 4) << 4, 16)
    o = (kk >> PB) & 0xFFFF
    rsel = pltpu.bitcast(jnp.where(o >= 0x8000, o ^ 0x8000, o ^ 0xFFFF) << 16, F32)

    rid = lax.broadcasted_iota(jnp.int32, (16, M), 0)

    def pick(buf):
        rows = [jnp.sum(jnp.where(rid == i - b, buf[pl.ds(b, 16), :].astype(F32), 0.0), axis=0, keepdims=True)
                for i, b in ((i1, b1), (i2, b2))]
        return jnp.concatenate([jnp.broadcast_to(r, (8, M)) for r in rows], axis=0)

    xf = pick(hn_buf)
    xs = xf.astype(BF16)
    hsel = pick(x_buf)
    g = _dot(xs, wg_buf[...])
    u = _dot(xs, wu_buf[...])
    g = _rb(g)
    g = _rb(g * _rb(1.0 / (1.0 + jnp.exp(-g))))
    gu = (g * _rb(u)).astype(BF16)
    y = None
    for t in range(gu.shape[1] // 128):
        yt = _dot(gu[:, t * 128:(t + 1) * 128], wd_buf[t * 128:(t + 1) * 128, :])
        y = yt if y is None else y + yt
    gate = _rb(1.0 / (1.0 + jnp.exp(-rsel)))
    y = _rb(_rb(y) * gate)
    new = hsel + _rb(xf + y)
    n1 = jnp.concatenate([new[0:8], new[0:8]], axis=0).astype(BF16)
    n2 = jnp.concatenate([new[8:16], new[8:16]], axis=0).astype(BF16)

    fix_buf[0:16, :] = jnp.where(rid == i1 - b1, n1, jnp.where(rid == i2 - b1, n2, out_buf[pl.ds(b1, 16), :]))
    fix_buf[16:32, :] = jnp.where(rid == i2 - b2, n2, out_buf[pl.ds(b2, 16), :])

    first_copy.wait()
    for i in range(1, nb):
        out_copy(i * TM - SR, TM, i).wait()
    last_copy.wait()
    f1 = pltpu.make_async_copy(fix_buf.at[pl.ds(0, 16), :], out_hbm.at[pl.ds(b1, 16), :], sem_out.at[0])
    f2 = pltpu.make_async_copy(fix_buf.at[pl.ds(16, 16), :], out_hbm.at[pl.ds(b2, 16), :], sem_out.at[1])
    f1.start()

    @pl.when(b1 != b2)
    def _():
        f2.start()
        f2.wait()

    f1.wait()


@jax.jit
def pallas_sequential_preLN__compressed_kv_cla__moe_arch_mod__prompt_kernel(
    A_x: jax.Array,
    A_c_kv: jax.Array,
    A_w_q: jax.Array,
    A_w_uk: jax.Array,
    A_w_uv: jax.Array,
    A_w_o: jax.Array,
    B_x: jax.Array,
    B_w_r: jax.Array,
    B_w_gate: jax.Array,
    B_w_up: jax.Array,
    B_w_down: jax.Array,
):
    del B_x
    B, S, M = A_x.shape
    assert B == 1 and A_c_kv.shape[1] == S
    C = A_c_kv.shape[2]
    H, D = A_w_q.shape[1], A_w_q.shape[2]
    F = B_w_gate.shape[1]

    any_spec = pl.BlockSpec(memory_space=pl.ANY)
    out = pl.pallas_call(
        _kernel,
        out_shape=jax.ShapeDtypeStruct((S, M), BF16),
        in_specs=[any_spec] * 10,
        out_specs=any_spec,
        scratch_shapes=[
            pltpu.VMEM((S, M), BF16),
            pltpu.VMEM((S // 2, M), U32),
            pltpu.VMEM((S, M), BF16),
            pltpu.VMEM((S, C), BF16),
            pltpu.VMEM((S // 2, C), U32),
            pltpu.VMEM((2, (M + 2 * C) // 8, 16, D), BF16),
            pltpu.VMEM((M // 2, 2 * D), U32),
            pltpu.VMEM((C // 2, 4 * D), U32),
            pltpu.VMEM((M,), BF16),
            pltpu.VMEM((H * D, M), BF16),
            pltpu.VMEM((M, F), BF16),
            pltpu.VMEM((M, F), BF16),
            pltpu.VMEM((F, M), BF16),
            pltpu.VMEM((2, S // 2, D), U32),
            pltpu.VMEM((2, S // 2, D), U32),
            pltpu.VMEM((2, S // 2, D), U32),
            pltpu.VMEM((H, S // 2, D), U32),
            pltpu.VMEM((SR, M), F32),
            pltpu.VMEM((S, M), BF16),
            pltpu.VMEM((32, M), BF16),
            pltpu.VMEM((1, M), F32),
            pltpu.VMEM((2, P, D), F32),
            pltpu.SemaphoreType.DMA((S // TP,)),
            pltpu.SemaphoreType.DMA((S // TP + NL,)),
            pltpu.SemaphoreType.DMA((5,)),
            pltpu.SemaphoreType.DMA((2,)),
            pltpu.SemaphoreType.DMA((S // TM + 1,)),
            pltpu.SMEM((1,), jnp.int32),
        ],
        compiler_params=pltpu.CompilerParams(
            vmem_limit_bytes=120 * 1024 * 1024,
            disable_bounds_checks=True,
            disable_semaphore_checks=True,
        ),
    )(
        A_x.reshape(S, M), A_c_kv.reshape(S, C),
        A_w_q.reshape(M // 8, 8, H, D), A_w_uk.reshape(C // 8, 8, H, D), A_w_uv.reshape(C // 8, 8, H, D),
        A_w_o.reshape(H * D, M), B_w_r, B_w_gate, B_w_up, B_w_down,
    )
    return out.reshape(B, S, M)
```

```python
import functools
import math

import jax
import jax.numpy as jnp
from jax import lax
import jax.experimental.pallas as pl
import jax.experimental.pallas.tpu as pltpu

F32 = jnp.float32
BF16 = jnp.bfloat16
U32 = jnp.uint32
NT = (((1,), (1,)), ((), ()))
NEG = -1e30
EPS = 1e-5
EPS_BF16 = 1.0013580322265625e-05

TQ = 128
TP = 256
LC = 192
NL = 4
TM = 256
SR = 64
P = 16
LK = 4
GL = 6


def _dot(a, b):
    return jnp.dot(a, b, preferred_element_type=F32)


def _rb(x):
    return x.astype(BF16).astype(F32)


def _unpack(u, odd):
    w = (u & U32(0xFFFF0000)) if odd else (u << 16)
    return pltpu.bitcast(w, F32).astype(BF16)


def _recip(x):
    r = pl.reciprocal(x, approx=True)
    return r * (2.0 - x * r)


def _zero_of(x):
    z = pltpu.bitcast(x, U32)
    return lax.shift_right_logical(lax.shift_right_logical(z, U32(16)), U32(16))


def _rows(start, size, mult):
    return pl.ds(start if isinstance(start, int) else pl.multiple_of(start, mult), size)


def _ld(ref, start, stop):
    return pltpu.bitcast(ref[start // 2:stop // 2, :], BF16)


def _kernel(*refs):
    one = refs[-1]
    one[0] = 1

    def body(_, c):
        _body(*refs[:-1])
        return c

    lax.fori_loop(0, one[0], body, 0)


def _body(x_hbm, c_hbm, wq_hbm, wk_hbm, wv_hbm, wo_hbm, wr_hbm, wg_hbm, wu_hbm, wd_hbm,
          out_hbm,
          x_buf, xn_buf, hn_buf, c_buf, cp_buf, w_buf, wp_q, wp_kv, wr_ref, wo_buf, wg_buf, wu_buf, wd_buf,
          q_all, k_all, v_all, ctx_buf, a_buf, out_buf, fix_buf, wr_buf, top_buf,
          sem_x, sem_c, sem_big, sem_w, sem_out):
    S, M = x_buf.shape
    C = c_buf.shape[1]
    H, _, D = ctx_buf.shape
    NP = H // 2
    NB = S // TQ
    NCH = S // TP
    PB = (S - 1).bit_length()
    assert S == 1 << PB and PB <= 13 and NCH >= 4
    scale = (D ** -0.5) * math.log2(math.e)
    sets = tuple((q_all.at[o], k_all.at[o], v_all.at[o]) for o in range(2))
    (q0, k0, v0), (q1, k1, v1) = sets

    QR, KR, VR = (0, M), (M, C), (M + C, C)

    def w_copies(src, rng, p, slot, parts=range(8)):
        return [
            pltpu.make_async_copy(src.at[:, s, pl.ds(2 * p, 2), :],
                                  w_buf.at[slot, pl.ds(rng[0] // 8, rng[1] // 8), pl.ds(2 * s, 2), :],
                                  sem_w.at[slot])
            for s in parts
        ]

    def w_start(p, slot, parts=range(8)):
        for src, rng in ((wk_hbm, KR), (wv_hbm, VR), (wq_hbm, QR)):
            for cp in w_copies(src, rng, p, slot, parts):
                cp.start()

    def w_wait(slot, start=0, n=M + 2 * C):
        part = w_buf.at[slot, pl.ds(start // 8, n // 8)]
        pltpu.make_async_copy(part, part, sem_w.at[slot]).wait()

    def w_load(slot, start, n):
        return pltpu.bitcast(w_buf[slot, start // 8:(start + n) // 8], U32).reshape(n, D)

    def x_copy(j):
        rows = _rows(j * TP, TP, TP)
        return pltpu.make_async_copy(x_hbm.at[rows, :], x_buf.at[rows, :], sem_x.at[j])

    big = [
        pltpu.make_async_copy(wo_hbm, wo_buf, sem_big.at[0]),
        pltpu.make_async_copy(wg_hbm, wg_buf, sem_big.at[1]),
        pltpu.make_async_copy(wu_hbm, wu_buf, sem_big.at[2]),
        pltpu.make_async_copy(wd_hbm, wd_buf, sem_big.at[3]),
    ]
    cp_wr = pltpu.make_async_copy(wr_hbm, wr_ref, sem_big.at[4])

    def scores(st, i, fused=False):
        q_buf, k_buf, _ = st
        row = lax.broadcasted_iota(jnp.int32, (TQ, TQ), 0)
        col = lax.broadcasted_iota(jnp.int32, (TQ, TQ), 1)
        qi = _ld(q_buf, i * TQ, (i + 1) * TQ)
        if fused:
            s = lax.dot_general(qi, _ld(k_buf, 0, (i + 1) * TQ), NT, preferred_element_type=F32)
            sd = jnp.where(col <= row, s[:, i * TQ:], NEG)
            return jnp.concatenate([s[:, :i * TQ], sd], axis=1) if i > 0 else sd
        sd = lax.dot_general(qi, _ld(k_buf, i * TQ, (i + 1) * TQ), NT, preferred_element_type=F32)
        sd = jnp.where(col <= row, sd, NEG)
        if i > 0:
            so = lax.dot_general(qi, _ld(k_buf, 0, i * TQ), NT, preferred_element_type=F32)
            return jnp.concatenate([so, sd], axis=1)
        return sd

    def softmax(s):
        m = jnp.max(s, axis=1, keepdims=True)
        p = jnp.exp2(s - m).astype(BF16)
        l = jnp.sum(p.astype(F32), axis=1, keepdims=True)
        return p, _recip(l)

    def context(h, v_buf, i, p, rl):
        o = _dot(p, _ld(v_buf, 0, (i + 1) * TQ))
        ctx_buf[h, i * TQ // 2:(i + 1) * TQ // 2, :] = pltpu.bitcast((o * rl).astype(BF16), U32)

    def attention(h, st, w, first):
        q_buf, k_buf, v_buf = st

        def c(i, cols=slice(None)):
            return pltpu.bitcast(cp_buf[i * TQ // 2:(i + 1) * TQ // 2, cols], BF16)

        head = {}
        if first:
            head = {i: _dot(c(i, slice(0, D)), w[1][:D]) for i in range(NB - 1, NB - 5, -1)}
        s = scores(st, NB - 1)
        for i in range(NB - 1, -1, -1):
            half = slice(i * TQ // 2, (i + 1) * TQ // 2)
            q_buf[half, :] = pltpu.bitcast((_dot(_ld(xn_buf, i * TQ, (i + 1) * TQ), w[0]) * scale).astype(BF16), U32)
            if i in head:
                k_buf[half, :] = pltpu.bitcast((_dot(c(i, slice(D, C)), w[1][D:]) + head[i]).astype(BF16), U32)
            else:
                k_buf[half, :] = pltpu.bitcast(_dot(c(i), w[1]).astype(BF16), U32)
            p, rl = softmax(s)
            if i > 0:
                s = scores(st, i - 1)
            context(h, v_buf, i, p, rl)
            v_buf[half, :] = pltpu.bitcast(_dot(c(i), w[2]).astype(BF16), U32)

    L0 = LC * NL
    CR = (S - L0) // NCH
    assert CR * NCH == S - L0 and CR % 16 == 0

    def c_lead_copy(t):
        rows = _rows(t * LC, LC, LC)
        return pltpu.make_async_copy(c_hbm.at[rows, :], c_buf.at[rows, :], sem_c.at[NCH + t])

    def c_tail_copy(j):
        rows = _rows(L0 + j * CR, CR, 16)
        return pltpu.make_async_copy(c_hbm.at[rows, :], c_buf.at[rows, :], sem_c.at[j])

    cp_wr.start()
    for cp in w_copies(wk_hbm, KR, 0, 0) + w_copies(wv_hbm, VR, 0, 0):
        cp.start()
    for t in range(NL):
        c_lead_copy(t).start(priority=1)

    def issue(j, _):
        x_copy(j).start(priority=1)
        c_tail_copy(j).start(priority=1)
        return 0

    lax.fori_loop(0, NCH, issue, 0)
    a_buf[...] = jnp.zeros(a_buf.shape, F32)
    top_buf[...] = jnp.zeros(top_buf.shape, F32)
    cp_wr.wait()
    wr_buf[...] = wr_ref[...].reshape(1, M).astype(F32)

    def unpack_pair(dst, col, start, n):
        for r in range(0, n, 64):
            u = w_load(0, start + r, 64)
            for odd in range(2):
                dst[r // 2:r // 2 + 32, col + odd * D:col + (odd + 1) * D] = pltpu.bitcast(_unpack(u, odd), U32)

    def project_kv(start, size):
        c = c_buf[_rows(start, size, 16), :]
        half = _rows(start >> 1, size // 2, 8)
        cp_buf[half, :] = pltpu.bitcast(c, U32)
        kv = _dot(c, pltpu.bitcast(wp_kv[...], BF16))
        for n, dst in enumerate((k0, k1, v0, v1)):
            dst[half, :] = pltpu.bitcast(kv[:, n * D:(n + 1) * D].astype(BF16), U32)

    w_wait(0, M, 2 * C)
    unpack_pair(wp_kv, 0, *KR)
    unpack_pair(wp_kv, 2 * D, *VR)

    def lead(t, _):
        c_lead_copy(t).wait()

        @pl.when(t == 0)
        def _():
            for cp in w_copies(wq_hbm, QR, 0, 0):
                cp.start()

        project_kv(t * LC, LC)
        return 0

    lax.fori_loop(0, NL, lead, 0)
    w_wait(0, *QR)
    unpack_pair(wp_q, 0, *QR)

    W0 = max(NCH - 5, 0)

    def mid(j, _):
        x_copy(j).wait()
        c_tail_copy(j).wait()

        @pl.when(jnp.logical_and(j >= W0, j < W0 + 4))
        def _():
            w_start(1, 1, [2 * (j - W0), 2 * (j - W0) + 1])

        x = x_buf[_rows(j * TP, TP, TP), :].astype(F32)
        xc = x - jnp.sum(x, axis=-1, keepdims=True) * (1.0 / M)
        var = jnp.sum(xc * xc, axis=-1, keepdims=True) * (1.0 / M)
        xn = (xc * lax.rsqrt(var + EPS)).astype(BF16)
        xn_buf[_rows(j * (TP // 2), TP // 2, TP // 2), :] = pltpu.bitcast(xn, U32)
        project_kv(L0 + j * CR, CR)
        for r in range(0, TP, 64):
            q = _dot(xn[r:r + 64], pltpu.bitcast(wp_q[...], BF16)) * scale
            half = _rows(j * (TP // 2) + r // 2, 32, 32)
            q0[half, :] = pltpu.bitcast(q[:, 0:D].astype(BF16), U32)
            q1[half, :] = pltpu.bitcast(q[:, D:2 * D].astype(BF16), U32)
        return 0

    lax.fori_loop(0, NCH, mid, 0)

    def pair_body(j, _):
        slot = (j + 1) & 1
        w_wait(slot)
        for odd in range(2):
            w = tuple(_unpack(w_load(slot, *r), odd) for r in (QR, KR, VR))
            if odd == 0:
                w_start(jnp.minimum(j + 2, NP - 1), 1 - slot)
                for t, cp in enumerate(big):
                    @pl.when(j == t + 1)
                    def _():
                        cp.start(priority=1)
            attention(2 * j + odd, sets[odd], w, odd == 0)
        return 0

    assert NP - 1 > len(big)
    lax.fori_loop(0, NP - 1, pair_body, 0)

    def last_body(o, _):
        pend = [scores(sets[0], NB - 1 - n, True) for n in range(LK)]
        for i in range(NB - 1, -1, -1):
            half = slice(i * TQ // 2, (i + 1) * TQ // 2)
            p, rl = softmax(pend.pop(0))
            if i >= LK:
                pend.append(scores(sets[0], i - LK, True))
            context(H - 2 + o, v0, i, p, rl)
            q0[half, :] = q1[half, :]
            k0[half, :] = k1[half, :]
            v0[half, :] = v1[half, :]
        return 0

    lax.fori_loop(0, 2, last_body, 0)

    for cp in big:
        cp.wait()
    w_wait(NP & 1)
    nb = S // TM
    NPC = SR // P

    def out_copy(start, size, n):
        rows = _rows(start, size, SR)
        return pltpu.make_async_copy(out_buf.at[rows, :], out_hbm.at[rows, :], sem_out.at[n])

    first_copy = out_copy(0, TM - SR, 0)
    last_copy = out_copy(S - SR, SR, nb)

    def finish(base, a):
        rows = _rows(base, P, P)
        hb = (x_buf[rows, :].astype(F32) + a).astype(BF16)
        x_buf[rows, :] = hb
        h = hb.astype(F32)
        mu = jnp.sum(h, axis=-1, keepdims=True) * (1.0 / M)
        mub = _rb(mu)
        d = h - mub
        dm = mu - mub
        var = jnp.sum(d * d, axis=-1, keepdims=True) * (1.0 / M) - dm * dm
        rs = _recip(_rb(jnp.sqrt(_rb(_rb(jnp.maximum(var, 0.0)) + EPS_BF16))))
        hnb = (_rb(d) * rs).astype(BF16)
        hn_buf[rows, :] = hnb
        hn = hnb.astype(F32)
        ob = (h + hn).astype(BF16)
        out_buf[rows, :] = ob
        return jnp.sum(hn * wr_buf[...], axis=-1, keepdims=True), ob

    def make_key(r, pos):
        r = _rb(r)
        bits = lax.shift_right_logical(pltpu.bitcast(r, jnp.int32), 16)
        o = jnp.where(bits > 0x8000, bits ^ 0xFFFF, bits | 0x8000)
        o = jnp.where(r != r, 0, o)
        return pltpu.bitcast((o << PB) | (S - 1 - pos) | 0x20000000, F32)

    def merge(top, key):
        best, second = top
        return jnp.maximum(best, key), jnp.maximum(second, jnp.minimum(best, key))

    def proj_body(i, _):
        lane = lax.broadcasted_iota(jnp.int32, (P, D), 1)
        rmat = jnp.zeros((P, D), F32)
        for t in range(TM // SR):
            rows = _rows(i * (TM // 2) + t * (SR // 2), SR // 2, SR // 2)
            prev = jnp.maximum(i * TM - SR, 0) if t == 0 else i * TM + (t - 1) * SR
            acc = []
            for hh in range(H):
                ctx = pltpu.bitcast(ctx_buf[hh, rows, :], BF16)
                if (hh + 1) % (H // NPC) == 0:
                    j = (hh + 1) // (H // NPC) - 1
                    ap = a_buf[j * P:(j + 1) * P, :]
                    if hh >= GL:
                        z = _zero_of(acc[hh - GL][0:P, 0:D])
                        ap = pltpu.bitcast(pltpu.bitcast(ap, U32) | jnp.concatenate([z] * (M // D), axis=1), F32)
                    r, ob = finish(prev + j * P, ap)
                    rmat = jnp.where(lane == t * NPC + j, r, rmat)
                    z = pltpu.bitcast(ob, U32)
                    z = _zero_of(functools.reduce(jnp.bitwise_or, [z[:, n * D:(n + 1) * D] for n in range(M // D)]))
                    cu = pltpu.bitcast(ctx, U32)
                    ctx = pltpu.bitcast(jnp.concatenate([cu[:P // 2] | z, cu[P // 2:]], axis=0), BF16)
                a = _dot(ctx, wo_buf[hh * D:(hh + 1) * D, :])
                acc.append(acc[-1] + a if acc else a)
            a_buf[...] = acc[-1]
        pos = i * TM - SR + lane * P + lax.broadcasted_iota(jnp.int32, (P, D), 0)
        live = jnp.logical_and(pos >= 0, lane < TM // P)
        top = merge((top_buf[0], top_buf[1]), jnp.where(live, make_key(rmat, pos), 0.0))
        top_buf[0] = top[0]
        top_buf[1] = top[1]

        @pl.when(i == 0)
        def _():
            first_copy.start()

        @pl.when(i > 0)
        def _():
            out_copy(i * TM - SR, TM, i).start()

        return 0

    lax.fori_loop(0, nb, proj_body, 0)
    best, second = top_buf[0], top_buf[1]
    b = jnp.max(best, axis=1, keepdims=True)
    top = (b, jnp.max(jnp.where(best == b, second, best), axis=1, keepdims=True))
    for j in range(NPC):
        base = S - SR + j * P
        r, _ = finish(base, a_buf[j * P:(j + 1) * P, :])
        top = merge(top, make_key(r, base + lax.broadcasted_iota(jnp.int32, (P, 1), 0)))
    last_copy.start()

    best, second = top
    key1 = jnp.max(best, axis=0, keepdims=True)
    key2 = jnp.max(jnp.where(best == key1, second, best), axis=0, keepdims=True)
    kk = jnp.concatenate([jnp.broadcast_to(key1, (8, 1)), jnp.broadcast_to(key2, (8, 1))], axis=0)
    kk = pltpu.bitcast(kk, jnp.int32)
    i1 = S - 1 - (kk[0, 0] & (S - 1))
    i2 = S - 1 - (kk[8, 0] & (S - 1))
    b1 = pl.multiple_of((i1 >> 4) << 4, 16)
    b2 = pl.multiple_of((i2 >> 4) << 4, 16)
    o = (kk >> PB) & 0xFFFF
    rsel = pltpu.bitcast(jnp.where(o >= 0x8000, o ^ 0x8000, o ^ 0xFFFF) << 16, F32)

    rid = lax.broadcasted_iota(jnp.int32, (16, M), 0)

    def pick(buf):
        rows = [jnp.sum(jnp.where(rid == i - b, buf[pl.ds(b, 16), :].astype(F32), 0.0), axis=0, keepdims=True)
                for i, b in ((i1, b1), (i2, b2))]
        return jnp.concatenate([jnp.broadcast_to(r, (8, M)) for r in rows], axis=0)

    xf = pick(hn_buf)
    xs = xf.astype(BF16)
    hsel = pick(x_buf)
    g = _dot(xs, wg_buf[...])
    u = _dot(xs, wu_buf[...])
    g = _rb(g)
    g = _rb(g * _rb(1.0 / (1.0 + jnp.exp(-g))))
    gu = (g * _rb(u)).astype(BF16)
    y = None
    for t in range(gu.shape[1] // 128):
        yt = _dot(gu[:, t * 128:(t + 1) * 128], wd_buf[t * 128:(t + 1) * 128, :])
        y = yt if y is None else y + yt
    gate = _rb(1.0 / (1.0 + jnp.exp(-rsel)))
    y = _rb(_rb(y) * gate)
    new = hsel + _rb(xf + y)
    n1 = jnp.concatenate([new[0:8], new[0:8]], axis=0).astype(BF16)
    n2 = jnp.concatenate([new[8:16], new[8:16]], axis=0).astype(BF16)

    fix_buf[0:16, :] = jnp.where(rid == i1 - b1, n1, jnp.where(rid == i2 - b1, n2, out_buf[pl.ds(b1, 16), :]))
    fix_buf[16:32, :] = jnp.where(rid == i2 - b2, n2, out_buf[pl.ds(b2, 16), :])

    first_copy.wait()
    for i in range(1, nb):
        out_copy(i * TM - SR, TM, i).wait()
    last_copy.wait()
    f1 = pltpu.make_async_copy(fix_buf.at[pl.ds(0, 16), :], out_hbm.at[pl.ds(b1, 16), :], sem_out.at[0])
    f2 = pltpu.make_async_copy(fix_buf.at[pl.ds(16, 16), :], out_hbm.at[pl.ds(b2, 16), :], sem_out.at[1])
    f1.start()

    @pl.when(b1 != b2)
    def _():
        f2.start()
        f2.wait()

    f1.wait()


@jax.jit
def pallas_sequential_preLN__compressed_kv_cla__moe_arch_mod__prompt_kernel(
    A_x: jax.Array,
    A_c_kv: jax.Array,
    A_w_q: jax.Array,
    A_w_uk: jax.Array,
    A_w_uv: jax.Array,
    A_w_o: jax.Array,
    B_x: jax.Array,
    B_w_r: jax.Array,
    B_w_gate: jax.Array,
    B_w_up: jax.Array,
    B_w_down: jax.Array,
):
    del B_x
    B, S, M = A_x.shape
    assert B == 1 and A_c_kv.shape[1] == S
    C = A_c_kv.shape[2]
    H, D = A_w_q.shape[1], A_w_q.shape[2]
    F = B_w_gate.shape[1]

    any_spec = pl.BlockSpec(memory_space=pl.ANY)
    out = pl.pallas_call(
        _kernel,
        out_shape=jax.ShapeDtypeStruct((S, M), BF16),
        in_specs=[any_spec] * 10,
        out_specs=any_spec,
        scratch_shapes=[
            pltpu.VMEM((S, M), BF16),
            pltpu.VMEM((S // 2, M), U32),
            pltpu.VMEM((S, M), BF16),
            pltpu.VMEM((S, C), BF16),
            pltpu.VMEM((S // 2, C), U32),
            pltpu.VMEM((2, (M + 2 * C) // 8, 16, D), BF16),
            pltpu.VMEM((M // 2, 2 * D), U32),
            pltpu.VMEM((C // 2, 4 * D), U32),
            pltpu.VMEM((M,), BF16),
            pltpu.VMEM((H * D, M), BF16),
            pltpu.VMEM((M, F), BF16),
            pltpu.VMEM((M, F), BF16),
            pltpu.VMEM((F, M), BF16),
            pltpu.VMEM((2, S // 2, D), U32),
            pltpu.VMEM((2, S // 2, D), U32),
            pltpu.VMEM((2, S // 2, D), U32),
            pltpu.VMEM((H, S // 2, D), U32),
            pltpu.VMEM((SR, M), F32),
            pltpu.VMEM((S, M), BF16),
            pltpu.VMEM((32, M), BF16),
            pltpu.VMEM((1, M), F32),
            pltpu.VMEM((2, P, D), F32),
            pltpu.SemaphoreType.DMA((S // TP,)),
            pltpu.SemaphoreType.DMA((S // TP + NL,)),
            pltpu.SemaphoreType.DMA((5,)),
            pltpu.SemaphoreType.DMA((2,)),
            pltpu.SemaphoreType.DMA((S // TM + 1,)),
            pltpu.SMEM((1,), jnp.int32),
        ],
        compiler_params=pltpu.CompilerParams(
            vmem_limit_bytes=120 * 1024 * 1024,
            disable_bounds_checks=True,
            disable_semaphore_checks=True,
        ),
    )(
        A_x.reshape(S, M), A_c_kv.reshape(S, C),
        A_w_q.reshape(M // 8, 8, H, D), A_w_uk.reshape(C // 8, 8, H, D), A_w_uv.reshape(C // 8, 8, H, D),
        A_w_o.reshape(H * D, M), B_w_r, B_w_gate, B_w_up, B_w_down,
    )
    return out.reshape(B, S, M)
```

```python
import functools
import math

import jax
import jax.numpy as jnp
from jax import lax
import jax.experimental.pallas as pl
import jax.experimental.pallas.tpu as pltpu

F32 = jnp.float32
BF16 = jnp.bfloat16
U32 = jnp.uint32
NT = (((1,), (1,)), ((), ()))
NEG = -1e30
EPS = 1e-5
EPS_BF16 = 1.0013580322265625e-05

TQ = 128
TP = 256
LC = 192
NL = 4
TM = 256
SUBS = (96, 96, 64)
SR = SUBS[-1]
P = 16
LK = 4
GW = 384


def _dot(a, b):
    return jnp.dot(a, b, preferred_element_type=F32)


def _rb(x):
    return x.astype(BF16).astype(F32)


def _unpack(u, odd):
    w = (u & U32(0xFFFF0000)) if odd else (u << 16)
    return pltpu.bitcast(w, F32).astype(BF16)


def _recip(x):
    r = pl.reciprocal(x, approx=True)
    return r * (2.0 - x * r)


def _zero_of(x):
    z = pltpu.bitcast(x, U32)
    return lax.shift_right_logical(lax.shift_right_logical(z, U32(16)), U32(16))


def _rows(start, size, mult):
    return pl.ds(start if isinstance(start, int) else pl.multiple_of(start, mult), size)


def _ld(ref, start, stop):
    return pltpu.bitcast(ref[start // 2:stop // 2, :], BF16)


def _kernel(*refs):
    one = refs[-1]
    one[0] = 1

    def body(_, c):
        _body(*refs[:-1])
        return c

    lax.fori_loop(0, one[0], body, 0)


def _body(x_hbm, c_hbm, wq_hbm, wk_hbm, wv_hbm, wo_hbm, wr_hbm, wg_hbm, wu_hbm, wd_hbm,
          out_hbm,
          x_buf, xn_buf, hn_buf, c_buf, cp_buf, w_buf, wp_q, wp_kv, wr_ref, wo_buf, wg_buf, wu_buf, wd_buf,
          q_all, k_all, v_all, ctx_buf, a_buf, out_buf, fix_buf, wr_buf, top_buf,
          sem_x, sem_c, sem_big, sem_w, sem_out):
    S, M = x_buf.shape
    C = c_buf.shape[1]
    H, _, D = ctx_buf.shape
    NP = H // 2
    NB = S // TQ
    NCH = S // TP
    PB = (S - 1).bit_length()
    assert S == 1 << PB and PB <= 13 and NCH >= 4
    scale = (D ** -0.5) * math.log2(math.e)
    sets = tuple((q_all.at[o], k_all.at[o], v_all.at[o]) for o in range(2))
    (q0, k0, v0), (q1, k1, v1) = sets

    QR, KR, VR = (0, M), (M, C), (M + C, C)

    def w_copies(src, rng, p, slot, parts=range(8)):
        return [
            pltpu.make_async_copy(src.at[:, s, pl.ds(2 * p, 2), :],
                                  w_buf.at[slot, pl.ds(rng[0] // 8, rng[1] // 8), pl.ds(2 * s, 2), :],
                                  sem_w.at[slot])
            for s in parts
        ]

    def w_start(p, slot, parts=range(8)):
        for src, rng in ((wk_hbm, KR), (wv_hbm, VR), (wq_hbm, QR)):
            for cp in w_copies(src, rng, p, slot, parts):
                cp.start()

    def w_wait(slot, start=0, n=M + 2 * C):
        part = w_buf.at[slot, pl.ds(start // 8, n // 8)]
        pltpu.make_async_copy(part, part, sem_w.at[slot]).wait()

    def w_load(slot, start, n):
        return pltpu.bitcast(w_buf[slot, start // 8:(start + n) // 8], U32).reshape(n, D)

    def x_copy(j):
        rows = _rows(j * TP, TP, TP)
        return pltpu.make_async_copy(x_hbm.at[rows, :], x_buf.at[rows, :], sem_x.at[j])

    big = [
        pltpu.make_async_copy(wo_hbm, wo_buf, sem_big.at[0]),
        pltpu.make_async_copy(wg_hbm, wg_buf, sem_big.at[1]),
        pltpu.make_async_copy(wu_hbm, wu_buf, sem_big.at[2]),
        pltpu.make_async_copy(wd_hbm, wd_buf, sem_big.at[3]),
    ]
    cp_wr = pltpu.make_async_copy(wr_hbm, wr_ref, sem_big.at[4])

    def scores(st, i, fused=False):
        q_buf, k_buf, _ = st
        row = lax.broadcasted_iota(jnp.int32, (TQ, TQ), 0)
        col = lax.broadcasted_iota(jnp.int32, (TQ, TQ), 1)
        qi = _ld(q_buf, i * TQ, (i + 1) * TQ)
        if fused:
            s = lax.dot_general(qi, _ld(k_buf, 0, (i + 1) * TQ), NT, preferred_element_type=F32)
            sd = jnp.where(col <= row, s[:, i * TQ:], NEG)
            return jnp.concatenate([s[:, :i * TQ], sd], axis=1) if i > 0 else sd
        sd = lax.dot_general(qi, _ld(k_buf, i * TQ, (i + 1) * TQ), NT, preferred_element_type=F32)
        sd = jnp.where(col <= row, sd, NEG)
        if i > 0:
            so = lax.dot_general(qi, _ld(k_buf, 0, i * TQ), NT, preferred_element_type=F32)
            return jnp.concatenate([so, sd], axis=1)
        return sd

    def softmax(s):
        m = jnp.max(s, axis=1, keepdims=True)
        p = jnp.exp2(s - m).astype(BF16)
        l = jnp.sum(p.astype(F32), axis=1, keepdims=True)
        return p, _recip(l)

    def context(h, v_buf, i, p, rl):
        o = _dot(p, _ld(v_buf, 0, (i + 1) * TQ))
        ctx_buf[h, i * TQ // 2:(i + 1) * TQ // 2, :] = pltpu.bitcast((o * rl).astype(BF16), U32)

    def attention(h, st, w, first):
        q_buf, k_buf, v_buf = st

        def c(i, cols=slice(None)):
            return pltpu.bitcast(cp_buf[i * TQ // 2:(i + 1) * TQ // 2, cols], BF16)

        head = {}
        if first:
            head = {i: _dot(c(i, slice(0, D)), w[1][:D]) for i in range(NB - 1, NB - 5, -1)}
        s = scores(st, NB - 1)
        for i in range(NB - 1, -1, -1):
            half = slice(i * TQ // 2, (i + 1) * TQ // 2)
            q_buf[half, :] = pltpu.bitcast((_dot(_ld(xn_buf, i * TQ, (i + 1) * TQ), w[0]) * scale).astype(BF16), U32)
            if i in head:
                k_buf[half, :] = pltpu.bitcast((_dot(c(i, slice(D, C)), w[1][D:]) + head[i]).astype(BF16), U32)
            else:
                k_buf[half, :] = pltpu.bitcast(_dot(c(i), w[1]).astype(BF16), U32)
            p, rl = softmax(s)
            if i > 0:
                s = scores(st, i - 1)
            context(h, v_buf, i, p, rl)
            v_buf[half, :] = pltpu.bitcast(_dot(c(i), w[2]).astype(BF16), U32)

    L0 = LC * NL
    CR = (S - L0) // NCH
    assert CR * NCH == S - L0 and CR % 16 == 0

    def c_lead_copy(t):
        rows = _rows(t * LC, LC, LC)
        return pltpu.make_async_copy(c_hbm.at[rows, :], c_buf.at[rows, :], sem_c.at[NCH + t])

    def c_tail_copy(j):
        rows = _rows(L0 + j * CR, CR, 16)
        return pltpu.make_async_copy(c_hbm.at[rows, :], c_buf.at[rows, :], sem_c.at[j])

    cp_wr.start()
    for cp in w_copies(wk_hbm, KR, 0, 0) + w_copies(wv_hbm, VR, 0, 0):
        cp.start()
    for t in range(NL):
        c_lead_copy(t).start(priority=1)

    def issue(j, _):
        x_copy(j).start(priority=1)
        c_tail_copy(j).start(priority=1)
        return 0

    lax.fori_loop(0, NCH, issue, 0)
    a_buf[...] = jnp.zeros(a_buf.shape, F32)
    top_buf[...] = jnp.zeros(top_buf.shape, F32)
    cp_wr.wait()
    wr_buf[...] = wr_ref[...].reshape(1, M).astype(F32)

    def unpack_pair(dst, col, start, n):
        for r in range(0, n, 64):
            u = w_load(0, start + r, 64)
            for odd in range(2):
                dst[r // 2:r // 2 + 32, col + odd * D:col + (odd + 1) * D] = pltpu.bitcast(_unpack(u, odd), U32)

    def project_kv(start, size):
        c = c_buf[_rows(start, size, 16), :]
        half = _rows(start >> 1, size // 2, 8)
        cp_buf[half, :] = pltpu.bitcast(c, U32)
        kv = _dot(c, pltpu.bitcast(wp_kv[...], BF16))
        for n, dst in enumerate((k0, k1, v0, v1)):
            dst[half, :] = pltpu.bitcast(kv[:, n * D:(n + 1) * D].astype(BF16), U32)

    w_wait(0, M, 2 * C)
    unpack_pair(wp_kv, 0, *KR)
    unpack_pair(wp_kv, 2 * D, *VR)

    def lead(t, _):
        c_lead_copy(t).wait()

        @pl.when(t == 0)
        def _():
            for cp in w_copies(wq_hbm, QR, 0, 0):
                cp.start()

        project_kv(t * LC, LC)
        return 0

    lax.fori_loop(0, NL, lead, 0)
    w_wait(0, *QR)
    unpack_pair(wp_q, 0, *QR)

    W0 = max(NCH - 5, 0)

    def mid(j, _):
        x_copy(j).wait()
        c_tail_copy(j).wait()

        @pl.when(jnp.logical_and(j >= W0, j < W0 + 4))
        def _():
            w_start(1, 1, [2 * (j - W0), 2 * (j - W0) + 1])

        x = x_buf[_rows(j * TP, TP, TP), :].astype(F32)
        xc = x - jnp.sum(x, axis=-1, keepdims=True) * (1.0 / M)
        var = jnp.sum(xc * xc, axis=-1, keepdims=True) * (1.0 / M)
        xn = (xc * lax.rsqrt(var + EPS)).astype(BF16)
        xn_buf[_rows(j * (TP // 2), TP // 2, TP // 2), :] = pltpu.bitcast(xn, U32)
        project_kv(L0 + j * CR, CR)
        for r in range(0, TP, 64):
            q = _dot(xn[r:r + 64], pltpu.bitcast(wp_q[...], BF16)) * scale
            half = _rows(j * (TP // 2) + r // 2, 32, 32)
            q0[half, :] = pltpu.bitcast(q[:, 0:D].astype(BF16), U32)
            q1[half, :] = pltpu.bitcast(q[:, D:2 * D].astype(BF16), U32)
        return 0

    lax.fori_loop(0, NCH, mid, 0)

    def pair_body(j, _):
        slot = (j + 1) & 1
        w_wait(slot)
        for odd in range(2):
            w = tuple(_unpack(w_load(slot, *r), odd) for r in (QR, KR, VR))
            if odd == 0:
                w_start(jnp.minimum(j + 2, NP - 1), 1 - slot)
                for t, cp in enumerate(big):
                    @pl.when(j == t + 1)
                    def _():
                        cp.start(priority=1)
            attention(2 * j + odd, sets[odd], w, odd == 0)
        return 0

    assert NP - 1 > len(big)
    lax.fori_loop(0, NP - 1, pair_body, 0)

    def last_body(o, _):
        pend = [scores(sets[0], NB - 1 - n, True) for n in range(LK)]
        for i in range(NB - 1, -1, -1):
            half = slice(i * TQ // 2, (i + 1) * TQ // 2)
            p, rl = softmax(pend.pop(0))
            if i >= LK:
                pend.append(scores(sets[0], i - LK, True))
            context(H - 2 + o, v0, i, p, rl)
            q0[half, :] = q1[half, :]
            k0[half, :] = k1[half, :]
            v0[half, :] = v1[half, :]
        return 0

    lax.fori_loop(0, 2, last_body, 0)

    for cp in big:
        cp.wait()
    w_wait(NP & 1)
    nb = S // TM
    assert sum(SUBS) == TM

    def out_copy(start, size, n):
        rows = _rows(start, size, 16)
        return pltpu.make_async_copy(out_buf.at[rows, :], out_hbm.at[rows, :], sem_out.at[n])

    first_copy = out_copy(0, TM - SR, 0)
    last_copy = out_copy(S - SR, SR, nb)

    def finish(base, a):
        rows = _rows(base, P, P)
        hb = (x_buf[rows, :].astype(F32) + a).astype(BF16)
        x_buf[rows, :] = hb
        h = hb.astype(F32)
        mu = jnp.sum(h, axis=-1, keepdims=True) * (1.0 / M)
        mub = _rb(mu)
        d = h - mub
        dm = mu - mub
        var = jnp.sum(d * d, axis=-1, keepdims=True) * (1.0 / M) - dm * dm
        rs = _recip(_rb(jnp.sqrt(_rb(_rb(jnp.maximum(var, 0.0)) + EPS_BF16))))
        hnb = (_rb(d) * rs).astype(BF16)
        hn_buf[rows, :] = hnb
        hn = hnb.astype(F32)
        ob = (h + hn).astype(BF16)
        out_buf[rows, :] = ob
        return jnp.sum(hn * wr_buf[...], axis=-1, keepdims=True), ob

    def make_key(r, pos):
        r = _rb(r)
        bits = lax.shift_right_logical(pltpu.bitcast(r, jnp.int32), 16)
        o = jnp.where(bits > 0x8000, bits ^ 0xFFFF, bits | 0x8000)
        o = jnp.where(r != r, 0, o)
        return pltpu.bitcast((o << PB) | (S - 1 - pos) | 0x20000000, F32)

    def merge(top, key):
        best, second = top
        return jnp.maximum(best, key), jnp.maximum(second, jnp.minimum(best, key))

    def proj_body(i, _):
        lane = lax.broadcasted_iota(jnp.int32, (P, D), 1)
        rmat = jnp.zeros((P, D), F32)
        off = 0
        npiece = 0
        for t, size in enumerate(SUBS):
            rows = _rows(i * (TM // 2) + off // 2, size // 2, 8)
            prev = jnp.maximum(i * TM - SR, 0) if t == 0 else i * TM + off - SUBS[t - 1]
            npc = SUBS[t - 1] // P
            gl = -(-GW // size)
            due = {max((j + 1) * H // npc - 1, gl + 1 + j): j for j in range(npc)}
            assert len(due) == npc and max(due) < H
            acc = []
            for hh in range(H):
                ctx = pltpu.bitcast(ctx_buf[hh, rows, :], BF16)
                if hh in due:
                    j = due[hh]
                    ap = a_buf[j * P:(j + 1) * P, :]
                    z = _zero_of(acc[hh - gl][0:P, 0:D])
                    ap = pltpu.bitcast(pltpu.bitcast(ap, U32) | jnp.concatenate([z] * (M // D), axis=1), F32)
                    r, ob = finish(prev + j * P, ap)
                    rmat = jnp.where(lane == npiece, r, rmat)
                    npiece += 1
                    z = pltpu.bitcast(ob, U32)
                    z = _zero_of(functools.reduce(jnp.bitwise_or, [z[:, n * D:(n + 1) * D] for n in range(M // D)]))
                    cu = pltpu.bitcast(ctx, U32)
                    ctx = pltpu.bitcast(jnp.concatenate([cu[:P // 2] | z, cu[P // 2:]], axis=0), BF16)
                a = _dot(ctx, wo_buf[hh * D:(hh + 1) * D, :])
                acc.append(acc[-1] + a if acc else a)
            a_buf[0:size, :] = acc[-1]
            off += size
        pos = i * TM - SR + lane * P + lax.broadcasted_iota(jnp.int32, (P, D), 0)
        live = jnp.logical_and(pos >= 0, lane < TM // P)
        top = merge((top_buf[0], top_buf[1]), jnp.where(live, make_key(rmat, pos), 0.0))
        top_buf[0] = top[0]
        top_buf[1] = top[1]

        @pl.when(i == 0)
        def _():
            first_copy.start()

        @pl.when(i > 0)
        def _():
            out_copy(i * TM - SR, TM, i).start()

        return 0

    lax.fori_loop(0, nb, proj_body, 0)
    best, second = top_buf[0], top_buf[1]
    b = jnp.max(best, axis=1, keepdims=True)
    top = (b, jnp.max(jnp.where(best == b, second, best), axis=1, keepdims=True))
    for j in range(SR // P):
        base = S - SR + j * P
        r, _ = finish(base, a_buf[j * P:(j + 1) * P, :])
        top = merge(top, make_key(r, base + lax.broadcasted_iota(jnp.int32, (P, 1), 0)))
    last_copy.start()

    best, second = top
    key1 = jnp.max(best, axis=0, keepdims=True)
    key2 = jnp.max(jnp.where(best == key1, second, best), axis=0, keepdims=True)
    kk = jnp.concatenate([jnp.broadcast_to(key1, (8, 1)), jnp.broadcast_to(key2, (8, 1))], axis=0)
    kk = pltpu.bitcast(kk, jnp.int32)
    i1 = S - 1 - (kk[0, 0] & (S - 1))
    i2 = S - 1 - (kk[8, 0] & (S - 1))
    b1 = pl.multiple_of((i1 >> 4) << 4, 16)
    b2 = pl.multiple_of((i2 >> 4) << 4, 16)
    o = (kk >> PB) & 0xFFFF
    rsel = pltpu.bitcast(jnp.where(o >= 0x8000, o ^ 0x8000, o ^ 0xFFFF) << 16, F32)

    rid = lax.broadcasted_iota(jnp.int32, (16, M), 0)

    def pick(buf):
        rows = [jnp.sum(jnp.where(rid == i - b, buf[pl.ds(b, 16), :].astype(F32), 0.0), axis=0, keepdims=True)
                for i, b in ((i1, b1), (i2, b2))]
        return jnp.concatenate([jnp.broadcast_to(r, (8, M)) for r in rows], axis=0)

    xf = pick(hn_buf)
    xs = xf.astype(BF16)
    hsel = pick(x_buf)
    g = _dot(xs, wg_buf[...])
    u = _dot(xs, wu_buf[...])
    g = _rb(g)
    g = _rb(g * _rb(1.0 / (1.0 + jnp.exp(-g))))
    gu = (g * _rb(u)).astype(BF16)
    y = None
    for t in range(gu.shape[1] // 128):
        yt = _dot(gu[:, t * 128:(t + 1) * 128], wd_buf[t * 128:(t + 1) * 128, :])
        y = yt if y is None else y + yt
    gate = _rb(1.0 / (1.0 + jnp.exp(-rsel)))
    y = _rb(_rb(y) * gate)
    new = hsel + _rb(xf + y)
    n1 = jnp.concatenate([new[0:8], new[0:8]], axis=0).astype(BF16)
    n2 = jnp.concatenate([new[8:16], new[8:16]], axis=0).astype(BF16)

    fix_buf[0:16, :] = jnp.where(rid == i1 - b1, n1, jnp.where(rid == i2 - b1, n2, out_buf[pl.ds(b1, 16), :]))
    fix_buf[16:32, :] = jnp.where(rid == i2 - b2, n2, out_buf[pl.ds(b2, 16), :])

    first_copy.wait()
    for i in range(1, nb):
        out_copy(i * TM - SR, TM, i).wait()
    last_copy.wait()
    f1 = pltpu.make_async_copy(fix_buf.at[pl.ds(0, 16), :], out_hbm.at[pl.ds(b1, 16), :], sem_out.at[0])
    f2 = pltpu.make_async_copy(fix_buf.at[pl.ds(16, 16), :], out_hbm.at[pl.ds(b2, 16), :], sem_out.at[1])
    f1.start()

    @pl.when(b1 != b2)
    def _():
        f2.start()
        f2.wait()

    f1.wait()


@jax.jit
def pallas_sequential_preLN__compressed_kv_cla__moe_arch_mod__prompt_kernel(
    A_x: jax.Array,
    A_c_kv: jax.Array,
    A_w_q: jax.Array,
    A_w_uk: jax.Array,
    A_w_uv: jax.Array,
    A_w_o: jax.Array,
    B_x: jax.Array,
    B_w_r: jax.Array,
    B_w_gate: jax.Array,
    B_w_up: jax.Array,
    B_w_down: jax.Array,
):
    del B_x
    B, S, M = A_x.shape
    assert B == 1 and A_c_kv.shape[1] == S
    C = A_c_kv.shape[2]
    H, D = A_w_q.shape[1], A_w_q.shape[2]
    F = B_w_gate.shape[1]

    any_spec = pl.BlockSpec(memory_space=pl.ANY)
    out = pl.pallas_call(
        _kernel,
        out_shape=jax.ShapeDtypeStruct((S, M), BF16),
        in_specs=[any_spec] * 10,
        out_specs=any_spec,
        scratch_shapes=[
            pltpu.VMEM((S, M), BF16),
            pltpu.VMEM((S // 2, M), U32),
            pltpu.VMEM((S, M), BF16),
            pltpu.VMEM((S, C), BF16),
            pltpu.VMEM((S // 2, C), U32),
            pltpu.VMEM((2, (M + 2 * C) // 8, 16, D), BF16),
            pltpu.VMEM((M // 2, 2 * D), U32),
            pltpu.VMEM((C // 2, 4 * D), U32),
            pltpu.VMEM((M,), BF16),
            pltpu.VMEM((H * D, M), BF16),
            pltpu.VMEM((M, F), BF16),
            pltpu.VMEM((M, F), BF16),
            pltpu.VMEM((F, M), BF16),
            pltpu.VMEM((2, S // 2, D), U32),
            pltpu.VMEM((2, S // 2, D), U32),
            pltpu.VMEM((2, S // 2, D), U32),
            pltpu.VMEM((H, S // 2, D), U32),
            pltpu.VMEM((max(SUBS), M), F32),
            pltpu.VMEM((S, M), BF16),
            pltpu.VMEM((32, M), BF16),
            pltpu.VMEM((1, M), F32),
            pltpu.VMEM((2, P, D), F32),
            pltpu.SemaphoreType.DMA((S // TP,)),
            pltpu.SemaphoreType.DMA((S // TP + NL,)),
            pltpu.SemaphoreType.DMA((5,)),
            pltpu.SemaphoreType.DMA((2,)),
            pltpu.SemaphoreType.DMA((S // TM + 1,)),
            pltpu.SMEM((1,), jnp.int32),
        ],
        compiler_params=pltpu.CompilerParams(
            vmem_limit_bytes=120 * 1024 * 1024,
            disable_bounds_checks=True,
            disable_semaphore_checks=True,
        ),
    )(
        A_x.reshape(S, M), A_c_kv.reshape(S, C),
        A_w_q.reshape(M // 8, 8, H, D), A_w_uk.reshape(C // 8, 8, H, D), A_w_uv.reshape(C // 8, 8, H, D),
        A_w_o.reshape(H * D, M), B_w_r, B_w_gate, B_w_up, B_w_down,
    )
    return out.reshape(B, S, M)
```
